```python
import jax
import jax.numpy as jnp

def _softmax(x, axis=-1):
    return jax.nn.softmax(x, axis=axis)
def _gelu(x):
    return jax.nn.gelu(x, approximate=True)
def _silu(x):
    return jax.nn.silu(x)
def _sigmoid(x):
    return jax.nn.sigmoid(x)
def _layernorm(x, axis=-1, eps=1e-5):
    m = jnp.mean(x, axis=axis, keepdims=True)
    v = jnp.var(x, axis=axis, keepdims=True)
    return (x - m) / jnp.sqrt(v + eps)
def _scatter_add(tgt, idx, src, axis=0):
    return tgt.at[idx].add(src)
def _segment_sum(src, seg, n):
    return jax.ops.segment_sum(src, seg, n)
class _Rng:
    def __init__(self, key):
        self._k = key
    def _next(self):
        self._k, sub = jax.random.split(self._k)
        return sub
    def normal(self, shape):
        return jax.random.normal(self._next(), shape, dtype=jnp.bfloat16)
    def randint(self, lo, hi, shape):
        return jax.random.randint(self._next(), shape, lo, hi, dtype=jnp.int32)
    def uniform(self, shape, lo=0.0, hi=1.0):
        return jax.random.uniform(self._next(), shape, jnp.bfloat16, lo, hi)
    def permutation(self, n):
        return jax.random.permutation(self._next(), n)


kernel_name = 'sequential_preLN__sliding_local_dilated__moe_arch_mod__prompt'

def setup_inputs():
    _rng = _Rng(jax.random.key(int.from_bytes(__import__("os").urandom(4), "little")))
    _w = (lambda a: (lambda t: t.astype(jnp.bfloat16) if jnp.issubdtype(t.dtype, jnp.floating) else t)(jnp.asarray(a)))
    def _A_setup():
        B, S, D = 1, 2048, 640
        return {
            "x": _w((lambda *s: _rng.normal(s) * 0.05)(B, S, D)),
            "wqkv": _w((lambda *s: _rng.normal(s) * 0.05)(D, 3 * D)),
            "wo": _w((lambda *s: _rng.normal(s) * 0.05)(D, D)),
        }
    _A_in = _A_setup()

    def _B_setup():
        B, S, D, F, C = 1, 2048, 640, 1536, 1
        return {
            "x": _w((lambda *s: _rng.normal(s) * 0.05)(B, S, D)),
            "w_r": _w((lambda *s: _rng.normal(s) * 0.05)(D)),
            "w_gate": _w((lambda *s: _rng.normal(s) * 0.05)(D, F)),
            "w_up": _w((lambda *s: _rng.normal(s) * 0.05)(D, F)),
            "w_down": _w((lambda *s: _rng.normal(s) * 0.05)(F, D)),
        }
    _B_in = _B_setup()

    return {
        "A_x": _A_in["x"],
        "A_wqkv": _A_in["wqkv"],
        "A_wo": _A_in["wo"],
        "B_x": _B_in["x"],
        "B_w_r": _B_in["w_r"],
        "B_w_gate": _B_in["w_gate"],
        "B_w_up": _B_in["w_up"],
        "B_w_down": _B_in["w_down"],
    }

def reference(A_x, A_wqkv, A_wo, B_x, B_w_r, B_w_gate, B_w_up, B_w_down):
    def _A_ref(x, wqkv, wo):
        B, S, D = x.shape
        H = 32; Dh = D // H
        W, dil = 8, 2
        qkv = (lambda x, *d: x.transpose(*d))((x @ wqkv).reshape(B, S, 3, H, Dh), 2, 0, 3, 1, 4)
        q, k, v = qkv[0], qkv[1], qkv[2]
        scale = Dh ** -0.5
        pos = jnp.arange(S)
        off = jnp.arange(W) * dil
        idx = pos[:, None] - off[None, :]
        mask = idx >= 0
        idx_c = jnp.where(mask, idx, 0).reshape(-1)
        kg = k[:, :, idx_c, :].reshape(B, H, S, W, Dh)
        vg = v[:, :, idx_c, :].reshape(B, H, S, W, Dh)
        logits = jnp.einsum("bhsd,bhswd->bhsw", q, kg) * scale
        logits = jnp.where(mask[None, None, :, :], logits, -1e9)
        attn = _softmax(logits, axis=-1)
        o = jnp.einsum("bhsw,bhswd->bhsd", attn, vg)
        return (lambda x, *d: x.transpose(*d))(o, 0, 2, 1, 3).reshape(B, S, D) @ wo

    def _B_ref(x, w_r, w_gate, w_up, w_down):
        B, S, D = x.shape
        C = 1
        r = x @ w_r
        idx = jnp.argsort(-r, axis=-1)[:, :C]
        idx_e = jnp.repeat(idx.reshape(B, C, 1), D, axis=2)
        x_sel = jnp.take_along_axis(x, idx_e, axis=1)
        g = _silu(x_sel @ w_gate)
        u = x_sel @ w_up
        y = (g * u) @ w_down
        r_sel = _sigmoid(jnp.take_along_axis(r, idx, axis=1))
        y = y * r_sel.reshape(B, C, 1)
        b_off = (jnp.arange(B) * S).reshape(B, 1)
        flat_idx = (idx + b_off).reshape(B * C)
        zero = (x * 0.0).reshape(B * S, D)
        upd = _scatter_add(zero, flat_idx, y.reshape(B * C, D), axis=0)
        return x + upd.reshape(B, S, D)

    x = A_x
    h = x + _A_ref(_layernorm(x, axis=-1), A_wqkv, A_wo)
    h2 = h + _B_ref(_layernorm(h, axis=-1), B_w_r, B_w_gate, B_w_up, B_w_down)
    return h2
```

```python
import functools
import math

import jax
import jax.numpy as jnp
from jax import lax
import jax.experimental.pallas as pl
import jax.experimental.pallas.tpu as pltpu

S = 2048
D = 640
H = 32
DH = 20
W = 8
DIL = 2
F = 1536
NJ = D // 128
HALO = 16
EPS = 1e-5
LOG2E = math.log2(math.e)
QSCALE = (DH ** -0.5) * LOG2E
NEG = -1e9 * LOG2E

TM = 256
NB = S // TM
RC = 8

f32 = jnp.float32
bf16 = jnp.bfloat16
u32 = jnp.uint32


def _layernorm(x):
    m = jnp.sum(x, axis=-1, keepdims=True) * (1.0 / D)
    xc = x - m
    v = jnp.sum(xc * xc, axis=-1, keepdims=True) * (1.0 / D)
    return xc * lax.rsqrt(v + EPS)


def _kernel(x_hbm, wqkv_hbm, wo_hbm, wr_ref, wg_hbm, wu_hbm, wd_hbm, out_hbm,
            xbuf, wraw, woraw, wp, wop, wg, wu, wd,
            xn, qb, kb, vb, ob, ln2b, outb, patch,
            sem_x, sem_w, sem_o, sem_p):
    def x_cp(i):
        return pltpu.make_async_copy(x_hbm.at[0, pl.ds(i * TM, TM), :],
                                     xbuf.at[pl.ds(i * TM, TM), :], sem_x.at[i])

    def wqkv_cp(p):
        return pltpu.make_async_copy(wqkv_hbm.at[:, pl.ds(p * D, D)],
                                     wraw.at[p], sem_w.at[p])

    def wo_cp(j):
        return pltpu.make_async_copy(wo_hbm.at[:, pl.ds(j * 128, 128)],
                                     woraw.at[j], sem_w.at[3 + j])

    ffn_cps = [pltpu.make_async_copy(wg_hbm, wg, sem_w.at[8]),
               pltpu.make_async_copy(wu_hbm, wu, sem_w.at[9]),
               pltpu.make_async_copy(wd_hbm, wd, sem_w.at[10])]

    def out_cp(i):
        return pltpu.make_async_copy(outb.at[pl.ds(i * TM, TM), :],
                                     out_hbm.at[0, pl.ds(i * TM, TM), :], sem_o.at[i])

    x_cp(0).start()
    for p in range(3):
        wqkv_cp(p).start()
    for j in range(NJ):
        wo_cp(j).start()
    for i in range(1, NB):
        x_cp(i).start()
    for c in ffn_cps:
        c.start()

    for j in range(NJ):
        kb[j, 0:HALO, :] = jnp.zeros((HALO, 128), f32)
        vb[j, 0:HALO, :] = jnp.zeros((HALO, 128), f32)

    lane = lax.broadcasted_iota(jnp.int32, (8, 128), 1)
    lm5 = lane % 5
    base_idx = 20 * (lane % 32) + 5 * (lane // 32)

    def permute_part(p):
        for j in range(NJ):
            idx = (base_idx + j) % 128
            masks = [lm5 == ((j - 3 * i) % 5) for i in range(NJ)]

            def body(rg, c):
                r0 = pl.multiple_of(rg * 16, 16)
                src = [pltpu.bitcast(wraw[p, pl.ds(r0, 16), i * 128:(i + 1) * 128], u32)
                       for i in range(NJ)]
                z = src[0]
                for i in range(1, NJ):
                    z = jnp.where(masks[i], src[i], z)
                o = jnp.take_along_axis(z, idx, axis=1)
                wp[pl.ds(pl.multiple_of(rg * 8, 8), 8),
                   p * D + j * 128: p * D + (j + 1) * 128] = o
                return c
            lax.fori_loop(0, D // 16, body, 0, unroll=8)

    for p in range(3):
        wqkv_cp(p).wait()
        permute_part(p)

    def permute_wo():
        for c in range(NJ):
            src = woraw.at[c].bitcast(u32)
            for m in range(DH // 2):
                for half in range(2):
                    a = src[pl.ds(m + 160 * half, 8, stride=20), :]
                    b = src[pl.ds(m + 10 + 160 * half, 8, stride=20), :]
                    lo = (a & jnp.uint32(0xFFFF)) | (b << 16)
                    hi = (a >> 16) | (b & jnp.uint32(0xFFFF0000))
                    for d, val in ((2 * m, lo), (2 * m + 1, hi)):
                        j, g = d % 5, d // 5
                        r = (j * 128 + g * 32) // 2 + 8 * half
                        wop[r:r + 8, c * 128:(c + 1) * 128] = val

    for j in range(NJ):
        wo_cp(j).wait()
    permute_wo()

    wr = wr_ref[...].astype(f32).reshape(1, D)

    def stage_a(i):
        r0 = i * TM
        x = xbuf[r0:r0 + TM, :].astype(f32)
        xn[...] = pltpu.bitcast(_layernorm(x).astype(bf16), u32)
        lhs = pltpu.bitcast(xn[...], bf16)
        rhs = pltpu.bitcast(wp[...], bf16)
        qkv = jnp.dot(lhs, rhs, preferred_element_type=f32)
        for j in range(NJ):
            qb[j, r0:r0 + TM, :] = qkv[:, j * 128:(j + 1) * 128] * QSCALE
            kb[j, HALO + r0:HALO + r0 + TM, :] = qkv[:, D + j * 128:D + (j + 1) * 128]
            vb[j, HALO + r0:HALO + r0 + TM, :] = qkv[:, 2 * D + j * 128:2 * D + (j + 1) * 128]

    def stage_b(i, best):
        r0 = i * TM
        for c in range(TM // 16):
            halves = []
            for hh in range(2):
                a0 = r0 + c * 16 + hh * 8
                q = [qb[j, a0:a0 + 8, :] for j in range(NJ)]
                s = []
                for w in range(W):
                    k0 = HALO + a0 - DIL * w
                    t = q[0] * kb[0, k0:k0 + 8, :]
                    for j in range(1, NJ):
                        t = t + q[j] * kb[j, k0:k0 + 8, :]
                    t = t + pltpu.roll(t, 64, 1)
                    t = t + pltpu.roll(t, 32, 1)
                    if a0 - DIL * w < 0:
                        row = lax.broadcasted_iota(jnp.int32, (8, 128), 0) + (a0 - DIL * w)
                        t = jnp.where(row >= 0, t, NEG)
                    s.append(t)
                mx = s[0]
                for w in range(1, W):
                    mx = jnp.maximum(mx, s[w])
                p = [jnp.exp2(s[w] - mx) for w in range(W)]
                l = p[0]
                for w in range(1, W):
                    l = l + p[w]
                inv = pl.reciprocal(l, approx=True)
                o = []
                for j in range(NJ):
                    acc = None
                    for w in range(W):
                        k0 = HALO + a0 - DIL * w
                        term = p[w] * vb[j, k0:k0 + 8, :]
                        acc = term if acc is None else acc + term
                    o.append(acc * inv)
                halves.append(o)
            for j in range(NJ):
                o16 = jnp.concatenate([halves[0][j], halves[1][j]], axis=0).astype(bf16)
                ob[c * 8:(c + 1) * 8, j * 128:(j + 1) * 128] = pltpu.bitcast(o16, u32)
        att = jnp.dot(pltpu.bitcast(ob[...], bf16), pltpu.bitcast(wop[...], bf16),
                      preferred_element_type=f32)
        h = xbuf[r0:r0 + TM, :].astype(f32) + att
        ln2 = _layernorm(h)
        ln2b[r0 // 2:(r0 + TM) // 2, :] = pltpu.bitcast(ln2.astype(bf16), u32)
        outb[r0:r0 + TM, :] = (h + ln2).astype(bf16)
        r = jnp.sum(ln2 * wr, axis=-1, keepdims=True)
        bmax = jnp.max(r, axis=0, keepdims=True)
        rows = lax.broadcasted_iota(jnp.int32, (TM, 1), 0) + r0
        bidx = jnp.min(jnp.where(r == bmax, rows, S), axis=0, keepdims=True)
        if best is None:
            return bmax, bidx
        take = bmax > best[0]
        return jnp.where(take, bmax, best[0]), jnp.where(take, bidx, best[1])

    best = None
    x_cp(0).wait()
    stage_a(0)
    for i in range(1, NB):
        x_cp(i).wait()
    for i in range(NB):
        if i + 1 < NB:
            stage_a(i + 1)
        best = stage_b(i, best)
        out_cp(i).start()

    for c in ffn_cps:
        c.wait()
    rbest, ibest = best
    idx = jnp.clip(jnp.max(ibest), 0, S - 1)
    t16 = idx // 16
    xs = pltpu.bitcast(ln2b[pl.ds(pl.multiple_of(t16 * 8, 8), 8), :], bf16)
    g = jnp.dot(xs, wg[...], preferred_element_type=f32)
    u = jnp.dot(xs, wu[...], preferred_element_type=f32)
    a = (g * jax.nn.sigmoid(g) * u).astype(bf16)
    y = jnp.dot(a, wd[...], preferred_element_type=f32) * jax.nn.sigmoid(rbest)
    t0 = pl.multiple_of(t16 * 16, 16)
    rows = lax.broadcasted_iota(jnp.int32, (16, D), 0) + t0
    cur = outb[pl.ds(t0, 16), :].astype(f32)
    patch[...] = (cur + jnp.where(rows == idx, y, 0.0)).astype(bf16)
    for i in range(NB):
        out_cp(i).wait()
    pcp = pltpu.make_async_copy(patch, out_hbm.at[0, pl.ds(t0, 16), :], sem_p)
    pcp.start()
    pcp.wait()


@jax.jit
def pallas_sequential_preLN__sliding_local_dilated__moe_arch_mod__prompt_kernel(
    A_x: jax.Array,
    A_wqkv: jax.Array,
    A_wo: jax.Array,
    B_x: jax.Array,
    B_w_r: jax.Array,
    B_w_gate: jax.Array,
    B_w_up: jax.Array,
    B_w_down: jax.Array,
):
    del B_x
    any_spec = pl.BlockSpec(memory_space=pl.ANY)
    return pl.pallas_call(
        _kernel,
        in_specs=[any_spec, any_spec, any_spec,
                  pl.BlockSpec(memory_space=pltpu.VMEM),
                  any_spec, any_spec, any_spec],
        out_specs=any_spec,
        out_shape=jax.ShapeDtypeStruct((1, S, D), bf16),
        scratch_shapes=[
            pltpu.VMEM((S, D), bf16),
            pltpu.VMEM((3, D, D), bf16),
            pltpu.VMEM((NJ, D, 128), bf16),
            pltpu.VMEM((D // 2, 3 * D), u32),
            pltpu.VMEM((D // 2, D), u32),
            pltpu.VMEM((D, F), bf16),
            pltpu.VMEM((D, F), bf16),
            pltpu.VMEM((F, D), bf16),
            pltpu.VMEM((TM // 2, D), u32),
            pltpu.VMEM((NJ, S, 128), f32),
            pltpu.VMEM((NJ, HALO + S, 128), f32),
            pltpu.VMEM((NJ, HALO + S, 128), f32),
            pltpu.VMEM((TM // 2, D), u32),
            pltpu.VMEM((S // 2, D), u32),
            pltpu.VMEM((S, D), bf16),
            pltpu.VMEM((16, D), bf16),
            pltpu.SemaphoreType.DMA((NB,)),
            pltpu.SemaphoreType.DMA((11,)),
            pltpu.SemaphoreType.DMA((NB,)),
            pltpu.SemaphoreType.DMA,
        ],
        compiler_params=pltpu.CompilerParams(vmem_limit_bytes=100 * 1024 * 1024),
        name="preln_swa_mod",
    )(A_x, A_wqkv, A_wo, B_w_r, B_w_gate, B_w_up, B_w_down)
```

```python
import functools
import math

import jax
import jax.numpy as jnp
from jax import lax
import jax.experimental.pallas as pl
import jax.experimental.pallas.tpu as pltpu

S = 2048; D = 640; H = 32; DH = 20; W = 8; DIL = 2; F = 1536
NJ = D // 128
NF = F // 128
HALO = 16
EPS = 1e-5
LOG2E = math.log2(math.e)
QSCALE = (DH ** -0.5) * LOG2E
NEG = -1e9 * LOG2E

BLOCKS = [int(t) for t in "256,256,256,256,256,256,256,128,128".split(",")]
assert sum(BLOCKS) == S
NB = len(BLOCKS)
R0 = [sum(BLOCKS[:i]) for i in range(NB)]
TM = max(BLOCKS)
LASTF = float(0.85)
LEAD = float(300)
RCF = int(32)
LCF = int(64)
SPEC = int(1)
XD = 256
NXD = S // XD

f32 = jnp.float32
bf16 = jnp.bfloat16
u32 = jnp.uint32
i32 = jnp.int32


def _cat(xs):
    return jnp.concatenate(xs, axis=1)


def _kernel(x_hbm, wqkv_hbm, wo_hbm, wr_hbm, wg_hbm, wu_hbm, wd_hbm, out_hbm,
            xbuf, wraw, woraw, wp, wop, wg, wu, wd, wr_ref, wrb,
            xn0, xn1, qb0, qb1, kb0, kb1, vb0, vb1, ob0, ob1, ln2b, outb, patch,
            bestv, besti, zero_ref, sem):
    xn = (xn0, xn1); qb = (qb0, qb1); kb = (kb0, kb1); vb = (vb0, vb1); ob = (ob0, ob1)

    nsem = [0]

    def group(pairs):
        s = sem.at[nsem[0]]
        nsem[0] += 1
        return [pltpu.make_async_copy(a, b, s) for a, b in pairs]

    def cols(j):
        return pl.ds(j * 128, 128)

    x_cps = [group([(x_hbm.at[0, pl.ds(i * XD, XD), cols(j)], xbuf.at[j, pl.ds(i * XD, XD), :])
                    for j in range(NJ)]) for i in range(NXD)]
    HR = D // 2
    wq_cps = [group([(wqkv_hbm.at[pl.ds(hf * HR, HR), cols(j)], wraw.at[j, pl.ds(hf * HR, HR), :])
                     for j in range(NJ)]) for hf in range(2)]
    wkv_cps = [group([(wqkv_hbm.at[:, cols(p * NJ + j)], wraw.at[p * NJ + j]) for j in range(NJ)])
               for p in (1, 2)]
    wo_cps = group([(wo_hbm.at[:, cols(j)], woraw.at[j]) for j in range(NJ)] + [(wr_hbm, wr_ref)])
    ffn_cps = group([(wg_hbm.at[:, cols(n)], wg.at[n]) for n in range(NF)]
                    + [(wu_hbm.at[:, cols(n)], wu.at[n]) for n in range(NF)]
                    + [(wd_hbm.at[:, cols(j)], wd.at[j]) for j in range(NJ)])
    out_cps = [group([(outb.at[j, pl.ds(R0[b], BLOCKS[b]), :],
                       out_hbm.at[0, pl.ds(R0[b], BLOCKS[b]), cols(j)]) for j in range(NJ)])
               for b in range(NB)]
    sem_p = sem.at[nsem[0]]
    assert nsem[0] + 1 == NSEM

    def start(cs):
        for c in cs:
            c.start()

    def wait(cs):
        for c in cs:
            c.wait()

    def permute_part(p, rgs):
        lane = lax.broadcasted_iota(i32, (8, 128), 1)
        lm5 = lane % 5
        base_idx = 20 * (lane % 32) + 5 * (lane // 32)
        for j in range(NJ):
            idx = (base_idx + j) % 128
            masks = [lm5 == ((j - 3 * i) % 5) for i in range(NJ)]
            for rg in rgs:
                src = [wraw.at[p * NJ + i].bitcast(u32)[rg * 8:rg * 8 + 8, :] for i in range(NJ)]
                z = src[0]
                for i in range(1, NJ):
                    z = jnp.where(masks[i], src[i], z)
                o = jnp.take_along_axis(z, idx, axis=1)
                wp[rg * 8:rg * 8 + 8, p * D + j * 128: p * D + (j + 1) * 128] = o

    def permute_wo():
        for c in range(NJ):
            src = woraw.at[c].bitcast(u32)
            for m in range(DH // 2):
                for half in range(2):
                    a = src[pl.ds(m + 160 * half, 8, stride=20), :]
                    b = src[pl.ds(m + 10 + 160 * half, 8, stride=20), :]
                    lo = (a & jnp.uint32(0xFFFF)) | (b << 16)
                    hi = (a >> 16) | (b & jnp.uint32(0xFFFF0000))
                    for d, val in ((2 * m, lo), (2 * m + 1, hi)):
                        j, g = d % 5, d // 5
                        r = (j * 128 + g * 32) // 2 + 8 * half
                        wop[r:r + 8, c * 128:(c + 1) * 128] = val

    class Ctx:
        def __init__(self):
            self._never = None
            self.best = None
            self.res = []
            self.t = 0.0

        def add(self, val):
            dur = val.shape[0] * NJ / 4.0
            self.res.append((self.t, self.t + dur, val))
            self.t += dur

        def gate(self, t, val):
            if t is None or t < 0 or not self.res:
                return val
            for (t0, t1, tv) in self.res:
                if t < t1:
                    break
            frac = min(max((t - t0) / (t1 - t0), 0.0), 0.999)
            r = int(frac * (tv.shape[0] // 8)) * 8
            tok = tv[r:r + 8, :]
            if self._never is None:
                self._never = zero_ref[...] != 0
            if val.dtype != tok.dtype:
                tok = pltpu.bitcast(tok, val.dtype)
            return jnp.where(self._never, tok, val)

    def spread(t0, t1, c, n):
        return None if t0 is None else t0 + max(t1 - t0, 0.0) * c / n

    def load_x(cx, r, lc, t):
        out = []
        for j in range(NJ):
            v = xbuf.at[j].bitcast(u32)
            parts = [cx.gate(t, v[(r + k) // 2:(r + k) // 2 + 8, :]) for k in range(0, lc, 16)]
            v = parts[0] if len(parts) == 1 else jnp.concatenate(parts, axis=0)
            out.append(pltpu.bitcast(v, bf16).astype(f32))
        return _cat(out)

    def center(x):
        m = jnp.sum(x, axis=-1, keepdims=True) * (1.0 / D)
        xc = x - m
        v = jnp.sum(xc * xc, axis=-1, keepdims=True) * (1.0 / D)
        return xc, lax.rsqrt(v + EPS)

    def ln1(cx, b, t0=None, t1=None, lc=16):
        n = BLOCKS[b] // lc
        for c in range(n):
            xc, rs = center(load_x(cx, R0[b] + c * lc, lc, spread(t0, t1, c, n)))
            xn[b % 2][c * lc // 2:(c + 1) * lc // 2, :] = pltpu.bitcast((xc * rs).astype(bf16), u32)

    def qkv_tiles(cx, b, tiles):
        m = BLOCKS[b]
        lhs = pltpu.bitcast(xn[b % 2][0:m // 2, :], bf16)
        for n in tiles:
            rhs = pltpu.bitcast(wp[:, n * 128:(n + 1) * 128], bf16)
            t = jnp.dot(lhs, rhs, preferred_element_type=f32)
            cx.add(t)
            p, j = divmod(n, NJ)
            if p == 0:
                qb[b % 2][j, 0:m, :] = t
            else:
                dst = (kb, vb)[p - 1]
                if b > 0:
                    mp = BLOCKS[b - 1]
                    dst[b % 2][j, 0:HALO, :] = dst[(b - 1) % 2][j, mp:mp + HALO, :]
                dst[b % 2][j, HALO:HALO + m, :] = t

    def attn(cx, b, t0=None, t1=None, rc=8):
        qr, kr, vr = qb[b % 2], kb[b % 2], vb[b % 2]
        n = BLOCKS[b] // rc
        for c in range(n):
            a0 = c * rc
            sc = cx.gate(spread(t0, t1, c, n), jnp.full((8, 128), QSCALE, f32))
            if rc > 8:
                sc = jnp.tile(sc, (rc // 8, 1))
            q = [qr[j, a0:a0 + rc, :] * sc for j in range(NJ)]
            tt = []
            for w in range(W):
                k0 = HALO + a0 - DIL * w
                acc = q[0] * kr[0, k0:k0 + rc, :]
                for j in range(1, NJ):
                    acc = acc + q[j] * kr[j, k0:k0 + rc, :]
                tt.append(acc)
            r1 = [pltpu.roll(tt[w], 64, 1) for w in range(W)]
            tt = [tt[w] + r1[w] for w in range(W)]
            r2 = [pltpu.roll(tt[w], 32, 1) for w in range(W)]
            s = [tt[w] + r2[w] for w in range(W)]
            for w in range(W):
                if b == 0 and a0 - DIL * w < 0:
                    row = lax.broadcasted_iota(i32, (rc, 128), 0) + (a0 - DIL * w)
                    s[w] = jnp.where(row >= 0, s[w], NEG)
            mx = functools.reduce(jnp.maximum, s)
            p = [jnp.exp2(s[w] - mx) for w in range(W)]
            l = functools.reduce(lambda a, b: a + b, p)
            inv = pl.reciprocal(l, approx=True)
            o = []
            for j in range(NJ):
                acc = None
                for w in range(W):
                    k0 = HALO + a0 - DIL * w
                    term = p[w] * vr[j, k0:k0 + rc, :]
                    acc = term if acc is None else acc + term
                o.append(acc * inv)
            if rc == 8 and c % 2 == 0:
                prev = o
                continue
            if rc == 8:
                o = [jnp.concatenate([prev[j], o[j]], axis=0) for j in range(NJ)]
                a0 -= 8
            rows = o[0].shape[0]
            for j in range(NJ):
                ob[b % 2][a0 // 2:(a0 + rows) // 2, j * 128:(j + 1) * 128] = pltpu.bitcast(o[j].astype(bf16), u32)

    def wo_tiles(cx, b):
        m = BLOCKS[b]
        lhs = pltpu.bitcast(ob[b % 2][0:m // 2, :], bf16)
        att = []
        for n in range(NJ):
            rhs = pltpu.bitcast(wop[:, n * 128:(n + 1) * 128], bf16)
            t = jnp.dot(lhs, rhs, preferred_element_type=f32)
            cx.add(t)
            att.append(t)
        return att

    def post(cx, b, att, t0=None, t1=None, lc=16):
        r0 = R0[b]
        n = BLOCKS[b] // lc
        for c in range(n):
            a0 = c * lc
            h = load_x(cx, r0 + a0, lc, spread(t0, t1, c, n)) + _cat([att[j][a0:a0 + lc, :] for j in range(NJ)])
            xc, rs = center(h)
            r = jnp.sum(xc * jnp.tile(wrb[...], (lc // 8, 1)), axis=-1, keepdims=True) * rs
            ln2 = xc * rs
            ln2b[(r0 + a0) // 2:(r0 + a0 + lc) // 2, :] = pltpu.bitcast(ln2.astype(bf16), u32)
            o = pltpu.bitcast((h + ln2).astype(bf16), u32)
            for j in range(NJ):
                outb.at[j].bitcast(u32)[(r0 + a0) // 2:(r0 + a0 + lc) // 2, :] = o[:, j * 128:(j + 1) * 128]
            for k in range(0, lc, 8):
                rk = r[k:k + 8, :]
                if cx.best is None:
                    cx.best = (rk, jnp.full((8, 1), r0 + a0 + k, i32))
                else:
                    bv, bi = cx.best
                    take = rk > bv
                    cx.best = (jnp.where(take, rk, bv), jnp.where(take, r0 + a0 + k, bi))
        start(out_cps[b])

    def load_best(cx):
        cx.best = (bestv[:, 0:1], besti[:, 0:1])

    def save_best(cx):
        bestv[...] = jnp.broadcast_to(cx.best[0], (8, 128))
        besti[...] = jnp.broadcast_to(cx.best[1], (8, 128))

    def argmax_of(bv, bi):
        rowid = bi + lax.broadcasted_iota(i32, (8, 128), 0)
        rbest = jnp.max(bv, axis=0, keepdims=True)
        idx = jnp.clip(jnp.min(jnp.where(bv == rbest, rowid, S)), 0, S - 1)
        return rbest, idx

    def ffn_up(idx):
        t16 = idx // 16
        xs = pltpu.bitcast(ln2b[pl.ds(pl.multiple_of(t16 * 8, 8), 8), :], bf16)
        a = []
        for n in range(NF):
            g = jnp.dot(xs, pltpu.bitcast(wg.at[n].bitcast(u32)[...], bf16), preferred_element_type=f32)
            u = jnp.dot(xs, pltpu.bitcast(wu.at[n].bitcast(u32)[...], bf16), preferred_element_type=f32)
            a.append((g * jax.nn.sigmoid(g) * u).astype(bf16))
        return _cat(a)

    def ffn_down(a, rbest, idx):
        sg = jax.nn.sigmoid(rbest)
        t16 = idx // 16
        hit = (lax.broadcasted_iota(i32, (16, 128), 0) + t16 * 16) == idx
        for j in range(NJ):
            y = jnp.dot(a, pltpu.bitcast(wd.at[j].bitcast(u32)[...], bf16), preferred_element_type=f32) * sg
            cur = pltpu.bitcast(outb.at[j].bitcast(u32)[pl.ds(pl.multiple_of(t16 * 8, 8), 8), :], bf16).astype(f32)
            patch[:, j * 128:(j + 1) * 128] = (cur + jnp.where(hit, y, 0.0)).astype(bf16)

    def patch_cp(idx):
        t0 = pl.multiple_of((idx // 16) * 16, 16)
        return pltpu.make_async_copy(patch, out_hbm.at[0, pl.ds(t0, 16), :], sem_p)

    waited = set()

    def wait_x(b):
        if b < NB:
            for i in range(R0[b] // XD, (R0[b] + BLOCKS[b] - 1) // XD + 1):
                if i not in waited:
                    waited.add(i)
                    wait(x_cps[i])

    def g0():
        start(x_cps[0]); start(wq_cps[0]); start(wq_cps[1]); start(x_cps[1])
        start(wkv_cps[0]); start(wkv_cps[1]); start(x_cps[2]); start(wo_cps)
        for i in range(3, NXD):
            start(x_cps[i])
        start(ffn_cps)
        zero_ref[...] = jnp.zeros((8, 128), i32)
        for j in range(NJ):
            kb0[j, 0:HALO, :] = jnp.zeros((HALO, 128), f32)
            vb0[j, 0:HALO, :] = jnp.zeros((HALO, 128), f32)
        cx = Ctx()
        wait_x(0)
        ln1(cx, 0, lc=64)
        wait(wq_cps[0])
        permute_part(0, range(0, 20))
        wait(wq_cps[1])
        permute_part(0, range(20, 40))

    def g1():
        cx = Ctx()
        wait_x(1)
        qkv_tiles(cx, 0, range(0, 5))
        ln1(cx, 1, -LEAD, LASTF * cx.t - LEAD)

    def g2():
        cx = Ctx()
        wait(wkv_cps[0])
        qkv_tiles(cx, 1, range(0, 5))
        permute_part(1, range(40))

    def g3():
        cx = Ctx()
        wait(wkv_cps[1])
        qkv_tiles(cx, 0, range(5, 10))
        permute_part(2, range(40))
        qkv_tiles(cx, 0, range(10, 15))

    def g4():
        cx = Ctx()
        wait_x(2)
        wait(wo_cps)
        wrb[...] = jnp.broadcast_to(wr_ref[...].astype(f32).reshape(1, D), (8, D))
        qkv_tiles(cx, 1, range(5, 15))
        permute_wo()
        attn(cx, 0, -LEAD, LASTF * cx.t - LEAD)
        ln1(cx, 2, -LEAD, LASTF * cx.t - LEAD)

    def main_step(i):
        cx = Ctx()
        wait_x(i + 2)
        if i > 1:
            load_best(cx)
        att = wo_tiles(cx, i - 1)
        tw = cx.t
        qkv_tiles(cx, i + 1, range(15))
        tl = LASTF * cx.t - LEAD
        attn(cx, i, -LEAD, tl)
        if i + 2 < NB:
            ln1(cx, i + 2, -LEAD, tw - LEAD)
        post(cx, i - 1, att, tw, tl)
        save_best(cx)

    L = NB - 1

    def final():
        cx = Ctx()
        wait(ffn_cps)
        for b in range(L - 1):
            wait(out_cps[b])
        bv0, bi0 = bestv[...], besti[...]
        if SPEC:
            rbest0, idx0 = argmax_of(bv0, bi0)
        att = wo_tiles(cx, L - 1)
        if SPEC:
            a = ffn_up(idx0)
        attn(cx, L, rc=RCF)
        att2 = wo_tiles(cx, L)
        if SPEC:
            ffn_down(a, rbest0, idx0)
        post(cx, L - 1, att, lc=min(LCF, BLOCKS[L - 1]))
        post(cx, L, att2, lc=min(LCF, BLOCKS[L]))
        bv1 = jnp.broadcast_to(cx.best[0], (8, 128))
        bi1 = jnp.broadcast_to(cx.best[1], (8, 128))

        def redo():
            take = bv1 > bv0
            rbest, idx = argmax_of(jnp.where(take, bv1, bv0), jnp.where(take, bi1, bi0))
            ffn_down(ffn_up(idx), rbest, idx)
            wait(out_cps[L - 1]); wait(out_cps[L])
            pc = patch_cp(idx)
            pc.start()
            pc.wait()

        if SPEC:
            miss = jnp.max(jnp.where(bv1 > rbest0, 1, 0)) > 0
            pl.when(miss)(redo)

            @pl.when(jnp.logical_not(miss))
            def _():
                pc = patch_cp(idx0)
                pc.start()
                wait(out_cps[L - 1]); wait(out_cps[L])
                pc.wait()
        else:
            redo()

    steps = [g0, g1, g2, g3, g4] + [functools.partial(main_step, i) for i in range(1, L)] + [final]
    assert len(steps) == NSTEPS
    pid = pl.program_id(0)
    for n, fn in enumerate(steps):
        pl.when(pid == n)(fn)


NSTEPS = 5 + (NB - 2) + 1
NSEM = NXD + 2 + 2 + 1 + 1 + NB + 1


@jax.jit
def pallas_sequential_preLN__sliding_local_dilated__moe_arch_mod__prompt_kernel(
    A_x, A_wqkv, A_wo, B_x, B_w_r, B_w_gate, B_w_up, B_w_down,
):
    del B_x
    any_spec = pl.BlockSpec(memory_space=pl.ANY)
    return pl.pallas_call(
        _kernel,
        grid=(NSTEPS,),
        in_specs=[any_spec] * 7,
        out_specs=any_spec,
        out_shape=jax.ShapeDtypeStruct((1, S, D), bf16),
        scratch_shapes=[
            pltpu.VMEM((NJ, S, 128), bf16),
            pltpu.VMEM((3 * NJ, D, 128), bf16),
            pltpu.VMEM((NJ, D, 128), bf16),
            pltpu.VMEM((D // 2, 3 * D), u32),
            pltpu.VMEM((D // 2, D), u32),
            pltpu.VMEM((NF, D, 128), bf16),
            pltpu.VMEM((NF, D, 128), bf16),
            pltpu.VMEM((NJ, F, 128), bf16),
            pltpu.VMEM((D,), bf16),
            pltpu.VMEM((8, D), f32),
            pltpu.VMEM((TM // 2, D), u32),
            pltpu.VMEM((TM // 2, D), u32),
            pltpu.VMEM((NJ, TM, 128), f32),
            pltpu.VMEM((NJ, TM, 128), f32),
            pltpu.VMEM((NJ, HALO + TM, 128), f32),
            pltpu.VMEM((NJ, HALO + TM, 128), f32),
            pltpu.VMEM((NJ, HALO + TM, 128), f32),
            pltpu.VMEM((NJ, HALO + TM, 128), f32),
            pltpu.VMEM((TM // 2, D), u32),
            pltpu.VMEM((TM // 2, D), u32),
            pltpu.VMEM((S // 2, D), u32),
            pltpu.VMEM((NJ, S, 128), bf16),
            pltpu.VMEM((16, D), bf16),
            pltpu.VMEM((8, 128), f32),
            pltpu.VMEM((8, 128), i32),
            pltpu.VMEM((8, 128), i32),
            pltpu.SemaphoreType.DMA((NSEM,)),
        ],
        compiler_params=pltpu.CompilerParams(vmem_limit_bytes=100 * 1024 * 1024,
                                             dimension_semantics=("arbitrary",),
                                             disable_semaphore_checks=bool(int(1))),
        name="preln_swa_mod",
    )(A_x, A_wqkv, A_wo, B_w_r, B_w_gate, B_w_up, B_w_down)
```

```python
import functools
import math

import jax
import jax.numpy as jnp
from jax import lax
import jax.experimental.pallas as pl
import jax.experimental.pallas.tpu as pltpu

S = 2048; D = 640; H = 32; DH = 20; W = 8; DIL = 2; F = 1536
NJ = D // 128
NF = F // 128
HALO = 16
EPS = 1e-5
LOG2E = math.log2(math.e)
QSCALE = (DH ** -0.5) * LOG2E
NEG = -1e9 * LOG2E

BLOCKS = [int(t) for t in "256,256,256,256,256,256,256,128,128".split(",")]
assert sum(BLOCKS) == S
NB = len(BLOCKS)
R0 = [sum(BLOCKS[:i]) for i in range(NB)]
TM = max(BLOCKS)
LASTF = float(0.92)
FSPLIT = int(3)
PER = {int(a.split(":")[0]): (float(a.split(":")[1]), float(a.split(":")[2]))
       for a in "5:150:0.95,6:150:0.95,7:150:0.95,8:150:0.95,9:150:0.95,10:100:0.87,11:100:0.87".split(",") if a}
LEAD = float(200)
RCF = int(16)
LCF = int(32)
SPEC = int(1)
NOH = int(0)
KSPLIT = int(1)
FLAT = int(1)
FG = float(700)
FGL = float(200)
PG = float(0)
PSPAN = float(300)
PGRP = int(8)
PF = float(0.8)
PL = float(200)
LN2G3 = int(0)
GIANT = int(0)
HOMO = int(0)
LN2S1 = int(0)
FASTRS = int(1)
CUTS = [int(c) for c in "".split(",") if c]
SPARE = 8
XD = 256
NXD = S // XD
assert BLOCKS[0] <= XD and BLOCKS[0] + BLOCKS[1] == 2 * XD

f32 = jnp.float32
bf16 = jnp.bfloat16
u32 = jnp.uint32
i32 = jnp.int32


def _cat(xs):
    return jnp.concatenate(xs, axis=1)


def _kernel(x_hbm, wqkv_hbm, wo_hbm, wr_hbm, wg_hbm, wu_hbm, wd_hbm, out_hbm,
            xbuf, xpre, wraw, woraw, wp, wop, wg, wu, wd, wr_ref, wrb,
            xn0, xn1, qb0, qb1, kb0, kb1, vb0, vb1, ob0, ob1, ln2b, outb, patch,
            bestv, besti, zero_ref, one, sem):
    xn = (xn0, xn1); qb = (qb0, qb1); kb = (kb0, kb1); vb = (vb0, vb1); ob = (ob0, ob1)

    nsem = [0]

    def group(pairs):
        s = sem.at[nsem[0]]
        nsem[0] += 1
        return [pltpu.make_async_copy(a, b, s) for a, b in pairs]

    def cols(j):
        return pl.ds(j * 128, 128)

    x_cps = [group([(x_hbm.at[0, pl.ds(i * XD, XD), cols(j)], xbuf.at[j, pl.ds(i * XD, XD), :])
                    for j in range(NJ)]) if i >= 2 else None for i in range(NXD)]
    HR = D // 2
    xp_cps = [group([(x_hbm.at[0, pl.ds(i * XD, XD), :], xpre.at[pl.ds(i * XD, XD), :])]) for i in range(2)]
    wq_cps = [group([(wqkv_hbm.at[pl.ds(hf * HR, HR), pl.ds(0, D)], wraw.at[0, pl.ds(hf * HR, HR), :])])
              for hf in range(2)]
    wkv_cps = [group([(wqkv_hbm.at[:, pl.ds(p * D, D)], wraw.at[p])]) for p in (1, 2)]
    wo_cps = group([(wo_hbm.at[:, cols(j)], woraw.at[j]) for j in range(NJ)] + [(wr_hbm, wr_ref)])
    ffn_cps = group([(wg_hbm.at[:, cols(n)], wg.at[n]) for n in range(NF)]
                    + [(wu_hbm.at[:, cols(n)], wu.at[n]) for n in range(NF)]
                    + [(wd_hbm.at[:, cols(j)], wd.at[j]) for j in range(NJ)])
    out_cps = [group([(outb.at[j, pl.ds(R0[b], BLOCKS[b]), :],
                       out_hbm.at[0, pl.ds(R0[b], BLOCKS[b]), cols(j)]) for j in range(NJ)])
               for b in range(NB)]
    sem_p = sem.at[nsem[0]]
    assert nsem[0] + 1 == NSEM

    def start(cs):
        for c in cs:
            c.start()

    def wait(cs):
        for c in cs:
            c.wait()

    def permute_part(p, rgs, cx=None, t0=None, t1=None):
        lane = lax.broadcasted_iota(i32, (8, 128), 1)
        lm5 = lane % 5
        base_idx = 20 * (lane % 32) + 5 * (lane // 32)
        rgs = list(rgs)
        ngrp = NJ * ((len(rgs) + PGRP - 1) // PGRP)
        gi = 0
        for j in range(NJ):
            idx = (base_idx + j) % 128
            for k, rg in enumerate(rgs):
                if k % PGRP == 0:
                    lg = lm5 if cx is None else cx.gate(spread(t0, t1, gi, ngrp), lm5)
                    masks = [lg == ((j - 3 * i) % 5) for i in range(NJ)]
                    gi += 1
                src = [pltpu.bitcast(wraw[p, rg * 16:rg * 16 + 16, i * 128:(i + 1) * 128], u32) for i in range(NJ)]
                z = src[0]
                for i in range(1, NJ):
                    z = jnp.where(masks[i], src[i], z)
                o = jnp.take_along_axis(z, idx, axis=1)
                wp[rg * 8:rg * 8 + 8, p * D + j * 128: p * D + (j + 1) * 128] = o

    def permute_wo():
        for c in range(NJ):
            src = woraw.at[c].bitcast(u32)
            for m in range(DH // 2):
                for half in range(2):
                    a = src[pl.ds(m + 160 * half, 8, stride=20), :]
                    b = src[pl.ds(m + 10 + 160 * half, 8, stride=20), :]
                    lo = (a & jnp.uint32(0xFFFF)) | (b << 16)
                    hi = (a >> 16) | (b & jnp.uint32(0xFFFF0000))
                    for d, val in ((2 * m, lo), (2 * m + 1, hi)):
                        j, g = d % 5, d // 5
                        r = (j * 128 + g * 32) // 2 + 8 * half
                        wop[r:r + 8, c * 128:(c + 1) * 128] = val

    class Ctx:
        def __init__(self):
            self._never = None
            self.best = None
            self.res = []
            self.pend = []
            self.done = []
            self.t = 0.0

        def add(self, val, dur):
            self.res.append((self.t, self.t + dur, val))
            self.t += dur

        def gate(self, t, val):
            if t is None or t < 0 or not self.res:
                return val
            for (t0, t1, tv) in self.res:
                if t < t1:
                    break
            frac = min(max((t - t0) / (t1 - t0), 0.0), 0.999)
            r = int(frac * (tv.shape[0] // 8)) * 8
            tok = tv[r:r + 8, :]
            if self._never is None:
                self._never = zero_ref[...] != 0
            if val.dtype != tok.dtype:
                tok = pltpu.bitcast(tok, val.dtype)
            return jnp.where(self._never, tok, val)

    def emit_tiles(cx):
        pend, cx.pend = cx.pend, []
        KA = 512
        groups = []
        for p in pend:
            if groups and len(groups[-1]) < 4 and (groups[-1][0][0].shape == p[0].shape or not HOMO):
                groups[-1].append(p)
            else:
                groups.append([p])
        for grp in groups:
            if not KSPLIT:
                for lhs, wref, n, sink in grp:
                    rhs = pltpu.bitcast(wref[:, n * 128:(n + 1) * 128], bf16)
                    t = jnp.dot(lhs, rhs, preferred_element_type=f32)
                    cx.add(t, lhs.shape[0] * NJ / 4.0)
                    sink(t)
                continue
            tb = []
            for lhs, wref, n, sink in grp:
                rhs = pltpu.bitcast(wref[KA // 2:, n * 128:(n + 1) * 128], bf16)
                if len(grp) == 4 or not HOMO:
                    tb.append(jnp.dot(lhs[:, KA:], rhs, preferred_element_type=f32))
                else:
                    mq = lhs.shape[0] // 4
                    tb.append(jnp.concatenate(
                        [jnp.dot(lhs[r:r + mq, KA:], rhs, preferred_element_type=f32)
                         for r in range(0, 4 * mq, mq)], axis=0))
            cx.add(tb[-1], sum(p[0].shape[0] for p in grp) / 4.0)
            for (lhs, wref, n, sink), b in zip(grp, tb):
                rhs = pltpu.bitcast(wref[:KA // 2, n * 128:(n + 1) * 128], bf16)
                t = jnp.dot(lhs[:, :KA], rhs, preferred_element_type=f32) + b
                cx.add(t, float(lhs.shape[0]))
                sink(t)

    def spread(t0, t1, c, n):
        return None if t0 is None else t0 + max(t1 - t0, 0.0) * c / n

    def load_x(cx, r, lc, t, pre=False):
        out = []
        for j in range(NJ):
            if pre:
                parts = [cx.gate(t, pltpu.bitcast(xpre[r + k:r + k + 16, j * 128:(j + 1) * 128], u32))
                         for k in range(0, lc, 16)]
            else:
                v = xbuf.at[j].bitcast(u32)
                parts = [cx.gate(t, v[(r + k) // 2:(r + k) // 2 + 8, :]) for k in range(0, lc, 16)]
            v = parts[0] if len(parts) == 1 else jnp.concatenate(parts, axis=0)
            out.append(pltpu.bitcast(v, bf16).astype(f32))
        return _cat(out)

    def center(x):
        m = jnp.sum(x, axis=-1, keepdims=True) * (1.0 / D)
        xc = x - m
        v = jnp.sum(xc * xc, axis=-1, keepdims=True) * (1.0 / D)
        if FASTRS:
            return xc, jnp.exp2(jnp.log(v + EPS) * (-0.5 * LOG2E)), m
        return xc, lax.rsqrt(v + EPS), m

    def ln1(cx, b, t0=None, t1=None, lc=16, lo=0, hi=None):
        hi = BLOCKS[b] if hi is None else hi
        starts = list(range(lo, hi, lc))
        for c, a0 in enumerate(starts):
            n = min(lc, hi - a0)
            xc, rs, _ = center(load_x(cx, R0[b] + a0, n, spread(t0, t1, c, len(starts)), pre=b < 2))
            y = xc * rs
            xn[b % 2][a0 // 2:(a0 + n) // 2, :] = pltpu.bitcast(y.astype(bf16), u32)
            cx.done.append(pltpu.bitcast(y[0:8, 512:640], u32))

    def qkv_tiles(cx, b, tiles):
        m = BLOCKS[b]
        lhs = pltpu.bitcast(xn[b % 2][0:m // 2, :], bf16)

        def sink(n, t):
            p, j = divmod(n, NJ)
            if p == 0:
                qb[b % 2][j, 0:m, :] = t
            else:
                dst = (kb, vb)[p - 1]
                if b > 0:
                    mp = BLOCKS[b - 1]
                    dst[b % 2][j, 0:HALO, :] = dst[(b - 1) % 2][j, mp:mp + HALO, :]
                dst[b % 2][j, HALO:HALO + m, :] = t
        for n in tiles:
            cx.pend.append((lhs, wp, n, functools.partial(sink, n)))

    def attn(cx, b, t0=None, t1=None, rc=8):
        qr, kr, vr = qb[b % 2], kb[b % 2], vb[b % 2]
        n = BLOCKS[b] // rc
        for c in range(n):
            a0 = c * rc
            sc = cx.gate(spread(t0, t1, c, n), jnp.full((8, 128), QSCALE, f32))
            if rc > 8:
                sc = jnp.tile(sc, (rc // 8, 1))
            q = [qr[j, a0:a0 + rc, :] * sc for j in range(NJ)]
            tt = []
            for w in range(W):
                k0 = HALO + a0 - DIL * w
                acc = q[0] * kr[0, k0:k0 + rc, :]
                for j in range(1, NJ):
                    acc = acc + q[j] * kr[j, k0:k0 + rc, :]
                tt.append(acc)
            r1 = [pltpu.roll(tt[w], 64, 1) for w in range(W)]
            tt = [tt[w] + r1[w] for w in range(W)]
            r2 = [pltpu.roll(tt[w], 32, 1) for w in range(W)]
            s = [tt[w] + r2[w] for w in range(W)]
            for w in range(W):
                if b == 0 and a0 - DIL * w < 0:
                    row = lax.broadcasted_iota(i32, (rc, 128), 0) + (a0 - DIL * w)
                    s[w] = jnp.where(row >= 0, s[w], NEG)
            mx = functools.reduce(jnp.maximum, s)
            p = [jnp.exp2(s[w] - mx) for w in range(W)]
            l = functools.reduce(lambda a, b: a + b, p)
            inv = pl.reciprocal(l, approx=True)
            o = []
            for j in range(NJ):
                acc = None
                for w in range(W):
                    k0 = HALO + a0 - DIL * w
                    term = p[w] * vr[j, k0:k0 + rc, :]
                    acc = term if acc is None else acc + term
                o.append(acc * inv)
            if rc == 8 and c % 2 == 0:
                prev = o
                continue
            if rc == 8:
                o = [jnp.concatenate([prev[j], o[j]], axis=0) for j in range(NJ)]
                a0 -= 8
            rows = o[0].shape[0]
            for j in range(NJ):
                ob[b % 2][a0 // 2:(a0 + rows) // 2, j * 128:(j + 1) * 128] = pltpu.bitcast(o[j].astype(bf16), u32)

    def wo_tiles(cx, b):
        m = BLOCKS[b]
        lhs = pltpu.bitcast(ob[b % 2][0:m // 2, :], bf16)
        att = []

        def sink(t):
            att.append(t)
            cx.tw = cx.t
        for n in range(NJ):
            cx.pend.append((lhs, wop, n, sink))
        return att

    def post(cx, b, att, t0=None, t1=None, lc=16):
        r0 = R0[b]
        n = BLOCKS[b] // lc
        for c in range(n):
            a0 = c * lc
            h = load_x(cx, r0 + a0, lc, spread(t0, t1, c, n), pre=b < 2) + _cat([att[j][a0:a0 + lc, :] for j in range(NJ)])
            xc, rs, mean = center(h)
            r = jnp.sum(xc * jnp.tile(wrb[...], (lc // 8, 1)), axis=-1, keepdims=True) * rs
            ln2 = xc * rs
            ln2b[(r0 + a0) // 2:(r0 + a0 + lc) // 2, :] = pltpu.bitcast(ln2.astype(bf16), u32)
            o = pltpu.bitcast(((xc * (rs + 1.0) + mean) if NOH else (h + ln2)).astype(bf16), u32)
            for j in range(NJ):
                outb.at[j].bitcast(u32)[(r0 + a0) // 2:(r0 + a0 + lc) // 2, :] = o[:, j * 128:(j + 1) * 128]
            for k in range(0, lc, 8):
                rk = r[k:k + 8, :]
                if cx.best is None:
                    cx.best = (rk, jnp.full((8, 1), r0 + a0 + k, i32))
                else:
                    bv, bi = cx.best
                    take = rk > bv
                    cx.best = (jnp.where(take, rk, bv), jnp.where(take, r0 + a0 + k, bi))
        cx.done.append(pltpu.bitcast(jnp.broadcast_to(cx.best[0], (8, 128)), u32))
        start(out_cps[b])

    def load_best(cx):
        cx.best = (bestv[:, 0:1], besti[:, 0:1])

    def save_best(cx):
        bestv[...] = jnp.broadcast_to(cx.best[0], (8, 128))
        besti[...] = jnp.broadcast_to(cx.best[1], (8, 128))

    def argmax_of(bv, bi):
        rowid = bi + lax.broadcasted_iota(i32, (8, 128), 0)
        rbest = jnp.max(bv, axis=0, keepdims=True)
        idx = jnp.clip(jnp.min(jnp.where(bv == rbest, rowid, S)), 0, S - 1)
        return rbest, idx

    def ffn_up(idx, tiles=range(NF)):
        t16 = idx // 16
        xs = pltpu.bitcast(ln2b[pl.ds(pl.multiple_of(t16 * 8, 8), 8), :], bf16)
        a = []
        for n in tiles:
            g = jnp.dot(xs, pltpu.bitcast(wg.at[n].bitcast(u32)[...], bf16), preferred_element_type=f32)
            u = jnp.dot(xs, pltpu.bitcast(wu.at[n].bitcast(u32)[...], bf16), preferred_element_type=f32)
            a.append((g * jax.nn.sigmoid(g) * u).astype(bf16))
        return a

    def ffn_down(a, rbest, idx):
        a = _cat(a)
        sg = jax.nn.sigmoid(rbest)
        t16 = idx // 16
        hit = (lax.broadcasted_iota(i32, (16, 128), 0) + t16 * 16) == idx
        for j in range(NJ):
            y = jnp.dot(a, pltpu.bitcast(wd.at[j].bitcast(u32)[...], bf16), preferred_element_type=f32) * sg
            cur = pltpu.bitcast(outb.at[j].bitcast(u32)[pl.ds(pl.multiple_of(t16 * 8, 8), 8), :], bf16).astype(f32)
            patch[:, j * 128:(j + 1) * 128] = (cur + jnp.where(hit, y, 0.0)).astype(bf16)

    def patch_cp(idx):
        t0 = pl.multiple_of((idx // 16) * 16, 16)
        return pltpu.make_async_copy(patch, out_hbm.at[0, pl.ds(t0, 16), :], sem_p)

    waited = set()

    def wait_x(b):
        if b < NB:
            for i in range(R0[b] // XD, (R0[b] + BLOCKS[b] - 1) // XD + 1):
                if i not in waited:
                    waited.add(i)
                    wait(x_cps[i])

    def g0():
        start(xp_cps[0]); start(wq_cps[0]); start(wq_cps[1]); start(xp_cps[1])
        start(wkv_cps[0]); start(wkv_cps[1]); start(x_cps[2]); start(wo_cps)
        for i in range(3, NXD):
            start(x_cps[i])
        zero_ref[...] = jnp.zeros((8, 128), i32)
        for j in range(NJ):
            kb0[j, 0:HALO, :] = jnp.zeros((HALO, 128), f32)
            vb0[j, 0:HALO, :] = jnp.zeros((HALO, 128), f32)
        cx = Ctx()
        wait(xp_cps[0])
        ln1(cx, 0, lc=64)
        ln1(cx, 1, lc=64, hi=XD - BLOCKS[0])
        wait(wq_cps[0])
        permute_part(0, range(0, 20))
        wait(wq_cps[1])
        permute_part(0, range(20, 40))

    def g1():
        cx = Ctx()
        wait(xp_cps[1])
        qkv_tiles(cx, 0, range(0, 5))
        emit_tiles(cx)
        lead, lastf = PER.get(1, (LEAD, LASTF))
        ln1(cx, 1, -lead, lastf * cx.t - lead, lo=XD - BLOCKS[0])

    def g2():
        cx = Ctx()
        wait(wkv_cps[0])
        qkv_tiles(cx, 1, range(0, 5))
        emit_tiles(cx)
        permute_part(1, range(40), cx, -PL, PF * cx.t - PL) if PF else permute_part(1, range(40))

    def g3():
        cx = Ctx()
        wait(wkv_cps[1])
        if LN2G3:
            wait_x(2)
        qkv_tiles(cx, 0, range(5, 10))
        emit_tiles(cx)
        permute_part(2, range(40), cx, -PL, PF * cx.t - PL) if PF else permute_part(2, range(40))
        th = cx.t
        qkv_tiles(cx, 0, range(10, 15))
        emit_tiles(cx)
        if LN2G3:
            ln1(cx, 2, th - 400, 0.9 * cx.t - 200)

    def g4():
        cx = Ctx()
        wait_x(2)
        wait(wo_cps)
        start(ffn_cps)
        wrb[...] = jnp.broadcast_to(wr_ref[...].astype(f32).reshape(1, D), (8, D))
        qkv_tiles(cx, 1, range(5, 15))
        emit_tiles(cx)
        permute_wo()
        lead, lastf = PER.get(4, (LEAD, LASTF))
        attn(cx, 0, -lead, lastf * cx.t - lead)
        if not LN2G3 and not LN2S1:
            ln1(cx, 2, -lead, lastf * cx.t - lead)

    def main_step(i, cx):
        ts = cx.t
        att = wo_tiles(cx, i - 1)
        if i == 1 and LN2S1:
            emit_tiles(cx)
            ln1(cx, 2, -100.0, cx.t - 500.0)
        qkv_tiles(cx, i + 1, range(15))
        emit_tiles(cx)
        tw = cx.tw
        lead, lastf = PER.get(4 + i, (LEAD, LASTF))
        tl = ts + lastf * (cx.t - ts) - lead
        attn(cx, i, ts - lead, tl)
        if i + 2 < NB:
            if i == 1 and LN2S1:
                ln1(cx, i + 2, tw, tl)
            else:
                ln1(cx, i + 2, ts - lead, tw - lead)
        post(cx, i - 1, att, tw, tl)

    def sep_step(i):
        cx = Ctx()
        wait_x(i + 2)
        if i > 1:
            load_best(cx)
        main_step(i, cx)
        save_best(cx)

    def fence(cx, i):
        z = pl.multiple_of(one[0] - 1, 8)
        zf = jnp.zeros((8, 128), f32)
        qb[(i + 1) % 2][0, pl.ds(z + TM, 8), :] = zf
        kb[(i + 1) % 2][0, pl.ds(z + HALO + TM, 8), :] = zf
        vb[(i + 1) % 2][0, pl.ds(z + HALO + TM, 8), :] = zf
        xn[i % 2][pl.ds(z + TM // 2, 8), 0:128] = jnp.zeros((8, 128), u32)
        ob[i % 2][pl.ds(z + TM // 2, 8), 0:128] = functools.reduce(jnp.bitwise_or, cx.done)
        cx.done = []

    def giant(lo, hi):
        cx = Ctx()
        for i in range(lo, hi):
            wait_x(i + 2)
        if lo > 1:
            load_best(cx)
        for i in range(lo, hi):
            main_step(i, cx)
            if i + 1 < hi:
                fence(cx, i)
        save_best(cx)

    L = NB - 1

    def final():
        cx = Ctx()
        wait(ffn_cps)
        for b in range(L - 2):
            wait(out_cps[b])
        bv0, bi0 = bestv[...], besti[...]
        if SPEC:
            rbest0, idx0 = argmax_of(bv0, bi0)
        att = wo_tiles(cx, L - 1)
        emit_tiles(cx)
        if SPEC:
            a = ffn_up(idx0, range(FSPLIT))
        if FG:
            attn(cx, L, -FGL, FG - FGL, rc=RCF)
        else:
            attn(cx, L, rc=RCF)
        t1 = cx.t
        att2 = wo_tiles(cx, L)
        emit_tiles(cx)
        if SPEC:
            a = a + ffn_up(idx0, range(FSPLIT, NF))
            ffn_down(a, rbest0, idx0)
        post(cx, L - 1, att, t1 + PG, t1 + PG + PSPAN, lc=min(LCF, BLOCKS[L - 1]))
        post(cx, L, att2, lc=min(LCF, BLOCKS[L]))
        bv1 = jnp.broadcast_to(cx.best[0], (8, 128))
        bi1 = jnp.broadcast_to(cx.best[1], (8, 128))

        def redo():
            take = bv1 > bv0
            rbest, idx = argmax_of(jnp.where(take, bv1, bv0), jnp.where(take, bi1, bi0))
            ffn_down(ffn_up(idx), rbest, idx)
            wait(out_cps[L - 2]); wait(out_cps[L - 1]); wait(out_cps[L])
            pc = patch_cp(idx)
            pc.start()
            pc.wait()

        if SPEC:
            miss = jnp.max(jnp.where(bv1 > rbest0, 1, 0)) > 0
            pl.when(miss)(redo)

            @pl.when(jnp.logical_not(miss))
            def _():
                wait(out_cps[L - 2])
                pc = patch_cp(idx0)
                pc.start()
                wait(out_cps[L - 1]); wait(out_cps[L])
                pc.wait()
        else:
            redo()

    if GIANT:
        cuts = list(range(1, L, GIANT)) + [L]
        if CUTS:
            cuts = CUTS
        mids = [functools.partial(giant, a, b) for a, b in zip(cuts[:-1], cuts[1:])]
    else:
        mids = [functools.partial(sep_step, i) for i in range(1, L)]
    steps = [g0, g1, g2, g3, g4] + mids + [final]
    pid = pl.program_id(0)

    def wrap(n, fn):
        def scoped():
            with jax.named_scope(f"step{n}"):
                fn()
        return fn

    if FLAT:
        @pl.when(pid == 0)
        def _():
            one[0] = 1
            wrap(0, steps[0])()

        @pl.when(pid == 1)
        def _():
            v = one[0]
            for n, fn in enumerate(steps[1:]):
                pl.when(v > -n)(wrap(n + 1, fn))
    else:
        for n, fn in enumerate(steps):
            pl.when(pid == n)(wrap(n, fn))


NSTEPS = 5 + (NB - 2) + 1
NSEM = NXD + 2 + 2 + 1 + 1 + NB + 1


@jax.jit
def pallas_sequential_preLN__sliding_local_dilated__moe_arch_mod__prompt_kernel(
    A_x, A_wqkv, A_wo, B_x, B_w_r, B_w_gate, B_w_up, B_w_down,
):
    del B_x
    any_spec = pl.BlockSpec(memory_space=pl.ANY)
    return pl.pallas_call(
        _kernel,
        grid=(2 if FLAT else NSTEPS,),
        in_specs=[any_spec] * 7,
        out_specs=any_spec,
        out_shape=jax.ShapeDtypeStruct((1, S, D), bf16),
        scratch_shapes=[
            pltpu.VMEM((NJ, S, 128), bf16),
            pltpu.VMEM((2 * XD, D), bf16),
            pltpu.VMEM((3, D, D), bf16),
            pltpu.VMEM((NJ, D, 128), bf16),
            pltpu.VMEM((D // 2, 3 * D), u32),
            pltpu.VMEM((D // 2, D), u32),
            pltpu.VMEM((NF, D, 128), bf16),
            pltpu.VMEM((NF, D, 128), bf16),
            pltpu.VMEM((NJ, F, 128), bf16),
            pltpu.VMEM((D,), bf16),
            pltpu.VMEM((8, D), f32),
            pltpu.VMEM((TM // 2 + SPARE, D), u32),
            pltpu.VMEM((TM // 2 + SPARE, D), u32),
            pltpu.VMEM((NJ, TM + SPARE, 128), f32),
            pltpu.VMEM((NJ, TM + SPARE, 128), f32),
            pltpu.VMEM((NJ, HALO + TM + SPARE, 128), f32),
            pltpu.VMEM((NJ, HALO + TM + SPARE, 128), f32),
            pltpu.VMEM((NJ, HALO + TM + SPARE, 128), f32),
            pltpu.VMEM((NJ, HALO + TM + SPARE, 128), f32),
            pltpu.VMEM((TM // 2 + SPARE, D), u32),
            pltpu.VMEM((TM // 2 + SPARE, D), u32),
            pltpu.VMEM((S // 2, D), u32),
            pltpu.VMEM((NJ, S, 128), bf16),
            pltpu.VMEM((16, D), bf16),
            pltpu.VMEM((8, 128), f32),
            pltpu.VMEM((8, 128), i32),
            pltpu.VMEM((8, 128), i32),
            pltpu.SMEM((1,), i32),
            pltpu.SemaphoreType.DMA((NSEM,)),
        ],
        compiler_params=pltpu.CompilerParams(vmem_limit_bytes=100 * 1024 * 1024,
                                             dimension_semantics=("arbitrary",),
                                             disable_semaphore_checks=bool(int(1))),
        name="preln_swa_mod",
    )(A_x, A_wqkv, A_wo, B_w_r, B_w_gate, B_w_up, B_w_down)
```

```python
import functools
import math

import jax
import jax.numpy as jnp
from jax import lax
import jax.experimental.pallas as pl
import jax.experimental.pallas.tpu as pltpu

S = 2048; D = 640; H = 32; DH = 20; W = 8; DIL = 2; F = 1536
NJ = D // 128
NF = F // 128
HALO = 16
EPS = 1e-5
LOG2E = math.log2(math.e)
QSCALE = (DH ** -0.5) * LOG2E
NEG = -1e9 * LOG2E

BLOCKS = [int(t) for t in "256,256,256,256,256,256,256,128,128".split(",")]
assert sum(BLOCKS) == S
NB = len(BLOCKS)
R0 = [sum(BLOCKS[:i]) for i in range(NB)]
TM = max(BLOCKS)
LASTF = float(0.92)
FSPLIT = int(3)
PER = {int(a.split(":")[0]): (float(a.split(":")[1]), float(a.split(":")[2]))
       for a in "5:150:0.95,6:150:0.95,7:150:0.95,8:150:0.95,9:150:0.95,10:100:0.87,11:100:0.87".split(",") if a}
LEAD = float(200)
RCF = int(16)
LCF = int(16)
SPEC = int(1)
NOH = int(0)
KSPLIT = int(1)
FLAT = int(1)
FG = float(655)
FGL = float(165)
PG = float(45)
PSPAN = float(132)
PGRP = int(4)
PF = float(0.78)
PL = float(82)
LN2G3 = int(0)
GIANT = int(0)
HOMO = int(0)
LN2S1 = int(0)
FASTRS = int(1)
CUTS = [int(c) for c in "".split(",") if c]
PTOK = int(0)
WFENCE = int(1)
LNFIRST = int(0)
_WDEF = {1: (0, 0, -229, 957, 0, 0), 4: (-238, 401, 233, 1728, -1, -1),
         5: (-178, 564, -158, 1968, -159, 650), 6: (-58, 323, -142, 2124, 173, 377), 7: (-58, 323, -142, 2124, 173, 377),
         8: (-58, 323, -142, 2124, 173, 377), 9: (-14, 490, -252, 1611, 24, 602),
         10: (-79, 762, -82, 1505, -85, 690), 11: (67, 654, -281, 1219, 157, 337)}
WIN = dict(_WDEF)
SPARE = 8
XD = 256
NXD = S // XD
assert BLOCKS[0] <= XD and BLOCKS[0] + BLOCKS[1] == 2 * XD

f32 = jnp.float32
bf16 = jnp.bfloat16
u32 = jnp.uint32
i32 = jnp.int32


def _cat(xs):
    return jnp.concatenate(xs, axis=1)


def _kernel(x_hbm, wqkv_hbm, wo_hbm, wr_hbm, wg_hbm, wu_hbm, wd_hbm, out_hbm,
            xbuf, xpre, wraw, woraw, wp, wop, wg, wu, wd, wr_ref, wrb,
            xn0, xn1, qb0, qb1, kb0, kb1, vb0, vb1, ob0, ob1, ln2b, outb, patch,
            bestv, besti, zero_ref, one, sem):
    xn = (xn0, xn1); qb = (qb0, qb1); kb = (kb0, kb1); vb = (vb0, vb1); ob = (ob0, ob1)

    nsem = [0]

    def group(pairs):
        s = sem.at[nsem[0]]
        nsem[0] += 1
        return [pltpu.make_async_copy(a, b, s) for a, b in pairs]

    def cols(j):
        return pl.ds(j * 128, 128)

    x_cps = [group([(x_hbm.at[0, pl.ds(i * XD, XD), cols(j)], xbuf.at[j, pl.ds(i * XD, XD), :])
                    for j in range(NJ)]) if i >= 2 else None for i in range(NXD)]
    HR = D // 2
    xp_cps = [group([(x_hbm.at[0, pl.ds(i * XD, XD), :], xpre.at[pl.ds(i * XD, XD), :])]) for i in range(2)]
    wq_cps = [group([(wqkv_hbm.at[pl.ds(hf * HR, HR), pl.ds(0, D)], wraw.at[0, pl.ds(hf * HR, HR), :])])
              for hf in range(2)]
    wkv_cps = [group([(wqkv_hbm.at[:, pl.ds(p * D, D)], wraw.at[p])]) for p in (1, 2)]
    wo_cps = group([(wo_hbm.at[:, cols(j)], woraw.at[j]) for j in range(NJ)] + [(wr_hbm, wr_ref)])
    ffn_cps = group([(wg_hbm.at[:, cols(n)], wg.at[n]) for n in range(NF)]
                    + [(wu_hbm.at[:, cols(n)], wu.at[n]) for n in range(NF)]
                    + [(wd_hbm.at[:, cols(j)], wd.at[j]) for j in range(NJ)])
    out_cps = [group([(outb.at[j, pl.ds(R0[b], BLOCKS[b]), :],
                       out_hbm.at[0, pl.ds(R0[b], BLOCKS[b]), cols(j)]) for j in range(NJ)])
               for b in range(NB)]
    sem_p = sem.at[nsem[0]]
    assert nsem[0] + 1 == NSEM

    def start(cs):
        for c in cs:
            c.start()

    def wait(cs):
        for c in cs:
            c.wait()

    def permute_part(p, rgs, cx=None, t0=None, t1=None):
        lane = lax.broadcasted_iota(i32, (8, 128), 1)
        lm5 = lane % 5
        base_idx = 20 * (lane % 32) + 5 * (lane // 32)
        rgs = list(rgs)
        ngrp = NJ * ((len(rgs) + PGRP - 1) // PGRP)
        gi = 0
        for j in range(NJ):
            idx = (base_idx + j) % 128
            for k, rg in enumerate(rgs):
                if k % PGRP == 0:
                    lg = lm5 if cx is None else cx.gate(spread(t0, t1, gi, ngrp), lm5)
                    masks = [lg == ((j - 3 * i) % 5) for i in range(NJ)]
                    gi += 1
                src = [pltpu.bitcast(wraw[p, rg * 16:rg * 16 + 16, i * 128:(i + 1) * 128], u32) for i in range(NJ)]
                z = src[0]
                for i in range(1, NJ):
                    z = jnp.where(masks[i], src[i], z)
                o = jnp.take_along_axis(z, idx, axis=1)
                wp[rg * 8:rg * 8 + 8, p * D + j * 128: p * D + (j + 1) * 128] = o

    def permute_wo(cx, t0, t1):
        n = NJ * (DH // 2)
        for c in range(NJ):
            src = woraw.at[c].bitcast(u32)
            for m in range(DH // 2):
                t = spread(t0, t1, c * (DH // 2) + m, n)
                mlo = cx.gate(t, jnp.full((8, 128), 0xFFFF, u32))
                sh = cx.gate(t, jnp.full((8, 128), 16, u32))
                for half in range(2):
                    a = src[pl.ds(m + 160 * half, 8, stride=20), :]
                    b = src[pl.ds(m + 10 + 160 * half, 8, stride=20), :]
                    lo = (a & mlo) | (b << sh)
                    hi = (a >> sh) | (b & ~mlo)
                    for d, val in ((2 * m, lo), (2 * m + 1, hi)):
                        j, g = d % 5, d // 5
                        r = (j * 128 + g * 32) // 2 + 8 * half
                        wop[r:r + 8, c * 128:(c + 1) * 128] = val

    class Ctx:
        def __init__(self):
            self._never = None
            self.best = None
            self.res = []
            self.pend = []
            self.done = []
            self.t = 0.0

        def add(self, val, dur):
            self.res.append((self.t, self.t + dur, val))
            self.t += dur

        def gate(self, t, val):
            if t is None or t < 0 or not self.res:
                return val
            for (t0, t1, tv) in self.res:
                if t < t1:
                    break
            frac = min(max((t - t0) / (t1 - t0), 0.0), 0.999)
            r = int(frac * (tv.shape[0] // 8)) * 8
            tok = tv[r:r + 8, :]
            if self._never is None:
                self._never = zero_ref[...] != 0
            if val.dtype != tok.dtype:
                tok = pltpu.bitcast(tok, val.dtype)
            return jnp.where(self._never, tok, val)

    def emit_tiles(cx):
        pend, cx.pend = cx.pend, []
        KA = 512
        groups = []
        for p in pend:
            if groups and len(groups[-1]) < 4 and (groups[-1][0][0].shape == p[0].shape or not HOMO):
                groups[-1].append(p)
            else:
                groups.append([p])
        for grp in groups:
            if not KSPLIT:
                for lhs, wref, n, sink in grp:
                    rhs = pltpu.bitcast(wref[:D // 2, n * 128:(n + 1) * 128], bf16)
                    t = jnp.dot(lhs, rhs, preferred_element_type=f32)
                    cx.add(t, lhs.shape[0] * NJ / 4.0)
                    sink(t)
                continue
            tb = []
            for lhs, wref, n, sink in grp:
                rhs = pltpu.bitcast(wref[KA // 2:D // 2, n * 128:(n + 1) * 128], bf16)
                if len(grp) == 4 or not HOMO:
                    tb.append(jnp.dot(lhs[:, KA:], rhs, preferred_element_type=f32))
                else:
                    mq = lhs.shape[0] // 4
                    tb.append(jnp.concatenate(
                        [jnp.dot(lhs[r:r + mq, KA:], rhs, preferred_element_type=f32)
                         for r in range(0, 4 * mq, mq)], axis=0))
            cx.add(tb[-1], sum(p[0].shape[0] for p in grp) / 4.0)
            for (lhs, wref, n, sink), b in zip(grp, tb):
                rhs = pltpu.bitcast(wref[:KA // 2, n * 128:(n + 1) * 128], bf16)
                t = jnp.dot(lhs[:, :KA], rhs, preferred_element_type=f32) + b
                cx.add(t, float(lhs.shape[0]))
                sink(t)

    def spread(t0, t1, c, n):
        return None if t0 is None else t0 + max(t1 - t0, 0.0) * c / n

    def load_x(cx, r, lc, t, pre=False):
        out = []
        for j in range(NJ):
            if pre:
                parts = [cx.gate(t, pltpu.bitcast(xpre[r + k:r + k + 16, j * 128:(j + 1) * 128], u32))
                         for k in range(0, lc, 16)]
            else:
                v = xbuf.at[j].bitcast(u32)
                parts = [cx.gate(t, v[(r + k) // 2:(r + k) // 2 + 8, :]) for k in range(0, lc, 16)]
            v = parts[0] if len(parts) == 1 else jnp.concatenate(parts, axis=0)
            out.append(pltpu.bitcast(v, bf16).astype(f32))
        return _cat(out)

    def center(x):
        m = jnp.sum(x, axis=-1, keepdims=True) * (1.0 / D)
        xc = x - m
        v = jnp.sum(xc * xc, axis=-1, keepdims=True) * (1.0 / D)
        if FASTRS:
            return xc, jnp.exp2(jnp.log(v + EPS) * (-0.5 * LOG2E)), m
        return xc, lax.rsqrt(v + EPS), m

    def ln1(cx, b, t0=None, t1=None, lc=16, lo=0, hi=None):
        hi = BLOCKS[b] if hi is None else hi
        starts = list(range(lo, hi, lc))
        for c, a0 in enumerate(starts):
            n = min(lc, hi - a0)
            xc, rs, _ = center(load_x(cx, R0[b] + a0, n, spread(t0, t1, c, len(starts)), pre=b < 2))
            y = xc * rs
            xn[b % 2][a0 // 2:(a0 + n) // 2, :] = pltpu.bitcast(y.astype(bf16), u32)
            cx.done.append(pltpu.bitcast(y[0:8, 512:640], u32))

    def qkv_tiles(cx, b, tiles):
        m = BLOCKS[b]
        lhs = pltpu.bitcast(xn[b % 2][0:m // 2, :], bf16)

        def sink(n, t):
            p, j = divmod(n, NJ)
            if p == 0:
                qb[b % 2][j, 0:m, :] = t
            else:
                dst = (kb, vb)[p - 1]
                if b > 0:
                    mp = BLOCKS[b - 1]
                    dst[b % 2][j, 0:HALO, :] = dst[(b - 1) % 2][j, mp:mp + HALO, :]
                dst[b % 2][j, HALO:HALO + m, :] = t
        for n in tiles:
            cx.pend.append((lhs, wp, n, functools.partial(sink, n)))

    def attn(cx, b, t0=None, t1=None, rc=8):
        qr, kr, vr = qb[b % 2], kb[b % 2], vb[b % 2]
        n = BLOCKS[b] // rc
        for c in range(n):
            a0 = c * rc
            sc = cx.gate(spread(t0, t1, c, n), jnp.full((8, 128), QSCALE, f32))
            if rc > 8:
                sc = jnp.tile(sc, (rc // 8, 1))
            q = [qr[j, a0:a0 + rc, :] * sc for j in range(NJ)]
            tt = []
            for w in range(W):
                k0 = HALO + a0 - DIL * w
                acc = q[0] * kr[0, k0:k0 + rc, :]
                for j in range(1, NJ):
                    acc = acc + q[j] * kr[j, k0:k0 + rc, :]
                tt.append(acc)
            r1 = [pltpu.roll(tt[w], 64, 1) for w in range(W)]
            tt = [tt[w] + r1[w] for w in range(W)]
            r2 = [pltpu.roll(tt[w], 32, 1) for w in range(W)]
            s = [tt[w] + r2[w] for w in range(W)]
            for w in range(W):
                if b == 0 and a0 - DIL * w < 0:
                    row = lax.broadcasted_iota(i32, (rc, 128), 0) + (a0 - DIL * w)
                    s[w] = jnp.where(row >= 0, s[w], NEG)
            mx = functools.reduce(jnp.maximum, s)
            p = [jnp.exp2(s[w] - mx) for w in range(W)]
            l = functools.reduce(lambda a, b: a + b, p)
            inv = pl.reciprocal(l, approx=True)
            o = []
            for j in range(NJ):
                acc = None
                for w in range(W):
                    k0 = HALO + a0 - DIL * w
                    term = p[w] * vr[j, k0:k0 + rc, :]
                    acc = term if acc is None else acc + term
                o.append(acc * inv)
            if rc == 8 and c % 2 == 0:
                prev = o
                continue
            if rc == 8:
                o = [jnp.concatenate([prev[j], o[j]], axis=0) for j in range(NJ)]
                a0 -= 8
            rows = o[0].shape[0]
            for j in range(NJ):
                ob[b % 2][a0 // 2:(a0 + rows) // 2, j * 128:(j + 1) * 128] = pltpu.bitcast(o[j].astype(bf16), u32)

    def wo_tiles(cx, b):
        m = BLOCKS[b]
        lhs = pltpu.bitcast(ob[b % 2][0:m // 2, :], bf16)
        att = []

        def sink(t):
            att.append(t)
            cx.tw = cx.t
        for n in range(NJ):
            cx.pend.append((lhs, wop, n, sink))
        return att

    def post(cx, b, att, t0=None, t1=None, lc=16):
        r0 = R0[b]
        n = BLOCKS[b] // lc
        for c in range(n):
            a0 = c * lc
            h = load_x(cx, r0 + a0, lc, spread(t0, t1, c, n), pre=b < 2) + _cat([att[j][a0:a0 + lc, :] for j in range(NJ)])
            xc, rs, mean = center(h)
            r = jnp.sum(xc * jnp.tile(wrb[...], (lc // 8, 1)), axis=-1, keepdims=True) * rs
            ln2 = xc * rs
            ln2b[(r0 + a0) // 2:(r0 + a0 + lc) // 2, :] = pltpu.bitcast(ln2.astype(bf16), u32)
            o = pltpu.bitcast(((xc * (rs + 1.0) + mean) if NOH else (h + ln2)).astype(bf16), u32)
            for j in range(NJ):
                outb.at[j].bitcast(u32)[(r0 + a0) // 2:(r0 + a0 + lc) // 2, :] = o[:, j * 128:(j + 1) * 128]
            if PTOK:
                cx.done.append(pltpu.bitcast(ln2[0:8, 512:640], u32))
            for k in range(0, lc, 8):
                rk = r[k:k + 8, :]
                if cx.best is None:
                    cx.best = (rk, jnp.full((8, 1), r0 + a0 + k, i32))
                else:
                    bv, bi = cx.best
                    take = rk > bv
                    cx.best = (jnp.where(take, rk, bv), jnp.where(take, r0 + a0 + k, bi))
        cx.done.append(pltpu.bitcast(jnp.broadcast_to(cx.best[0], (8, 128)), u32))
        start(out_cps[b])

    def load_best(cx):
        cx.best = (bestv[:, 0:1], besti[:, 0:1])

    def save_best(cx):
        bestv[...] = jnp.broadcast_to(cx.best[0], (8, 128))
        besti[...] = jnp.broadcast_to(cx.best[1], (8, 128))

    def argmax_of(bv, bi):
        rowid = bi + lax.broadcasted_iota(i32, (8, 128), 0)
        rbest = jnp.max(bv, axis=0, keepdims=True)
        idx = jnp.clip(jnp.min(jnp.where(bv == rbest, rowid, S)), 0, S - 1)
        return rbest, idx

    def ffn_up(idx, tiles=range(NF)):
        t16 = idx // 16
        xs = pltpu.bitcast(ln2b[pl.ds(pl.multiple_of(t16 * 8, 8), 8), :], bf16)
        a = []
        for n in tiles:
            g = jnp.dot(xs, pltpu.bitcast(wg.at[n].bitcast(u32)[...], bf16), preferred_element_type=f32)
            u = jnp.dot(xs, pltpu.bitcast(wu.at[n].bitcast(u32)[...], bf16), preferred_element_type=f32)
            a.append((g * jax.nn.sigmoid(g) * u).astype(bf16))
        return a

    def ffn_down(a, rbest, idx):
        a = _cat(a)
        sg = jax.nn.sigmoid(rbest)
        t16 = idx // 16
        hit = (lax.broadcasted_iota(i32, (16, 128), 0) + t16 * 16) == idx
        for j in range(NJ):
            y = jnp.dot(a, pltpu.bitcast(wd.at[j].bitcast(u32)[...], bf16), preferred_element_type=f32) * sg
            cur = pltpu.bitcast(outb.at[j].bitcast(u32)[pl.ds(pl.multiple_of(t16 * 8, 8), 8), :], bf16).astype(f32)
            patch[:, j * 128:(j + 1) * 128] = (cur + jnp.where(hit, y, 0.0)).astype(bf16)

    def patch_cp(idx):
        t0 = pl.multiple_of((idx // 16) * 16, 16)
        return pltpu.make_async_copy(patch, out_hbm.at[0, pl.ds(t0, 16), :], sem_p)

    waited = set()

    def wait_x(b):
        if b < NB:
            for i in range(R0[b] // XD, (R0[b] + BLOCKS[b] - 1) // XD + 1):
                if i not in waited:
                    waited.add(i)
                    wait(x_cps[i])

    def g0():
        start(xp_cps[0]); start(wq_cps[0]); start(wq_cps[1]); start(xp_cps[1])
        start(wkv_cps[0]); start(wkv_cps[1]); start(x_cps[2]); start(wo_cps)
        for i in range(3, NXD):
            start(x_cps[i])
        zero_ref[...] = jnp.zeros((8, 128), i32)
        for j in range(NJ):
            kb0[j, 0:HALO, :] = jnp.zeros((HALO, 128), f32)
            vb0[j, 0:HALO, :] = jnp.zeros((HALO, 128), f32)
        cx = Ctx()
        wait(xp_cps[0])
        ln1(cx, 0, lc=64)
        ln1(cx, 1, lc=64, hi=XD - BLOCKS[0])
        wait(wq_cps[0])
        permute_part(0, range(0, 20))
        wait(wq_cps[1])
        permute_part(0, range(20, 40))

    def g1():
        cx = Ctx()
        wait(xp_cps[1])
        qkv_tiles(cx, 0, range(0, 5))
        emit_tiles(cx)
        ln1(cx, 1, WIN[1][2], WIN[1][3], lo=XD - BLOCKS[0])

    def g2():
        cx = Ctx()
        wait(wkv_cps[0])
        qkv_tiles(cx, 1, range(0, 5))
        emit_tiles(cx)
        permute_part(1, range(40), cx, -PL, PF * cx.t - PL) if PF else permute_part(1, range(40))

    def g3():
        cx = Ctx()
        wait(wkv_cps[1])
        if LN2G3:
            wait_x(2)
        qkv_tiles(cx, 0, range(5, 10))
        emit_tiles(cx)
        permute_part(2, range(40), cx, -PL, PF * cx.t - PL) if PF else permute_part(2, range(40))
        th = cx.t
        qkv_tiles(cx, 0, range(10, 15))
        emit_tiles(cx)
        if LN2G3:
            ln1(cx, 2, th - 400, 0.9 * cx.t - 200)

    def g4():
        cx = Ctx()
        wait_x(2)
        wait(wo_cps)
        start(ffn_cps)
        wrb[...] = jnp.broadcast_to(wr_ref[...].astype(f32).reshape(1, D), (8, D))
        qkv_tiles(cx, 1, range(5, 15))
        emit_tiles(cx)
        permute_wo(cx, WIN[4][4], WIN[4][5])
        a0, a1, l0, l1, p0, p1 = WIN[4]
        attn(cx, 0, a0, cx.t - a1)
        ln1(cx, 2, l0, l1)

    def main_step(i, cx):
        ts = cx.t
        att = wo_tiles(cx, i - 1)
        if i == 1 and LN2S1:
            emit_tiles(cx)
            ln1(cx, 2, -100.0, cx.t - 500.0)
        qkv_tiles(cx, i + 1, range(15))
        emit_tiles(cx)
        tw = cx.tw
        a0, a1, l0, l1, p0, p1 = WIN[4 + i]
        attn(cx, i, ts + a0, cx.t - a1)
        if i + 2 < NB:
            ln1(cx, i + 2, ts + l0, ts + l1)
        post(cx, i - 1, att, tw + p0, cx.t - p1)

    def sep_step(i):
        cx = Ctx()
        wait_x(i + 2)
        if i > 1:
            load_best(cx)
        main_step(i, cx)
        save_best(cx)

    def fence(cx, i):
        z = pl.multiple_of(one[0] - 1, 8)
        zf = jnp.zeros((8, 128), f32)
        qb[(i + 1) % 2][0, pl.ds(z + TM, 8), :] = zf
        kb[(i + 1) % 2][0, pl.ds(z + HALO + TM, 8), :] = zf
        vb[(i + 1) % 2][0, pl.ds(z + HALO + TM, 8), :] = zf
        xn[i % 2][pl.ds(z + TM // 2, 8), 0:128] = jnp.zeros((8, 128), u32)
        ob[i % 2][pl.ds(z + TM // 2, 8), 0:128] = functools.reduce(jnp.bitwise_or, cx.done)
        if WFENCE:
            wp[pl.ds(z + D // 2, 8), 0:128] = jnp.zeros((8, 128), u32)
            wop[pl.ds(z + D // 2, 8), 0:128] = jnp.zeros((8, 128), u32)
        cx.done = []

    def giant(lo, hi):
        cx = Ctx()
        for i in range(lo, hi):
            wait_x(i + 2)
        if lo > 1:
            load_best(cx)
        for i in range(lo, hi):
            main_step(i, cx)
            if i + 1 < hi:
                fence(cx, i)
        save_best(cx)

    L = NB - 1

    def final():
        cx = Ctx()
        wait(ffn_cps)
        for b in range(L - 2):
            wait(out_cps[b])
        bv0, bi0 = bestv[...], besti[...]
        if SPEC:
            rbest0, idx0 = argmax_of(bv0, bi0)
        att = wo_tiles(cx, L - 1)
        emit_tiles(cx)
        if SPEC:
            a = ffn_up(idx0, range(FSPLIT))
        if FG:
            attn(cx, L, -FGL, FG - FGL, rc=RCF)
        else:
            attn(cx, L, rc=RCF)
        t1 = cx.t
        att2 = wo_tiles(cx, L)
        emit_tiles(cx)
        if SPEC:
            a = a + ffn_up(idx0, range(FSPLIT, NF))
            ffn_down(a, rbest0, idx0)
        post(cx, L - 1, att, t1 + PG, t1 + PG + PSPAN, lc=min(LCF, BLOCKS[L - 1]))
        post(cx, L, att2, lc=min(LCF, BLOCKS[L]))
        bv1 = jnp.broadcast_to(cx.best[0], (8, 128))
        bi1 = jnp.broadcast_to(cx.best[1], (8, 128))

        def redo():
            take = bv1 > bv0
            rbest, idx = argmax_of(jnp.where(take, bv1, bv0), jnp.where(take, bi1, bi0))
            ffn_down(ffn_up(idx), rbest, idx)
            wait(out_cps[L - 2]); wait(out_cps[L - 1]); wait(out_cps[L])
            pc = patch_cp(idx)
            pc.start()
            pc.wait()

        if SPEC:
            miss = jnp.max(jnp.where(bv1 > rbest0, 1, 0)) > 0
            pl.when(miss)(redo)

            @pl.when(jnp.logical_not(miss))
            def _():
                wait(out_cps[L - 2])
                pc = patch_cp(idx0)
                pc.start()
                wait(out_cps[L - 1]); wait(out_cps[L])
                pc.wait()
        else:
            redo()

    if GIANT:
        cuts = list(range(1, L, GIANT)) + [L]
        if CUTS:
            cuts = CUTS
        mids = [functools.partial(giant, a, b) for a, b in zip(cuts[:-1], cuts[1:])]
    else:
        mids = [functools.partial(sep_step, i) for i in range(1, L)]
    steps = [g0, g1, g2, g3, g4] + mids + [final]
    pid = pl.program_id(0)

    def wrap(n, fn):
        def scoped():
            with jax.named_scope(f"step{n}"):
                fn()
        return fn

    if FLAT:
        @pl.when(pid == 0)
        def _():
            one[0] = 1
            wrap(0, steps[0])()

        @pl.when(pid == 1)
        def _():
            v = one[0]
            for n, fn in enumerate(steps[1:]):
                pl.when(v > -n)(wrap(n + 1, fn))
    else:
        for n, fn in enumerate(steps):
            pl.when(pid == n)(wrap(n, fn))


NSTEPS = 5 + (NB - 2) + 1
NSEM = NXD + 2 + 2 + 1 + 1 + NB + 1


@jax.jit
def pallas_sequential_preLN__sliding_local_dilated__moe_arch_mod__prompt_kernel(
    A_x, A_wqkv, A_wo, B_x, B_w_r, B_w_gate, B_w_up, B_w_down,
):
    del B_x
    any_spec = pl.BlockSpec(memory_space=pl.ANY)
    return pl.pallas_call(
        _kernel,
        grid=(2 if FLAT else NSTEPS,),
        in_specs=[any_spec] * 7,
        out_specs=any_spec,
        out_shape=jax.ShapeDtypeStruct((1, S, D), bf16),
        scratch_shapes=[
            pltpu.VMEM((NJ, S, 128), bf16),
            pltpu.VMEM((2 * XD, D), bf16),
            pltpu.VMEM((3, D, D), bf16),
            pltpu.VMEM((NJ, D, 128), bf16),
            pltpu.VMEM((D // 2 + SPARE, 3 * D), u32),
            pltpu.VMEM((D // 2 + SPARE, D), u32),
            pltpu.VMEM((NF, D, 128), bf16),
            pltpu.VMEM((NF, D, 128), bf16),
            pltpu.VMEM((NJ, F, 128), bf16),
            pltpu.VMEM((D,), bf16),
            pltpu.VMEM((8, D), f32),
            pltpu.VMEM((TM // 2 + SPARE, D), u32),
            pltpu.VMEM((TM // 2 + SPARE, D), u32),
            pltpu.VMEM((NJ, TM + SPARE, 128), f32),
            pltpu.VMEM((NJ, TM + SPARE, 128), f32),
            pltpu.VMEM((NJ, HALO + TM + SPARE, 128), f32),
            pltpu.VMEM((NJ, HALO + TM + SPARE, 128), f32),
            pltpu.VMEM((NJ, HALO + TM + SPARE, 128), f32),
            pltpu.VMEM((NJ, HALO + TM + SPARE, 128), f32),
            pltpu.VMEM((TM // 2 + SPARE, D), u32),
            pltpu.VMEM((TM // 2 + SPARE, D), u32),
            pltpu.VMEM((S // 2, D), u32),
            pltpu.VMEM((NJ, S, 128), bf16),
            pltpu.VMEM((16, D), bf16),
            pltpu.VMEM((8, 128), f32),
            pltpu.VMEM((8, 128), i32),
            pltpu.VMEM((8, 128), i32),
            pltpu.SMEM((1,), i32),
            pltpu.SemaphoreType.DMA((NSEM,)),
        ],
        compiler_params=pltpu.CompilerParams(vmem_limit_bytes=100 * 1024 * 1024,
                                             dimension_semantics=("arbitrary",),
                                             disable_semaphore_checks=bool(int(1))),
        name="preln_swa_mod",
    )(A_x, A_wqkv, A_wo, B_w_r, B_w_gate, B_w_up, B_w_down)
```

```python
import functools
import math

import jax
import jax.numpy as jnp
from jax import lax
import jax.experimental.pallas as pl
import jax.experimental.pallas.tpu as pltpu

S = 2048; D = 640; H = 32; DH = 20; W = 8; DIL = 2; F = 1536
NJ = D // 128
NF = F // 128
HALO = 16
EPS = 1e-5
LOG2E = math.log2(math.e)
QSCALE = (DH ** -0.5) * LOG2E
NEG = -1e9 * LOG2E

BLOCKS = [int(t) for t in "256,256,256,256,256,256,256,128,128".split(",")]
assert sum(BLOCKS) == S
NB = len(BLOCKS)
R0 = [sum(BLOCKS[:i]) for i in range(NB)]
TM = max(BLOCKS)
LASTF = float(0.92)
FSPLIT = int(4)
PER = {int(a.split(":")[0]): (float(a.split(":")[1]), float(a.split(":")[2]))
       for a in "5:150:0.95,6:150:0.95,7:150:0.95,8:150:0.95,9:150:0.95,10:100:0.87,11:100:0.87".split(",") if a}
LEAD = float(200)
RCF = int(8)
LCF = int(16)
SPEC = int(1)
NOH = int(0)
KSPLIT = int(1)
FLAT = int(1)
FG = float(451)
FGL = float(337)
PG = float(215)
PSPAN = float(293)
PGRP = int(4)
PF = float(0.28)
PL = float(398)
LN2G3 = int(0)
GIANT = int(0)
HOMO = int(0)
LN2S1 = int(0)
FASTRS = int(1)
CUTS = [int(c) for c in "".split(",") if c]
PTOK = int(0)
WFENCE = int(1)
LNFIRST = int(0)
_WDEF = {1: (0, 0, -229, 957, 0, 0), 4: (683, 480, 566, 2734, -298, 818),
         5: (-273, 374, 356, 2648, 202, 319), 6: (-58, 323, -142, 2124, 173, 377), 7: (-58, 323, -142, 2124, 173, 377),
         8: (-58, 323, -142, 2124, 173, 377), 9: (-83, 510, -216, 1258, -42, 637),
         10: (-79, 762, -82, 1505, -85, 690), 11: (116, 753, -228, 1249, 133, 368)}
WIN = dict(_WDEF)
RAWG = [tuple(int(t) for t in a.split("-")) for a in "0-2,2-4,4-6,6-9,9-11,11-13,13-15".split(",")]
X1POS = int(5)
TASKS = {}
for _s in "2:w0:012;3:w0:34,o0:01234;4:w1:0123;5:o1:012;6:o1:34,w1:4,w2:012;7:o2:01234,w2:34".split(";"):
    _g, _r = _s.split(":", 1)
    TASKS[int(_g)] = [(t[0], int(t[1]), [int(c) for c in t.split(":")[1]]) for t in _r.split(",")]
assert all(sorted(j for ts in TASKS.values() for k, p, js in ts if (k, p) == kp for j in js) == list(range(5))
           for kp in [(k, p) for k in "wo" for p in range(3)])
PW0 = float(-137)
PW1 = float(680)
LC1 = int(32)
SPARE = 8
XD = 256
NXD = S // XD
assert BLOCKS[0] == XD and BLOCKS[1] == XD

f32 = jnp.float32
bf16 = jnp.bfloat16
u32 = jnp.uint32
i32 = jnp.int32


def _cat(xs):
    return jnp.concatenate(xs, axis=1)


def _kernel(x_hbm, wqkv_hbm, wo_hbm, wr_hbm, wg_hbm, wu_hbm, wd_hbm, out_hbm,
            xbuf, xpre, wraw, rawb, woraw, wp, wop, wg, wu, wd, wr_ref, wrb,
            xn0, xn1, qb0, qb1, kb0, kb1, vb0, vb1, ob0, ob1, ln2b, outb, patch,
            bestv, besti, zero_ref, one, sem):
    xn = (xn0, xn1); qb = (qb0, qb1); kb = (kb0, kb1); vb = (vb0, vb1); ob = (ob0, ob1)

    nsem = [0]

    def group(pairs):
        s = sem.at[nsem[0]]
        nsem[0] += 1
        return [pltpu.make_async_copy(a, b, s) for a, b in pairs]

    def cols(j):
        return pl.ds(j * 128, 128)

    x_cps = [group([(x_hbm.at[0, pl.ds(i * XD, XD), cols(j)], xbuf.at[j, pl.ds(i * XD, XD), :])
                    for j in range(NJ)]) if i >= 2 else None for i in range(NXD)]
    xp_cps = [group([(x_hbm.at[0, pl.ds(i * XD, XD), :], xpre.at[pl.ds(i * XD, XD), :])]) for i in range(2)]
    wg_cps = [group([(wqkv_hbm.at[:, pl.ds(a * 128, (b - a) * 128)], wraw.at[:, pl.ds(a * 128, (b - a) * 128)])])
              for a, b in RAWG]
    wo_cps = group([(wo_hbm.at[:, cols(j)], woraw.at[j]) for j in range(NJ)] + [(wr_hbm, wr_ref)])
    ffn_cps = group([(wg_hbm.at[:, cols(n)], wg.at[n]) for n in range(NF)]
                    + [(wu_hbm.at[:, cols(n)], wu.at[n]) for n in range(NF)]
                    + [(wd_hbm.at[:, cols(j)], wd.at[j]) for j in range(NJ)])
    out_cps = [group([(outb.at[j, pl.ds(R0[b], BLOCKS[b]), :],
                       out_hbm.at[0, pl.ds(R0[b], BLOCKS[b]), cols(j)]) for j in range(NJ)])
               for b in range(NB)]
    sem_p = sem.at[nsem[0]]
    assert nsem[0] + 1 == NSEM

    def start(cs):
        for c in cs:
            c.start()

    def wait(cs):
        for c in cs:
            c.wait()

    def lane_perm(load, store, nrg, cx, t0, t1, js):
        lane = lax.broadcasted_iota(i32, (8, 128), 1)
        lm5 = lane % 5
        base_idx = 20 * (lane % 32) + 5 * (lane // 32)
        ngrp = len(js) * ((nrg + PGRP - 1) // PGRP)
        gi = 0
        for j in js:
            idx = (base_idx + j) % 128
            for rg in range(nrg):
                if rg % PGRP == 0:
                    lg = cx.gate(spread(t0, t1, gi, ngrp), lm5)
                    masks = [lg == ((j - 3 * i) % 5) for i in range(NJ)]
                    gi += 1
                src = [load(i, rg) for i in range(NJ)]
                z = src[0]
                for i in range(1, NJ):
                    z = jnp.where(masks[i], src[i], z)
                store(j, rg, jnp.take_along_axis(z, idx, axis=1))

    def perm_w(cx, p, t0, t1, js):
        def load(i, rg):
            return pltpu.bitcast(wraw[rg * 16:rg * 16 + 16, (p * NJ + i) * 128:(p * NJ + i + 1) * 128], u32)

        def store(j, rg, z):
            wp[rg * 8:rg * 8 + 8, p * D + j * 128: p * D + (j + 1) * 128] = z
        lane_perm(load, store, D // 16, cx, t0, t1, js)

    def perm_out(cx, p, t0, t1, js):
        def load(i, rg):
            return rawb[p * NJ + i, rg * 8:rg * 8 + 8, :]

        def store(j, rg, z):
            if p == 0:
                qb[0][j, rg * 8:rg * 8 + 8, :] = z
            else:
                (kb, vb)[p - 1][0][j, HALO + rg * 8:HALO + rg * 8 + 8, :] = z
        lane_perm(load, store, XD // 8, cx, t0, t1, js)

    def permute_wo(cx, t0, t1):
        n = NJ * (DH // 2)
        for c in range(NJ):
            src = woraw.at[c].bitcast(u32)
            for m in range(DH // 2):
                t = spread(t0, t1, c * (DH // 2) + m, n)
                mlo = cx.gate(t, jnp.full((8, 128), 0xFFFF, u32))
                sh = cx.gate(t, jnp.full((8, 128), 16, u32))
                for half in range(2):
                    a = src[pl.ds(m + 160 * half, 8, stride=20), :]
                    b = src[pl.ds(m + 10 + 160 * half, 8, stride=20), :]
                    lo = (a & mlo) | (b << sh)
                    hi = (a >> sh) | (b & ~mlo)
                    for d, val in ((2 * m, lo), (2 * m + 1, hi)):
                        j, g = d % 5, d // 5
                        r = (j * 128 + g * 32) // 2 + 8 * half
                        wop[r:r + 8, c * 128:(c + 1) * 128] = val

    class Ctx:
        def __init__(self):
            self._never = None
            self.best = None
            self.res = []
            self.pend = []
            self.done = []
            self.t = 0.0

        def add(self, val, dur):
            self.res.append((self.t, self.t + dur, val))
            self.t += dur

        def gate(self, t, val):
            if t is None or t < 0 or not self.res:
                return val
            for (t0, t1, tv) in self.res:
                if t < t1:
                    break
            frac = min(max((t - t0) / (t1 - t0), 0.0), 0.999)
            r = int(frac * (tv.shape[0] // 8)) * 8
            tok = tv[r:r + 8, :]
            if self._never is None:
                self._never = zero_ref[...] != 0
            if val.dtype != tok.dtype:
                tok = pltpu.bitcast(tok, val.dtype)
            return jnp.where(self._never, tok, val)

    def emit_tiles(cx, balance=False):
        pend, cx.pend = cx.pend, []
        KA = 512
        for g in range(0, len(pend), 4):
            grp = pend[g:g + 4]
            nsp = 4 // math.gcd(len(grp), 4) if balance else 1
            tb = []
            for lhs, rhs_fn, sink in grp:
                rhs = rhs_fn(KA, D)
                mq = lhs.shape[0] // nsp
                parts = [jnp.dot(lhs[r:r + mq, KA:], rhs, preferred_element_type=f32)
                         for r in range(0, lhs.shape[0], mq)]
                tb.append(parts[0] if nsp == 1 else jnp.concatenate(parts, axis=0))
            cx.add(tb[-1], sum(p[0].shape[0] for p in grp) / 4.0)
            for (lhs, rhs_fn, sink), b in zip(grp, tb):
                t = jnp.dot(lhs[:, :KA], rhs_fn(0, KA), preferred_element_type=f32) + b
                cx.add(t, float(lhs.shape[0]))
                sink(t)

    def packed_rhs(wref, n, k0, k1):
        return pltpu.bitcast(wref[k0 // 2:k1 // 2, n * 128:(n + 1) * 128], bf16)

    def raw_tiles(cx, tiles):
        lhs = pltpu.bitcast(xn[0][0:XD // 2, :], bf16)

        def sink(n, t):
            rawb[n] = t
        for n in tiles:
            cx.pend.append((lhs, lambda k0, k1, n=n: wraw[k0:k1, n * 128:(n + 1) * 128],
                            functools.partial(sink, n)))
        emit_tiles(cx, balance=True)

    def spread(t0, t1, c, n):
        return None if t0 is None else t0 + max(t1 - t0, 0.0) * c / n

    def load_x(cx, r, lc, t, pre=False):
        out = []
        for j in range(NJ):
            if pre:
                parts = [cx.gate(t, pltpu.bitcast(xpre[r + k:r + k + 16, j * 128:(j + 1) * 128], u32))
                         for k in range(0, lc, 16)]
            else:
                v = xbuf.at[j].bitcast(u32)
                parts = [cx.gate(t, v[(r + k) // 2:(r + k) // 2 + 8, :]) for k in range(0, lc, 16)]
            v = parts[0] if len(parts) == 1 else jnp.concatenate(parts, axis=0)
            out.append(pltpu.bitcast(v, bf16).astype(f32))
        return _cat(out)

    def center(x):
        m = jnp.sum(x, axis=-1, keepdims=True) * (1.0 / D)
        xc = x - m
        v = jnp.sum(xc * xc, axis=-1, keepdims=True) * (1.0 / D)
        if FASTRS:
            return xc, jnp.exp2(jnp.log(v + EPS) * (-0.5 * LOG2E)), m
        return xc, lax.rsqrt(v + EPS), m

    def ln1(cx, b, t0=None, t1=None, lc=16, lo=0, hi=None):
        hi = BLOCKS[b] if hi is None else hi
        starts = list(range(lo, hi, lc))
        for c, a0 in enumerate(starts):
            n = min(lc, hi - a0)
            xc, rs, _ = center(load_x(cx, R0[b] + a0, n, spread(t0, t1, c, len(starts)), pre=b < 2))
            y = xc * rs
            xn[b % 2][a0 // 2:(a0 + n) // 2, :] = pltpu.bitcast(y.astype(bf16), u32)
            cx.done.append(pltpu.bitcast(y[0:8, 512:640], u32))

    def qkv_tiles(cx, b, tiles):
        m = BLOCKS[b]
        lhs = pltpu.bitcast(xn[b % 2][0:m // 2, :], bf16)

        def sink(n, t):
            p, j = divmod(n, NJ)
            if p == 0:
                qb[b % 2][j, 0:m, :] = t
            else:
                dst = (kb, vb)[p - 1]
                if b > 0:
                    mp = BLOCKS[b - 1]
                    dst[b % 2][j, 0:HALO, :] = dst[(b - 1) % 2][j, mp:mp + HALO, :]
                dst[b % 2][j, HALO:HALO + m, :] = t
        for n in tiles:
            cx.pend.append((lhs, functools.partial(packed_rhs, wp, n), functools.partial(sink, n)))

    def attn(cx, b, t0=None, t1=None, rc=8):
        qr, kr, vr = qb[b % 2], kb[b % 2], vb[b % 2]
        n = BLOCKS[b] // rc
        for c in range(n):
            a0 = c * rc
            sc = cx.gate(spread(t0, t1, c, n), jnp.full((8, 128), QSCALE, f32))
            if rc > 8:
                sc = jnp.tile(sc, (rc // 8, 1))
            q = [qr[j, a0:a0 + rc, :] * sc for j in range(NJ)]
            tt = []
            for w in range(W):
                k0 = HALO + a0 - DIL * w
                acc = q[0] * kr[0, k0:k0 + rc, :]
                for j in range(1, NJ):
                    acc = acc + q[j] * kr[j, k0:k0 + rc, :]
                tt.append(acc)
            r1 = [pltpu.roll(tt[w], 64, 1) for w in range(W)]
            tt = [tt[w] + r1[w] for w in range(W)]
            r2 = [pltpu.roll(tt[w], 32, 1) for w in range(W)]
            s = [tt[w] + r2[w] for w in range(W)]
            for w in range(W):
                if b == 0 and a0 - DIL * w < 0:
                    row = lax.broadcasted_iota(i32, (rc, 128), 0) + (a0 - DIL * w)
                    s[w] = jnp.where(row >= 0, s[w], NEG)
            mx = functools.reduce(jnp.maximum, s)
            p = [jnp.exp2(s[w] - mx) for w in range(W)]
            l = functools.reduce(lambda a, b: a + b, p)
            inv = pl.reciprocal(l, approx=True)
            o = []
            for j in range(NJ):
                acc = None
                for w in range(W):
                    k0 = HALO + a0 - DIL * w
                    term = p[w] * vr[j, k0:k0 + rc, :]
                    acc = term if acc is None else acc + term
                o.append(acc * inv)
            if rc == 8 and c % 2 == 0:
                prev = o
                continue
            if rc == 8:
                o = [jnp.concatenate([prev[j], o[j]], axis=0) for j in range(NJ)]
                a0 -= 8
            rows = o[0].shape[0]
            for j in range(NJ):
                ob[b % 2][a0 // 2:(a0 + rows) // 2, j * 128:(j + 1) * 128] = pltpu.bitcast(o[j].astype(bf16), u32)

    def wo_tiles(cx, b):
        m = BLOCKS[b]
        lhs = pltpu.bitcast(ob[b % 2][0:m // 2, :], bf16)
        att = []

        def sink(t):
            att.append(t)
            cx.tw = cx.t
        for n in range(NJ):
            cx.pend.append((lhs, functools.partial(packed_rhs, wop, n), sink))
        return att

    def post(cx, b, att, t0=None, t1=None, lc=16):
        r0 = R0[b]
        n = BLOCKS[b] // lc
        for c in range(n):
            a0 = c * lc
            h = load_x(cx, r0 + a0, lc, spread(t0, t1, c, n), pre=b < 2) + _cat([att[j][a0:a0 + lc, :] for j in range(NJ)])
            xc, rs, mean = center(h)
            r = jnp.sum(xc * jnp.tile(wrb[...], (lc // 8, 1)), axis=-1, keepdims=True) * rs
            ln2 = xc * rs
            ln2b[(r0 + a0) // 2:(r0 + a0 + lc) // 2, :] = pltpu.bitcast(ln2.astype(bf16), u32)
            o = pltpu.bitcast(((xc * (rs + 1.0) + mean) if NOH else (h + ln2)).astype(bf16), u32)
            for j in range(NJ):
                outb.at[j].bitcast(u32)[(r0 + a0) // 2:(r0 + a0 + lc) // 2, :] = o[:, j * 128:(j + 1) * 128]
            if PTOK:
                cx.done.append(pltpu.bitcast(ln2[0:8, 512:640], u32))
            for k in range(0, lc, 8):
                rk = r[k:k + 8, :]
                if cx.best is None:
                    cx.best = (rk, jnp.full((8, 1), r0 + a0 + k, i32))
                else:
                    bv, bi = cx.best
                    take = rk > bv
                    cx.best = (jnp.where(take, rk, bv), jnp.where(take, r0 + a0 + k, bi))
        cx.done.append(pltpu.bitcast(jnp.broadcast_to(cx.best[0], (8, 128)), u32))
        start(out_cps[b])

    def load_best(cx):
        cx.best = (bestv[:, 0:1], besti[:, 0:1])

    def save_best(cx):
        bestv[...] = jnp.broadcast_to(cx.best[0], (8, 128))
        besti[...] = jnp.broadcast_to(cx.best[1], (8, 128))

    def argmax_of(bv, bi, nrows=S):
        rowid = bi + lax.broadcasted_iota(i32, (8, 128), 0)
        rbest = jnp.max(bv, axis=0, keepdims=True)
        idx = jnp.clip(jnp.min(jnp.where(bv == rbest, rowid, S)), 0, nrows - 1)
        return rbest, idx

    def ffn_up(idx, tiles=range(NF)):
        t16 = idx // 16
        xs = pltpu.bitcast(ln2b[pl.ds(pl.multiple_of(t16 * 8, 8), 8), :], bf16)
        a = []
        for n in tiles:
            g = jnp.dot(xs, pltpu.bitcast(wg.at[n].bitcast(u32)[...], bf16), preferred_element_type=f32)
            u = jnp.dot(xs, pltpu.bitcast(wu.at[n].bitcast(u32)[...], bf16), preferred_element_type=f32)
            a.append((g * jax.nn.sigmoid(g) * u).astype(bf16))
        return a

    def ffn_down(a, rbest, idx):
        a = _cat(a)
        sg = jax.nn.sigmoid(rbest)
        t16 = idx // 16
        hit = (lax.broadcasted_iota(i32, (16, 128), 0) + t16 * 16) == idx
        for j in range(NJ):
            y = jnp.dot(a, pltpu.bitcast(wd.at[j].bitcast(u32)[...], bf16), preferred_element_type=f32) * sg
            cur = pltpu.bitcast(outb.at[j].bitcast(u32)[pl.ds(pl.multiple_of(t16 * 8, 8), 8), :], bf16).astype(f32)
            patch[:, j * 128:(j + 1) * 128] = (cur + jnp.where(hit, y, 0.0)).astype(bf16)

    def patch_cp(idx):
        t0 = pl.multiple_of((idx // 16) * 16, 16)
        return pltpu.make_async_copy(patch, out_hbm.at[0, pl.ds(t0, 16), :], sem_p)

    waited = set()

    def wait_x(b):
        if b < NB:
            for i in range(R0[b] // XD, (R0[b] + BLOCKS[b] - 1) // XD + 1):
                if i not in waited:
                    waited.add(i)
                    wait(x_cps[i])

    def g0():
        start(xp_cps[0])
        for g in range(len(RAWG)):
            if g == X1POS:
                start(xp_cps[1])
            start(wg_cps[g])
        start(x_cps[2]); start(wo_cps)
        for i in range(3, NXD):
            start(x_cps[i])
        zero_ref[...] = jnp.zeros((8, 128), i32)
        for j in range(NJ):
            kb0[j, 0:HALO, :] = jnp.zeros((HALO, 128), f32)
            vb0[j, 0:HALO, :] = jnp.zeros((HALO, 128), f32)
        cx = Ctx()
        wait(xp_cps[0])
        ln1(cx, 0, lc=64)

    def raw_step(g):
        a, b = RAWG[g]
        cx = Ctx()
        if g == X1POS:
            wait(xp_cps[1])
        wait(wg_cps[g])
        raw_tiles(cx, range(a, b))
        if g == X1POS:
            ln1(cx, 1, lc=LC1)
        run_tasks(cx, g, -PL, PF * cx.t - PL)

    def run_tasks(cx, g, t0, t1):
        tasks = TASKS.get(g, [])
        cost = [len(js) * (40 if kind == "w" else 32) for kind, p, js in tasks]
        acc = 0
        for (kind, p, js), c in zip(tasks, cost):
            ta, tb = t0 + (t1 - t0) * acc / sum(cost), t0 + (t1 - t0) * (acc + c) / sum(cost)
            acc += c
            last = p * NJ + NJ - 1
            if kind == "w":
                assert g == len(RAWG) or last < RAWG[g][1]
                perm_w(cx, p, ta, tb, js)
            else:
                assert g == len(RAWG) or last < RAWG[g][0]
                perm_out(cx, p, ta, tb, js)

    def s0():
        cx = Ctx()
        wait_x(2)
        start(ffn_cps)
        a0, a1, l0, l1, p0, p1 = WIN[4]
        qkv_tiles(cx, 1, range(4))
        emit_tiles(cx)
        run_tasks(cx, len(RAWG), p0, p1)
        qkv_tiles(cx, 1, range(4, 15))
        emit_tiles(cx)
        attn(cx, 0, a0, cx.t - a1)
        ln1(cx, 2, l0, l1)

    def main_step(i, cx):
        ts = cx.t
        if i == 1:
            wrb[...] = jnp.broadcast_to(wr_ref[...].astype(f32).reshape(1, D), (8, D))
            qkv_tiles(cx, 2, range(4))
            emit_tiles(cx)
            permute_wo(cx, PW0, PW1)
            att = wo_tiles(cx, 0)
            qkv_tiles(cx, 2, range(4, 15))
        else:
            att = wo_tiles(cx, i - 1)
            qkv_tiles(cx, i + 1, range(15))
        emit_tiles(cx)
        tw = cx.tw
        a0, a1, l0, l1, p0, p1 = WIN[4 + i]
        attn(cx, i, ts + a0, cx.t - a1)
        if i + 2 < NB:
            ln1(cx, i + 2, ts + l0, ts + l1)
        post(cx, i - 1, att, tw + p0, cx.t - p1)

    def sep_step(i):
        cx = Ctx()
        if i == 1:
            wait(wo_cps)
        wait_x(i + 2)
        if i > 1:
            load_best(cx)
        main_step(i, cx)
        save_best(cx)

    def fence(cx, i):
        z = pl.multiple_of(one[0] - 1, 8)
        zf = jnp.zeros((8, 128), f32)
        qb[(i + 1) % 2][0, pl.ds(z + TM, 8), :] = zf
        kb[(i + 1) % 2][0, pl.ds(z + HALO + TM, 8), :] = zf
        vb[(i + 1) % 2][0, pl.ds(z + HALO + TM, 8), :] = zf
        xn[i % 2][pl.ds(z + TM // 2, 8), 0:128] = jnp.zeros((8, 128), u32)
        ob[i % 2][pl.ds(z + TM // 2, 8), 0:128] = functools.reduce(jnp.bitwise_or, cx.done)
        if WFENCE:
            wp[pl.ds(z + D // 2, 8), 0:128] = jnp.zeros((8, 128), u32)
            wop[pl.ds(z + D // 2, 8), 0:128] = jnp.zeros((8, 128), u32)
        cx.done = []

    def giant(lo, hi):
        cx = Ctx()
        for i in range(lo, hi):
            wait_x(i + 2)
        if lo > 1:
            load_best(cx)
        for i in range(lo, hi):
            main_step(i, cx)
            if i + 1 < hi:
                fence(cx, i)
        save_best(cx)

    L = NB - 1

    def final():
        cx = Ctx()
        wait(ffn_cps)
        for b in range(L - 2):
            wait(out_cps[b])
        bv0, bi0 = bestv[...], besti[...]
        if SPEC:
            rbest0, idx0 = argmax_of(bv0, bi0, R0[L - 1])
        att = wo_tiles(cx, L - 1)
        emit_tiles(cx)
        if SPEC:
            a = ffn_up(idx0, range(FSPLIT))
        if FG:
            attn(cx, L, -FGL, FG - FGL, rc=RCF)
        else:
            attn(cx, L, rc=RCF)
        t1 = cx.t
        att2 = wo_tiles(cx, L)
        emit_tiles(cx)
        if SPEC:
            a = a + ffn_up(idx0, range(FSPLIT, NF))
            ffn_down(a, rbest0, idx0)
        post(cx, L - 1, att, t1 + PG, t1 + PG + PSPAN, lc=min(LCF, BLOCKS[L - 1]))
        post(cx, L, att2, lc=min(LCF, BLOCKS[L]))
        bv1 = jnp.broadcast_to(cx.best[0], (8, 128))
        bi1 = jnp.broadcast_to(cx.best[1], (8, 128))

        def redo():
            take = bv1 > bv0
            rbest, idx = argmax_of(jnp.where(take, bv1, bv0), jnp.where(take, bi1, bi0))
            ffn_down(ffn_up(idx), rbest, idx)
            wait(out_cps[L - 2]); wait(out_cps[L - 1]); wait(out_cps[L])
            pc = patch_cp(idx)
            pc.start()
            pc.wait()

        if SPEC:
            miss = jnp.max(jnp.where(bv1 > rbest0, 1, 0)) > 0
            pl.when(miss)(redo)

            @pl.when(jnp.logical_not(miss))
            def _():
                wait(out_cps[L - 2])
                pc = patch_cp(idx0)
                pc.start()
                wait(out_cps[L - 1]); wait(out_cps[L])
                pc.wait()
        else:
            redo()

    if GIANT:
        cuts = list(range(1, L, GIANT)) + [L]
        if CUTS:
            cuts = CUTS
        mids = [functools.partial(giant, a, b) for a, b in zip(cuts[:-1], cuts[1:])]
    else:
        mids = [functools.partial(sep_step, i) for i in range(1, L)]
    steps = [g0] + [functools.partial(raw_step, g) for g in range(len(RAWG))] + [s0] + mids + [final]
    pid = pl.program_id(0)

    def wrap(n, fn):
        def scoped():
            with jax.named_scope(f"step{n}"):
                fn()
        return fn

    if FLAT:
        @pl.when(pid == 0)
        def _():
            one[0] = 1
            wrap(0, steps[0])()

        @pl.when(pid == 1)
        def _():
            v = one[0]
            for n, fn in enumerate(steps[1:]):
                pl.when(v > -n)(wrap(n + 1, fn))
    else:
        for n, fn in enumerate(steps):
            pl.when(pid == n)(wrap(n, fn))


NSTEPS = 5 + (NB - 2) + 1
NSEM = NXD + len(RAWG) + 1 + 1 + NB + 1


@jax.jit
def pallas_sequential_preLN__sliding_local_dilated__moe_arch_mod__prompt_kernel(
    A_x, A_wqkv, A_wo, B_x, B_w_r, B_w_gate, B_w_up, B_w_down,
):
    del B_x
    any_spec = pl.BlockSpec(memory_space=pl.ANY)
    return pl.pallas_call(
        _kernel,
        grid=(2 if FLAT else NSTEPS,),
        in_specs=[any_spec] * 7,
        out_specs=any_spec,
        out_shape=jax.ShapeDtypeStruct((1, S, D), bf16),
        scratch_shapes=[
            pltpu.VMEM((NJ, S, 128), bf16),
            pltpu.VMEM((2 * XD, D), bf16),
            pltpu.VMEM((D, 3 * D), bf16),
            pltpu.VMEM((3 * NJ, XD, 128), f32),
            pltpu.VMEM((NJ, D, 128), bf16),
            pltpu.VMEM((D // 2 + SPARE, 3 * D), u32),
            pltpu.VMEM((D // 2 + SPARE, D), u32),
            pltpu.VMEM((NF, D, 128), bf16),
            pltpu.VMEM((NF, D, 128), bf16),
            pltpu.VMEM((NJ, F, 128), bf16),
            pltpu.VMEM((D,), bf16),
            pltpu.VMEM((8, D), f32),
            pltpu.VMEM((TM // 2 + SPARE, D), u32),
            pltpu.VMEM((TM // 2 + SPARE, D), u32),
            pltpu.VMEM((NJ, TM + SPARE, 128), f32),
            pltpu.VMEM((NJ, TM + SPARE, 128), f32),
            pltpu.VMEM((NJ, HALO + TM + SPARE, 128), f32),
            pltpu.VMEM((NJ, HALO + TM + SPARE, 128), f32),
            pltpu.VMEM((NJ, HALO + TM + SPARE, 128), f32),
            pltpu.VMEM((NJ, HALO + TM + SPARE, 128), f32),
            pltpu.VMEM((TM // 2 + SPARE, D), u32),
            pltpu.VMEM((TM // 2 + SPARE, D), u32),
            pltpu.VMEM((S // 2, D), u32),
            pltpu.VMEM((NJ, S, 128), bf16),
            pltpu.VMEM((16, D), bf16),
            pltpu.VMEM((8, 128), f32),
            pltpu.VMEM((8, 128), i32),
            pltpu.VMEM((8, 128), i32),
            pltpu.SMEM((1,), i32),
            pltpu.SemaphoreType.DMA((NSEM,)),
        ],
        compiler_params=pltpu.CompilerParams(vmem_limit_bytes=100 * 1024 * 1024,
                                             dimension_semantics=("arbitrary",),
                                             disable_semaphore_checks=bool(int(1))),
        name="preln_swa_mod",
    )(A_x, A_wqkv, A_wo, B_w_r, B_w_gate, B_w_up, B_w_down)
```

```python
import functools
import math

import jax
import jax.numpy as jnp
from jax import lax
import jax.experimental.pallas as pl
import jax.experimental.pallas.tpu as pltpu

S = 2048
D = 640
DH = 20
W = 8
DIL = 2
F = 1536
NJ = D // 128
NF = F // 128
HALO = 16
EPS = 1e-5
LOG2E = math.log2(math.e)
QSCALE = (DH ** -0.5) * LOG2E
NEG = -1e9 * LOG2E
KA = 512

BLOCKS = [256, 256, 256, 256, 256, 256, 256, 128, 128]
NB = len(BLOCKS)
L = NB - 1
R0 = [sum(BLOCKS[:i]) for i in range(NB)]
TM = max(BLOCKS)
XD = 256
NXD = S // XD
assert sum(BLOCKS) == S and BLOCKS[0] == XD and BLOCKS[1] == XD

RAWG = [(0, 2), (2, 4), (4, 6), (6, 9), (9, 11), (11, 13), (13, 15)]
X1POS = 5
TASKS = {2: [("w", 0, (0, 1, 2))],
         3: [("w", 0, (3, 4)), ("o", 0, (0, 1, 2, 3, 4))],
         4: [("w", 1, (0, 1, 2, 3))],
         5: [("o", 1, (0, 1, 2))],
         6: [("o", 1, (3, 4)), ("w", 1, (4,)), ("w", 2, (0, 1, 2))],
         7: [("o", 2, (0, 1, 2, 3, 4)), ("w", 2, (3, 4))]}
assert all(sorted(j for ts in TASKS.values() for k, p, js in ts if (k, p) == kp for j in js) == list(range(NJ))
           for kp in [(k, p) for k in "wo" for p in range(3)])
WIN = {0: (729, 493, 509, 2471, -315, 805),
       1: (-273, 374, 356, 2648, 202, 319),
       2: (-58, 323, -142, 2124, 173, 377),
       3: (-58, 323, -142, 2124, 173, 377),
       4: (-58, 323, -142, 2124, 173, 377),
       5: (-83, 510, -216, 1258, -42, 637),
       6: (-79, 762, -82, 1505, -85, 690),
       7: (116, 753, -228, 1249, 133, 368)}
PERM_GROUP, PERM_FRAC, PERM_LEAD = 4, 0.28, 398.0
WO_WIN = (-137.0, 680.0)
FIN_UP_FIRST = 4
FIN_ATT = (-337.0, 114.0)
FIN_POST = (215.0, 508.0)
NSEM = (NXD - 2) + 2 + len(RAWG) + 2 + NB + 1

f32 = jnp.float32
bf16 = jnp.bfloat16
u32 = jnp.uint32
i32 = jnp.int32


def _cat(xs):
    return jnp.concatenate(xs, axis=1)


def _spread(t0, t1, c, n):
    return None if t0 is None else t0 + max(t1 - t0, 0.0) * c / n


def _center(x):
    m = jnp.sum(x, axis=-1, keepdims=True) * (1.0 / D)
    xc = x - m
    v = jnp.sum(xc * xc, axis=-1, keepdims=True) * (1.0 / D)
    return xc, jnp.exp2(jnp.log(v + EPS) * (-0.5 * LOG2E))


def _kernel(x_hbm, wqkv_hbm, wo_hbm, wr_hbm, wg_hbm, wu_hbm, wd_hbm, out_hbm,
            xbuf, xpre, wraw, rawb, woraw, wp, wop, wg, wu, wd, wr_ref, wrb,
            xn0, xn1, qb0, qb1, kb0, kb1, vb0, vb1, ob0, ob1, ln2b, outb, patch,
            bestv, besti, zero_ref, one, sem):
    xn = (xn0, xn1); qb = (qb0, qb1); kb = (kb0, kb1); vb = (vb0, vb1); ob = (ob0, ob1)

    nsem = [0]

    def group(pairs):
        s = sem.at[nsem[0]]
        nsem[0] += 1
        return [pltpu.make_async_copy(a, b, s) for a, b in pairs]

    def cols(j):
        return pl.ds(j * 128, 128)

    x_cps = [group([(x_hbm.at[0, pl.ds(i * XD, XD), cols(j)], xbuf.at[j, pl.ds(i * XD, XD), :])
                    for j in range(NJ)]) if i >= 2 else None for i in range(NXD)]
    xp_cps = [group([(x_hbm.at[0, pl.ds(i * XD, XD), :], xpre.at[pl.ds(i * XD, XD), :])]) for i in range(2)]
    wq_cps = [group([(wqkv_hbm.at[:, pl.ds(a * 128, (b - a) * 128)], wraw.at[:, pl.ds(a * 128, (b - a) * 128)])])
              for a, b in RAWG]
    wo_cps = group([(wo_hbm.at[:, cols(j)], woraw.at[j]) for j in range(NJ)] + [(wr_hbm, wr_ref)])
    ffn_cps = group([(wg_hbm.at[:, cols(n)], wg.at[n]) for n in range(NF)]
                    + [(wu_hbm.at[:, cols(n)], wu.at[n]) for n in range(NF)]
                    + [(wd_hbm.at[:, cols(j)], wd.at[j]) for j in range(NJ)])
    out_cps = [group([(outb.at[j, pl.ds(R0[b], BLOCKS[b]), :],
                       out_hbm.at[0, pl.ds(R0[b], BLOCKS[b]), cols(j)]) for j in range(NJ)])
               for b in range(NB)]
    sem_p = sem.at[nsem[0]]
    assert nsem[0] + 1 == NSEM

    def start(cs):
        for c in cs:
            c.start()

    def wait(cs):
        for c in cs:
            c.wait()

    waited = set()

    def wait_x(b):
        if b < NB:
            for i in range(R0[b] // XD, (R0[b] + BLOCKS[b] - 1) // XD + 1):
                if i not in waited:
                    waited.add(i)
                    wait(x_cps[i])

    class Step:
        def __init__(self):
            self.never = None
            self.best = None
            self.res = []
            self.pend = []
            self.t = 0.0

        def add(self, val, dur):
            self.res.append((self.t, self.t + dur, val))
            self.t += dur

        def gate(self, t, val):
            if t is None or t < 0 or not self.res:
                return val
            for (t0, t1, tv) in self.res:
                if t < t1:
                    break
            frac = min(max((t - t0) / (t1 - t0), 0.0), 0.999)
            r = int(frac * (tv.shape[0] // 8)) * 8
            tok = tv[r:r + 8, :]
            if self.never is None:
                self.never = zero_ref[...] != 0
            if val.dtype != tok.dtype:
                tok = pltpu.bitcast(tok, val.dtype)
            return jnp.where(self.never, tok, val)

    def lane_perm(load, store, nrg, cx, t0, t1, js):
        lane = lax.broadcasted_iota(i32, (8, 128), 1)
        lm5 = lane % 5
        base_idx = 20 * (lane % 32) + 5 * (lane // 32)
        ngrp = len(js) * ((nrg + PERM_GROUP - 1) // PERM_GROUP)
        gi = 0
        for j in js:
            idx = (base_idx + j) % 128
            for rg in range(nrg):
                if rg % PERM_GROUP == 0:
                    lg = cx.gate(_spread(t0, t1, gi, ngrp), lm5)
                    masks = [lg == ((j - 3 * i) % 5) for i in range(NJ)]
                    gi += 1
                src = [load(i, rg) for i in range(NJ)]
                z = src[0]
                for i in range(1, NJ):
                    z = jnp.where(masks[i], src[i], z)
                store(j, rg, jnp.take_along_axis(z, idx, axis=1))

    def perm_w(cx, p, t0, t1, js):
        def load(i, rg):
            return pltpu.bitcast(wraw[rg * 16:rg * 16 + 16, (p * NJ + i) * 128:(p * NJ + i + 1) * 128], u32)

        def store(j, rg, z):
            wp[rg * 8:rg * 8 + 8, p * D + j * 128: p * D + (j + 1) * 128] = z
        lane_perm(load, store, D // 16, cx, t0, t1, js)

    def perm_out(cx, p, t0, t1, js):
        def load(i, rg):
            return rawb[p * NJ + i, rg * 8:rg * 8 + 8, :]

        def store(j, rg, z):
            if p == 0:
                qb[0][j, rg * 8:rg * 8 + 8, :] = z
            else:
                (kb, vb)[p - 1][0][j, HALO + rg * 8:HALO + rg * 8 + 8, :] = z
        lane_perm(load, store, XD // 8, cx, t0, t1, js)

    def run_tasks(cx, g, t0, t1):
        tasks = TASKS.get(g, [])
        cost = [len(js) * (40 if kind == "w" else 32) for kind, p, js in tasks]
        acc = 0
        for (kind, p, js), c in zip(tasks, cost):
            ta, tb = t0 + (t1 - t0) * acc / sum(cost), t0 + (t1 - t0) * (acc + c) / sum(cost)
            acc += c
            last = p * NJ + NJ - 1
            if kind == "w":
                assert g == len(RAWG) or last < RAWG[g][1]
                perm_w(cx, p, ta, tb, js)
            else:
                assert g == len(RAWG) or last < RAWG[g][0]
                perm_out(cx, p, ta, tb, js)

    def perm_wo(cx, t0, t1):
        n = NJ * (DH // 2)
        for c in range(NJ):
            src = woraw.at[c].bitcast(u32)
            for m in range(DH // 2):
                t = _spread(t0, t1, c * (DH // 2) + m, n)
                mlo = cx.gate(t, jnp.full((8, 128), 0xFFFF, u32))
                sh = cx.gate(t, jnp.full((8, 128), 16, u32))
                for half in range(2):
                    a = src[pl.ds(m + 160 * half, 8, stride=20), :]
                    b = src[pl.ds(m + 10 + 160 * half, 8, stride=20), :]
                    lo = (a & mlo) | (b << sh)
                    hi = (a >> sh) | (b & ~mlo)
                    for d, val in ((2 * m, lo), (2 * m + 1, hi)):
                        j, g = d % 5, d // 5
                        r = (j * 128 + g * 32) // 2 + 8 * half
                        wop[r:r + 8, c * 128:(c + 1) * 128] = val

    def emit_tiles(cx, balance=False):
        pend, cx.pend = cx.pend, []
        for g in range(0, len(pend), 4):
            grp = pend[g:g + 4]
            nsp = 4 // math.gcd(len(grp), 4) if balance else 1
            tb = []
            for lhs, rhs_fn, sink in grp:
                rhs = rhs_fn(KA, D)
                mq = lhs.shape[0] // nsp
                parts = [jnp.dot(lhs[r:r + mq, KA:], rhs, preferred_element_type=f32)
                         for r in range(0, lhs.shape[0], mq)]
                tb.append(parts[0] if nsp == 1 else jnp.concatenate(parts, axis=0))
            cx.add(tb[-1], sum(p[0].shape[0] for p in grp) / 4.0)
            for (lhs, rhs_fn, sink), b in zip(grp, tb):
                t = jnp.dot(lhs[:, :KA], rhs_fn(0, KA), preferred_element_type=f32) + b
                cx.add(t, float(lhs.shape[0]))
                sink(t)

    def packed_rhs(wref, n, k0, k1):
        return pltpu.bitcast(wref[k0 // 2:k1 // 2, n * 128:(n + 1) * 128], bf16)

    def raw_tiles(cx, tiles):
        lhs = pltpu.bitcast(xn[0][0:XD // 2, :], bf16)

        def sink(n, t):
            rawb[n] = t
        for n in tiles:
            cx.pend.append((lhs, lambda k0, k1, n=n: wraw[k0:k1, n * 128:(n + 1) * 128],
                            functools.partial(sink, n)))
        emit_tiles(cx, balance=True)

    def qkv_tiles(cx, b, tiles):
        m = BLOCKS[b]
        lhs = pltpu.bitcast(xn[b % 2][0:m // 2, :], bf16)

        def sink(n, t):
            p, j = divmod(n, NJ)
            if p == 0:
                qb[b % 2][j, 0:m, :] = t
            else:
                dst = (kb, vb)[p - 1]
                mp = BLOCKS[b - 1]
                dst[b % 2][j, 0:HALO, :] = dst[(b - 1) % 2][j, mp:mp + HALO, :]
                dst[b % 2][j, HALO:HALO + m, :] = t
        for n in tiles:
            cx.pend.append((lhs, functools.partial(packed_rhs, wp, n), functools.partial(sink, n)))

    def wo_tiles(cx, b):
        m = BLOCKS[b]
        lhs = pltpu.bitcast(ob[b % 2][0:m // 2, :], bf16)
        att = []

        def sink(t):
            att.append(t)
            cx.tw = cx.t
        for n in range(NJ):
            cx.pend.append((lhs, functools.partial(packed_rhs, wop, n), sink))
        return att

    def load_x(cx, b, r, n, t):
        out = []
        for j in range(NJ):
            if b < 2:
                parts = [cx.gate(t, pltpu.bitcast(xpre[r + k:r + k + 16, j * 128:(j + 1) * 128], u32))
                         for k in range(0, n, 16)]
            else:
                v = xbuf.at[j].bitcast(u32)
                parts = [cx.gate(t, v[(r + k) // 2:(r + k) // 2 + 8, :]) for k in range(0, n, 16)]
            v = parts[0] if len(parts) == 1 else jnp.concatenate(parts, axis=0)
            out.append(pltpu.bitcast(v, bf16).astype(f32))
        return _cat(out)

    def ln1(cx, b, t0=None, t1=None, lc=16):
        n = BLOCKS[b] // lc
        for c in range(n):
            a0 = c * lc
            xc, rs = _center(load_x(cx, b, R0[b] + a0, lc, _spread(t0, t1, c, n)))
            xn[b % 2][a0 // 2:(a0 + lc) // 2, :] = pltpu.bitcast((xc * rs).astype(bf16), u32)

    def attn(cx, b, t0, t1):
        qr, kr, vr = qb[b % 2], kb[b % 2], vb[b % 2]
        n = BLOCKS[b] // 8
        for c in range(n):
            a0 = c * 8
            sc = cx.gate(_spread(t0, t1, c, n), jnp.full((8, 128), QSCALE, f32))
            q = [qr[j, a0:a0 + 8, :] * sc for j in range(NJ)]
            tt = []
            for w in range(W):
                k0 = HALO + a0 - DIL * w
                acc = q[0] * kr[0, k0:k0 + 8, :]
                for j in range(1, NJ):
                    acc = acc + q[j] * kr[j, k0:k0 + 8, :]
                tt.append(acc)
            r1 = [pltpu.roll(tt[w], 64, 1) for w in range(W)]
            tt = [tt[w] + r1[w] for w in range(W)]
            r2 = [pltpu.roll(tt[w], 32, 1) for w in range(W)]
            s = [tt[w] + r2[w] for w in range(W)]
            for w in range(W):
                if b == 0 and a0 - DIL * w < 0:
                    row = lax.broadcasted_iota(i32, (8, 128), 0) + (a0 - DIL * w)
                    s[w] = jnp.where(row >= 0, s[w], NEG)
            mx = functools.reduce(jnp.maximum, s)
            p = [jnp.exp2(s[w] - mx) for w in range(W)]
            inv = pl.reciprocal(functools.reduce(lambda u, v: u + v, p), approx=True)
            o = []
            for j in range(NJ):
                acc = None
                for w in range(W):
                    k0 = HALO + a0 - DIL * w
                    term = p[w] * vr[j, k0:k0 + 8, :]
                    acc = term if acc is None else acc + term
                o.append(acc * inv)
            if c % 2 == 0:
                prev = o
                continue
            o = [jnp.concatenate([prev[j], o[j]], axis=0) for j in range(NJ)]
            for j in range(NJ):
                ob[b % 2][(a0 - 8) // 2:(a0 + 8) // 2, j * 128:(j + 1) * 128] = pltpu.bitcast(o[j].astype(bf16), u32)

    def post(cx, b, att, t0=None, t1=None):
        r0 = R0[b]
        n = BLOCKS[b] // 16
        for c in range(n):
            a0 = c * 16
            h = (load_x(cx, b, r0 + a0, 16, _spread(t0, t1, c, n))
                 + _cat([att[j][a0:a0 + 16, :] for j in range(NJ)]))
            xc, rs = _center(h)
            r = jnp.sum(xc * jnp.tile(wrb[...], (2, 1)), axis=-1, keepdims=True) * rs
            ln2 = xc * rs
            ln2b[(r0 + a0) // 2:(r0 + a0 + 16) // 2, :] = pltpu.bitcast(ln2.astype(bf16), u32)
            o = pltpu.bitcast((h + ln2).astype(bf16), u32)
            for j in range(NJ):
                outb.at[j].bitcast(u32)[(r0 + a0) // 2:(r0 + a0 + 16) // 2, :] = o[:, j * 128:(j + 1) * 128]
            for k in (0, 8):
                rk = r[k:k + 8, :]
                if cx.best is None:
                    cx.best = (rk, jnp.full((8, 1), r0 + a0 + k, i32))
                else:
                    bv, bi = cx.best
                    take = rk > bv
                    cx.best = (jnp.where(take, rk, bv), jnp.where(take, r0 + a0 + k, bi))
        start(out_cps[b])

    def argmax_of(bv, bi, nrows):
        rowid = bi + lax.broadcasted_iota(i32, (8, 128), 0)
        rbest = jnp.max(bv, axis=0, keepdims=True)
        idx = jnp.clip(jnp.min(jnp.where(bv == rbest, rowid, S)), 0, nrows - 1)
        return rbest, idx

    def ffn_up(idx, tiles):
        t16 = idx // 16
        xs = pltpu.bitcast(ln2b[pl.ds(pl.multiple_of(t16 * 8, 8), 8), :], bf16)
        a = []
        for n in tiles:
            g = jnp.dot(xs, pltpu.bitcast(wg.at[n].bitcast(u32)[...], bf16), preferred_element_type=f32)
            u = jnp.dot(xs, pltpu.bitcast(wu.at[n].bitcast(u32)[...], bf16), preferred_element_type=f32)
            a.append((g * jax.nn.sigmoid(g) * u).astype(bf16))
        return a

    def ffn_down(a, rbest, idx):
        a = _cat(a)
        sg = jax.nn.sigmoid(rbest)
        t16 = idx // 16
        hit = (lax.broadcasted_iota(i32, (16, 128), 0) + t16 * 16) == idx
        for j in range(NJ):
            y = jnp.dot(a, pltpu.bitcast(wd.at[j].bitcast(u32)[...], bf16), preferred_element_type=f32) * sg
            cur = pltpu.bitcast(outb.at[j].bitcast(u32)[pl.ds(pl.multiple_of(t16 * 8, 8), 8), :], bf16).astype(f32)
            patch[:, j * 128:(j + 1) * 128] = (cur + jnp.where(hit, y, 0.0)).astype(bf16)

    def patch_cp(idx):
        t0 = pl.multiple_of((idx // 16) * 16, 16)
        return pltpu.make_async_copy(patch, out_hbm.at[0, pl.ds(t0, 16), :], sem_p)

    def first():
        start(xp_cps[0])
        for g in range(len(RAWG)):
            if g == X1POS:
                start(xp_cps[1])
            start(wq_cps[g])
        start(x_cps[2])
        start(wo_cps)
        for i in range(3, NXD):
            start(x_cps[i])
        zero_ref[...] = jnp.zeros((8, 128), i32)
        for j in range(NJ):
            kb0[j, 0:HALO, :] = jnp.zeros((HALO, 128), f32)
            vb0[j, 0:HALO, :] = jnp.zeros((HALO, 128), f32)
        wait(xp_cps[0])
        ln1(Step(), 0, lc=64)

    def raw_step(g):
        cx = Step()
        if g == X1POS:
            wait(xp_cps[1])
        wait(wq_cps[g])
        raw_tiles(cx, range(*RAWG[g]))
        if g == X1POS:
            ln1(cx, 1, lc=32)
        run_tasks(cx, g, -PERM_LEAD, PERM_FRAC * cx.t - PERM_LEAD)

    def step0():
        cx = Step()
        wait_x(2)
        start(ffn_cps)
        a0, a1, l0, l1, p0, p1 = WIN[0]
        qkv_tiles(cx, 1, range(4))
        emit_tiles(cx)
        run_tasks(cx, len(RAWG), p0, p1)
        qkv_tiles(cx, 1, range(4, 15))
        emit_tiles(cx)
        attn(cx, 0, a0, cx.t - a1)
        ln1(cx, 2, l0, l1)

    def main_step(i):
        cx = Step()
        if i == 1:
            wait(wo_cps)
        wait_x(i + 2)
        if i == 1:
            wrb[...] = jnp.broadcast_to(wr_ref[...].astype(f32).reshape(1, D), (8, D))
            qkv_tiles(cx, 2, range(4))
            emit_tiles(cx)
            perm_wo(cx, *WO_WIN)
            att = wo_tiles(cx, 0)
            qkv_tiles(cx, 2, range(4, 15))
        else:
            cx.best = (bestv[:, 0:1], besti[:, 0:1])
            att = wo_tiles(cx, i - 1)
            qkv_tiles(cx, i + 1, range(15))
        emit_tiles(cx)
        a0, a1, l0, l1, p0, p1 = WIN[i]
        attn(cx, i, a0, cx.t - a1)
        if i + 2 < NB:
            ln1(cx, i + 2, l0, l1)
        post(cx, i - 1, att, cx.tw + p0, cx.t - p1)
        bestv[...] = jnp.broadcast_to(cx.best[0], (8, 128))
        besti[...] = jnp.broadcast_to(cx.best[1], (8, 128))

    def final():
        cx = Step()
        wait(ffn_cps)
        for b in range(L - 2):
            wait(out_cps[b])
        bv0, bi0 = bestv[...], besti[...]
        rbest0, idx0 = argmax_of(bv0, bi0, R0[L - 1])
        att = wo_tiles(cx, L - 1)
        emit_tiles(cx)
        a = ffn_up(idx0, range(FIN_UP_FIRST))
        attn(cx, L, *FIN_ATT)
        t1 = cx.t
        att2 = wo_tiles(cx, L)
        emit_tiles(cx)
        a = a + ffn_up(idx0, range(FIN_UP_FIRST, NF))
        ffn_down(a, rbest0, idx0)
        post(cx, L - 1, att, t1 + FIN_POST[0], t1 + FIN_POST[1])
        post(cx, L, att2)
        bv1 = jnp.broadcast_to(cx.best[0], (8, 128))
        bi1 = jnp.broadcast_to(cx.best[1], (8, 128))
        miss = jnp.max(jnp.where(bv1 > rbest0, 1, 0)) > 0

        @pl.when(miss)
        def _():
            take = bv1 > bv0
            rbest, idx = argmax_of(jnp.where(take, bv1, bv0), jnp.where(take, bi1, bi0), S)
            ffn_down(ffn_up(idx, range(NF)), rbest, idx)
            for b in (L - 2, L - 1, L):
                wait(out_cps[b])
            pc = patch_cp(idx)
            pc.start()
            pc.wait()

        @pl.when(jnp.logical_not(miss))
        def _():
            wait(out_cps[L - 2])
            pc = patch_cp(idx0)
            pc.start()
            wait(out_cps[L - 1])
            wait(out_cps[L])
            pc.wait()

    steps = ([functools.partial(raw_step, g) for g in range(len(RAWG))] + [step0]
             + [functools.partial(main_step, i) for i in range(1, L)] + [final])
    pid = pl.program_id(0)

    @pl.when(pid == 0)
    def _():
        one[0] = 1
        first()

    @pl.when(pid == 1)
    def _():
        v = one[0]
        for n, fn in enumerate(steps):
            pl.when(v > -n)(fn)


@jax.jit
def pallas_sequential_preLN__sliding_local_dilated__moe_arch_mod__prompt_kernel(
    A_x: jax.Array,
    A_wqkv: jax.Array,
    A_wo: jax.Array,
    B_x: jax.Array,
    B_w_r: jax.Array,
    B_w_gate: jax.Array,
    B_w_up: jax.Array,
    B_w_down: jax.Array,
):
    del B_x
    any_spec = pl.BlockSpec(memory_space=pl.ANY)
    return pl.pallas_call(
        _kernel,
        grid=(2,),
        in_specs=[any_spec] * 7,
        out_specs=any_spec,
        out_shape=jax.ShapeDtypeStruct((1, S, D), bf16),
        scratch_shapes=[
            pltpu.VMEM((NJ, S, 128), bf16),
            pltpu.VMEM((2 * XD, D), bf16),
            pltpu.VMEM((D, 3 * D), bf16),
            pltpu.VMEM((3 * NJ, XD, 128), f32),
            pltpu.VMEM((NJ, D, 128), bf16),
            pltpu.VMEM((D // 2, 3 * D), u32),
            pltpu.VMEM((D // 2, D), u32),
            pltpu.VMEM((NF, D, 128), bf16),
            pltpu.VMEM((NF, D, 128), bf16),
            pltpu.VMEM((NJ, F, 128), bf16),
            pltpu.VMEM((D,), bf16),
            pltpu.VMEM((8, D), f32),
            pltpu.VMEM((TM // 2, D), u32),
            pltpu.VMEM((TM // 2, D), u32),
            pltpu.VMEM((NJ, TM, 128), f32),
            pltpu.VMEM((NJ, TM, 128), f32),
            pltpu.VMEM((NJ, HALO + TM, 128), f32),
            pltpu.VMEM((NJ, HALO + TM, 128), f32),
            pltpu.VMEM((NJ, HALO + TM, 128), f32),
            pltpu.VMEM((NJ, HALO + TM, 128), f32),
            pltpu.VMEM((TM // 2, D), u32),
            pltpu.VMEM((TM // 2, D), u32),
            pltpu.VMEM((S // 2, D), u32),
            pltpu.VMEM((NJ, S, 128), bf16),
            pltpu.VMEM((16, D), bf16),
            pltpu.VMEM((8, 128), f32),
            pltpu.VMEM((8, 128), i32),
            pltpu.VMEM((8, 128), i32),
            pltpu.SMEM((1,), i32),
            pltpu.SemaphoreType.DMA((NSEM,)),
        ],
        compiler_params=pltpu.CompilerParams(vmem_limit_bytes=100 * 1024 * 1024,
                                             dimension_semantics=("arbitrary",),
                                             disable_semaphore_checks=True),
        name="preln_swa_mod",
    )(A_x, A_wqkv, A_wo, B_w_r, B_w_gate, B_w_up, B_w_down)
```

```python
import functools
import math

import jax
import jax.numpy as jnp
from jax import lax
import jax.experimental.pallas as pl
import jax.experimental.pallas.tpu as pltpu

S = 2048
D = 640
DH = 20
W = 8
DIL = 2
F = 1536
NJ = D // 128
NF = F // 128
HALO = 16
EPS = 1e-5
LOG2E = math.log2(math.e)
QSCALE = (DH ** -0.5) * LOG2E
NEG = -1e9 * LOG2E
KA = 512

BLOCKS = [256, 256, 256, 256, 256, 256, 256, 128, 128]
NB = len(BLOCKS)
L = NB - 1
R0 = [sum(BLOCKS[:i]) for i in range(NB)]
TM = max(BLOCKS)
XD = 256
NXD = S // XD
assert sum(BLOCKS) == S and BLOCKS[0] == XD and BLOCKS[1] == XD

RAWG = [(0, 2), (2, 4), (4, 6), (6, 9), (9, 11), (11, 13), (13, 15)]
X1POS = 5
TASKS = {2: [("w", 0, (0, 1, 2))],
         3: [("w", 0, (3, 4)), ("o", 0, (0, 1, 2, 3, 4))],
         4: [("w", 1, (0, 1, 2, 3))],
         5: [("o", 1, (0, 1, 2))],
         6: [("o", 1, (3, 4)), ("w", 1, (4,)), ("w", 2, (0, 1, 2))],
         7: [("o", 2, (0, 1, 2, 3, 4)), ("w", 2, (3, 4))]}
assert all(sorted(j for ts in TASKS.values() for k, p, js in ts if (k, p) == kp for j in js) == list(range(NJ))
           for kp in [(k, p) for k in "wo" for p in range(3)])
WIN = {0: (721, 608, 518, 2324, -358, 786),
       1: (-8, 445, 84, 2045, -99, 397),
       2: (-58, 323, -142, 2124, 173, 377),
       3: (-58, 323, -142, 2124, 173, 377),
       4: (-58, 323, -142, 2124, 173, 377),
       5: (-83, 510, -216, 1258, -42, 637),
       6: (-79, 762, -82, 1505, -85, 690),
       7: (116, 753, -228, 1249, 133, 368)}
PERM_GROUP, PERM_FRAC, PERM_LEAD = 4, 0.28, 398.0
WO_WIN = (-270.0, 627.0)
FIN_UP_FIRST = 4
FIN_ATT = (-337.0, 114.0)
FIN_POST = (215.0, 508.0)
NSEM = (NXD - 2) + 2 + len(RAWG) + 2 + NB + 1

f32 = jnp.float32
bf16 = jnp.bfloat16
u32 = jnp.uint32
i32 = jnp.int32


def _cat(xs):
    return jnp.concatenate(xs, axis=1)


def _spread(t0, t1, c, n):
    return None if t0 is None else t0 + max(t1 - t0, 0.0) * c / n


def _center(x):
    m = jnp.sum(x, axis=-1, keepdims=True) * (1.0 / D)
    xc = x - m
    v = jnp.sum(xc * xc, axis=-1, keepdims=True) * (1.0 / D)
    return xc, jnp.exp2(jnp.log(v + EPS) * (-0.5 * LOG2E))


def _kernel(x_hbm, wqkv_hbm, wo_hbm, wr_hbm, wg_hbm, wu_hbm, wd_hbm, out_hbm,
            xbuf, xpre, wraw, rawb, woraw, wp, wop, wg, wu, wd, wr_ref, wrb,
            xn0, xn1, qb0, qb1, kb0, kb1, vb0, vb1, ob0, ob1, ln2b, outb, patch,
            bestv, besti, zero_ref, one, sem):
    xn = (xn0, xn1); qb = (qb0, qb1); kb = (kb0, kb1); vb = (vb0, vb1); ob = (ob0, ob1)

    nsem = [0]

    def group(pairs):
        s = sem.at[nsem[0]]
        nsem[0] += 1
        return [pltpu.make_async_copy(a, b, s) for a, b in pairs]

    def cols(j):
        return pl.ds(j * 128, 128)

    x_cps = [group([(x_hbm.at[0, pl.ds(i * XD, XD), cols(j)], xbuf.at[j, pl.ds(i * XD, XD), :])
                    for j in range(NJ)]) if i >= 2 else None for i in range(NXD)]
    xp_cps = [group([(x_hbm.at[0, pl.ds(i * XD, XD), :], xpre.at[pl.ds(i * XD, XD), :])]) for i in range(2)]
    wq_cps = [group([(wqkv_hbm.at[:, pl.ds(a * 128, (b - a) * 128)], wraw.at[:, pl.ds(a * 128, (b - a) * 128)])])
              for a, b in RAWG]
    wo_cps = group([(wo_hbm.at[:, cols(j)], woraw.at[j]) for j in range(NJ)] + [(wr_hbm, wr_ref)])
    ffn_cps = group([(wg_hbm.at[:, cols(n)], wg.at[n]) for n in range(NF)]
                    + [(wu_hbm.at[:, cols(n)], wu.at[n]) for n in range(NF)]
                    + [(wd_hbm.at[:, cols(j)], wd.at[j]) for j in range(NJ)])
    out_cps = [group([(outb.at[j, pl.ds(R0[b], BLOCKS[b]), :],
                       out_hbm.at[0, pl.ds(R0[b], BLOCKS[b]), cols(j)]) for j in range(NJ)])
               for b in range(NB)]
    sem_p = sem.at[nsem[0]]
    assert nsem[0] + 1 == NSEM

    def start(cs):
        for c in cs:
            c.start()

    def wait(cs):
        for c in cs:
            c.wait()

    waited = set()

    def wait_x(b):
        if b < NB:
            for i in range(R0[b] // XD, (R0[b] + BLOCKS[b] - 1) // XD + 1):
                if i not in waited:
                    waited.add(i)
                    wait(x_cps[i])

    class Step:
        def __init__(self):
            self.never = None
            self.best = None
            self.res = []
            self.pend = []
            self.t = 0.0

        def add(self, val, dur):
            self.res.append((self.t, self.t + dur, val))
            self.t += dur

        def gate(self, t, val):
            if t is None or t < 0 or not self.res:
                return val
            for (t0, t1, tv) in self.res:
                if t < t1:
                    break
            frac = min(max((t - t0) / (t1 - t0), 0.0), 0.999)
            r = int(frac * (tv.shape[0] // 8)) * 8
            tok = tv[r:r + 8, :]
            if self.never is None:
                self.never = zero_ref[...] != 0
            if val.dtype != tok.dtype:
                tok = pltpu.bitcast(tok, val.dtype)
            return jnp.where(self.never, tok, val)

    def lane_perm(load, store, nrg, cx, t0, t1, js):
        lane = lax.broadcasted_iota(i32, (8, 128), 1)
        lm5 = lane % 5
        base_idx = 20 * (lane % 32) + 5 * (lane // 32)
        ngrp = len(js) * ((nrg + PERM_GROUP - 1) // PERM_GROUP)
        gi = 0
        for j in js:
            idx = (base_idx + j) % 128
            for rg in range(nrg):
                if rg % PERM_GROUP == 0:
                    lg = cx.gate(_spread(t0, t1, gi, ngrp), lm5)
                    masks = [lg == ((j - 3 * i) % 5) for i in range(NJ)]
                    gi += 1
                src = [load(i, rg) for i in range(NJ)]
                z = src[0]
                for i in range(1, NJ):
                    z = jnp.where(masks[i], src[i], z)
                store(j, rg, jnp.take_along_axis(z, idx, axis=1))

    def perm_w(cx, p, t0, t1, js):
        def load(i, rg):
            return pltpu.bitcast(wraw[rg * 16:rg * 16 + 16, (p * NJ + i) * 128:(p * NJ + i + 1) * 128], u32)

        def store(j, rg, z):
            wp[rg * 8:rg * 8 + 8, p * D + j * 128: p * D + (j + 1) * 128] = z
        lane_perm(load, store, D // 16, cx, t0, t1, js)

    def perm_out(cx, p, t0, t1, js):
        def load(i, rg):
            return rawb[p * NJ + i, rg * 8:rg * 8 + 8, :]

        def store(j, rg, z):
            if p == 0:
                qb[0][j, rg * 8:rg * 8 + 8, :] = z
            else:
                (kb, vb)[p - 1][0][j, HALO + rg * 8:HALO + rg * 8 + 8, :] = z
        lane_perm(load, store, XD // 8, cx, t0, t1, js)

    def run_tasks(cx, g, t0, t1):
        tasks = TASKS.get(g, [])
        cost = [len(js) * (40 if kind == "w" else 32) for kind, p, js in tasks]
        acc = 0
        for (kind, p, js), c in zip(tasks, cost):
            ta, tb = t0 + (t1 - t0) * acc / sum(cost), t0 + (t1 - t0) * (acc + c) / sum(cost)
            acc += c
            last = p * NJ + NJ - 1
            if kind == "w":
                assert g == len(RAWG) or last < RAWG[g][1]
                perm_w(cx, p, ta, tb, js)
            else:
                assert g == len(RAWG) or last < RAWG[g][0]
                perm_out(cx, p, ta, tb, js)

    def perm_wo(cx, t0, t1):
        n = NJ * (DH // 2)
        for c in range(NJ):
            src = woraw.at[c].bitcast(u32)
            for m in range(DH // 2):
                t = _spread(t0, t1, c * (DH // 2) + m, n)
                mlo = cx.gate(t, jnp.full((8, 128), 0xFFFF, u32))
                sh = cx.gate(t, jnp.full((8, 128), 16, u32))
                for half in range(2):
                    a = src[pl.ds(m + 160 * half, 8, stride=20), :]
                    b = src[pl.ds(m + 10 + 160 * half, 8, stride=20), :]
                    lo = (a & mlo) | (b << sh)
                    hi = (a >> sh) | (b & ~mlo)
                    for d, val in ((2 * m, lo), (2 * m + 1, hi)):
                        j, g = d % 5, d // 5
                        r = (j * 128 + g * 32) // 2 + 8 * half
                        wop[r:r + 8, c * 128:(c + 1) * 128] = val

    def emit_tiles(cx, balance=False):
        pend, cx.pend = cx.pend, []
        for g in range(0, len(pend), 4):
            grp = pend[g:g + 4]
            nsp = 4 // math.gcd(len(grp), 4) if balance else 1
            tb = []
            for lhs, rhs_fn, sink in grp:
                rhs = rhs_fn(KA, D)
                mq = lhs.shape[0] // nsp
                parts = [jnp.dot(lhs[r:r + mq, KA:], rhs, preferred_element_type=f32)
                         for r in range(0, lhs.shape[0], mq)]
                tb.append(parts[0] if nsp == 1 else jnp.concatenate(parts, axis=0))
            cx.add(tb[-1], sum(p[0].shape[0] for p in grp) / 4.0)
            for (lhs, rhs_fn, sink), b in zip(grp, tb):
                t = jnp.dot(lhs[:, :KA], rhs_fn(0, KA), preferred_element_type=f32) + b
                cx.add(t, float(lhs.shape[0]))
                sink(t)

    def packed_rhs(wref, n, k0, k1):
        return pltpu.bitcast(wref[k0 // 2:k1 // 2, n * 128:(n + 1) * 128], bf16)

    def raw_tiles(cx, tiles):
        lhs = pltpu.bitcast(xn[0][0:XD // 2, :], bf16)

        def sink(n, t):
            rawb[n] = t
        for n in tiles:
            cx.pend.append((lhs, lambda k0, k1, n=n: wraw[k0:k1, n * 128:(n + 1) * 128],
                            functools.partial(sink, n)))
        emit_tiles(cx, balance=True)

    def qkv_tiles(cx, b, tiles):
        m = BLOCKS[b]
        lhs = pltpu.bitcast(xn[b % 2][0:m // 2, :], bf16)

        def sink(n, t):
            p, j = divmod(n, NJ)
            if p == 0:
                qb[b % 2][j, 0:m, :] = t
            else:
                dst = (kb, vb)[p - 1]
                mp = BLOCKS[b - 1]
                dst[b % 2][j, 0:HALO, :] = dst[(b - 1) % 2][j, mp:mp + HALO, :]
                dst[b % 2][j, HALO:HALO + m, :] = t
        for n in tiles:
            cx.pend.append((lhs, functools.partial(packed_rhs, wp, n), functools.partial(sink, n)))

    def wo_tiles(cx, b):
        m = BLOCKS[b]
        lhs = pltpu.bitcast(ob[b % 2][0:m // 2, :], bf16)
        att = []

        def sink(t):
            att.append(t)
            cx.tw = cx.t
        for n in range(NJ):
            cx.pend.append((lhs, functools.partial(packed_rhs, wop, n), sink))
        return att

    def load_x(cx, b, r, n, t):
        out = []
        for j in range(NJ):
            if b < 2:
                parts = [cx.gate(t, pltpu.bitcast(xpre[r + k:r + k + 16, j * 128:(j + 1) * 128], u32))
                         for k in range(0, n, 16)]
            else:
                v = xbuf.at[j].bitcast(u32)
                parts = [cx.gate(t, v[(r + k) // 2:(r + k) // 2 + 8, :]) for k in range(0, n, 16)]
            v = parts[0] if len(parts) == 1 else jnp.concatenate(parts, axis=0)
            out.append(pltpu.bitcast(v, bf16).astype(f32))
        return _cat(out)

    def ln1(cx, b, t0=None, t1=None, lc=16):
        n = BLOCKS[b] // lc
        for c in range(n):
            a0 = c * lc
            xc, rs = _center(load_x(cx, b, R0[b] + a0, lc, _spread(t0, t1, c, n)))
            xn[b % 2][a0 // 2:(a0 + lc) // 2, :] = pltpu.bitcast((xc * rs).astype(bf16), u32)

    def attn(cx, b, t0, t1):
        qr, kr, vr = qb[b % 2], kb[b % 2], vb[b % 2]
        n = BLOCKS[b] // 8
        for c in range(n):
            a0 = c * 8
            sc = cx.gate(_spread(t0, t1, c, n), jnp.full((8, 128), QSCALE, f32))
            q = [qr[j, a0:a0 + 8, :] * sc for j in range(NJ)]
            tt = []
            for w in range(W):
                k0 = HALO + a0 - DIL * w
                acc = q[0] * kr[0, k0:k0 + 8, :]
                for j in range(1, NJ):
                    acc = acc + q[j] * kr[j, k0:k0 + 8, :]
                tt.append(acc)
            r1 = [pltpu.roll(tt[w], 64, 1) for w in range(W)]
            tt = [tt[w] + r1[w] for w in range(W)]
            r2 = [pltpu.roll(tt[w], 32, 1) for w in range(W)]
            s = [tt[w] + r2[w] for w in range(W)]
            for w in range(W):
                if b == 0 and a0 - DIL * w < 0:
                    row = lax.broadcasted_iota(i32, (8, 128), 0) + (a0 - DIL * w)
                    s[w] = jnp.where(row >= 0, s[w], NEG)
            mx = functools.reduce(jnp.maximum, s)
            p = [jnp.exp2(s[w] - mx) for w in range(W)]
            inv = pl.reciprocal(functools.reduce(lambda u, v: u + v, p), approx=True)
            o = []
            for j in range(NJ):
                acc = None
                for w in range(W):
                    k0 = HALO + a0 - DIL * w
                    term = p[w] * vr[j, k0:k0 + 8, :]
                    acc = term if acc is None else acc + term
                o.append(acc * inv)
            if c % 2 == 0:
                prev = o
                continue
            o = [jnp.concatenate([prev[j], o[j]], axis=0) for j in range(NJ)]
            for j in range(NJ):
                ob[b % 2][(a0 - 8) // 2:(a0 + 8) // 2, j * 128:(j + 1) * 128] = pltpu.bitcast(o[j].astype(bf16), u32)

    def post(cx, b, att, t0=None, t1=None):
        r0 = R0[b]
        n = BLOCKS[b] // 16
        for c in range(n):
            a0 = c * 16
            h = (load_x(cx, b, r0 + a0, 16, _spread(t0, t1, c, n))
                 + _cat([att[j][a0:a0 + 16, :] for j in range(NJ)]))
            xc, rs = _center(h)
            r = jnp.sum(xc * jnp.tile(wrb[...], (2, 1)), axis=-1, keepdims=True) * rs
            ln2 = xc * rs
            ln2b[(r0 + a0) // 2:(r0 + a0 + 16) // 2, :] = pltpu.bitcast(ln2.astype(bf16), u32)
            o = pltpu.bitcast((h + ln2).astype(bf16), u32)
            for j in range(NJ):
                outb.at[j].bitcast(u32)[(r0 + a0) // 2:(r0 + a0 + 16) // 2, :] = o[:, j * 128:(j + 1) * 128]
            for k in (0, 8):
                rk = r[k:k + 8, :]
                if cx.best is None:
                    cx.best = (rk, jnp.full((8, 1), r0 + a0 + k, i32))
                else:
                    bv, bi = cx.best
                    take = rk > bv
                    cx.best = (jnp.where(take, rk, bv), jnp.where(take, r0 + a0 + k, bi))
        start(out_cps[b])

    def argmax_of(bv, bi, nrows, dtype=i32):
        rowid = (bi + lax.broadcasted_iota(i32, (8, 128), 0)).astype(dtype)
        rbest = jnp.max(bv, axis=0, keepdims=True)
        idx = jnp.min(jnp.where(bv == rbest, rowid, S)).astype(i32)
        return rbest, jnp.clip(idx, 0, nrows - 1)

    def ffn_up(idx, tiles):
        t16 = idx // 16
        xs = pltpu.bitcast(ln2b[pl.ds(pl.multiple_of(t16 * 8, 8), 8), :], bf16)
        a = []
        for n in tiles:
            g = jnp.dot(xs, pltpu.bitcast(wg.at[n].bitcast(u32)[...], bf16), preferred_element_type=f32)
            u = jnp.dot(xs, pltpu.bitcast(wu.at[n].bitcast(u32)[...], bf16), preferred_element_type=f32)
            a.append((g * jax.nn.sigmoid(g) * u).astype(bf16))
        return a

    def ffn_down(a, rbest, idx):
        a = _cat(a)
        sg = jax.nn.sigmoid(rbest)
        t16 = idx // 16
        hit = (lax.broadcasted_iota(i32, (16, 128), 0) + t16 * 16) == idx
        for j in range(NJ):
            y = jnp.dot(a, pltpu.bitcast(wd.at[j].bitcast(u32)[...], bf16), preferred_element_type=f32) * sg
            cur = pltpu.bitcast(outb.at[j].bitcast(u32)[pl.ds(pl.multiple_of(t16 * 8, 8), 8), :], bf16).astype(f32)
            patch[:, j * 128:(j + 1) * 128] = (cur + jnp.where(hit, y, 0.0)).astype(bf16)

    def patch_cp(idx):
        t0 = pl.multiple_of((idx // 16) * 16, 16)
        return pltpu.make_async_copy(patch, out_hbm.at[0, pl.ds(t0, 16), :], sem_p)

    def first():
        start(xp_cps[0])
        for g in range(len(RAWG)):
            if g == X1POS:
                start(xp_cps[1])
            start(wq_cps[g])
        start(x_cps[2])
        start(wo_cps)
        for i in range(3, NXD):
            start(x_cps[i])
        zero_ref[...] = jnp.zeros((8, 128), i32)
        for j in range(NJ):
            kb0[j, 0:HALO, :] = jnp.zeros((HALO, 128), f32)
            vb0[j, 0:HALO, :] = jnp.zeros((HALO, 128), f32)
        wait(xp_cps[0])
        ln1(Step(), 0, lc=64)

    def raw_step(g):
        cx = Step()
        if g == X1POS:
            wait(xp_cps[1])
        wait(wq_cps[g])
        raw_tiles(cx, range(*RAWG[g]))
        if g == X1POS:
            ln1(cx, 1, lc=32)
        run_tasks(cx, g, -PERM_LEAD, PERM_FRAC * cx.t - PERM_LEAD)

    def step0():
        cx = Step()
        wait_x(2)
        start(ffn_cps)
        a0, a1, l0, l1, p0, p1 = WIN[0]
        qkv_tiles(cx, 1, range(4))
        emit_tiles(cx)
        run_tasks(cx, len(RAWG), p0, p1)
        qkv_tiles(cx, 1, range(4, 15))
        emit_tiles(cx)
        attn(cx, 0, a0, cx.t - a1)
        ln1(cx, 2, l0, l1)

    def main_step(i):
        cx = Step()
        if i == 1:
            wait(wo_cps)
        wait_x(i + 2)
        if i == 1:
            wrb[...] = jnp.broadcast_to(wr_ref[...].astype(f32).reshape(1, D), (8, D))
            qkv_tiles(cx, 2, range(4))
            emit_tiles(cx)
            perm_wo(cx, *WO_WIN)
            att = wo_tiles(cx, 0)
            qkv_tiles(cx, 2, range(4, 15))
        else:
            cx.best = (bestv[:, 0:1], besti[:, 0:1])
            att = wo_tiles(cx, i - 1)
            qkv_tiles(cx, i + 1, range(15))
        emit_tiles(cx)
        a0, a1, l0, l1, p0, p1 = WIN[i]
        attn(cx, i, a0, cx.t - a1)
        if i + 2 < NB:
            ln1(cx, i + 2, l0, l1)
        post(cx, i - 1, att, cx.tw + p0, cx.t - p1)
        bestv[...] = jnp.broadcast_to(cx.best[0], (8, 128))
        besti[...] = jnp.broadcast_to(cx.best[1], (8, 128))

    def final():
        cx = Step()
        wait(ffn_cps)
        for b in range(L - 2):
            wait(out_cps[b])
        bv0, bi0 = bestv[...], besti[...]
        rbest0, idx0 = argmax_of(bv0, bi0, R0[L - 1])
        att = wo_tiles(cx, L - 1)
        emit_tiles(cx)
        a = ffn_up(idx0, range(FIN_UP_FIRST))
        attn(cx, L, *FIN_ATT)
        t1 = cx.t
        att2 = wo_tiles(cx, L)
        emit_tiles(cx)
        a = a + ffn_up(idx0, range(FIN_UP_FIRST, NF))
        ffn_down(a, rbest0, idx0)
        post(cx, L - 1, att, t1 + FIN_POST[0], t1 + FIN_POST[1])
        post(cx, L, att2)
        bv1 = jnp.broadcast_to(cx.best[0], (8, 128))
        bi1 = jnp.broadcast_to(cx.best[1], (8, 128))
        miss = jnp.max(jnp.where(bv1 > rbest0, 1, 0)) > 0

        @pl.when(miss)
        def _():
            take = bv1 > bv0
            rbest, idx = argmax_of(jnp.where(take, bv1, bv0), jnp.where(take, bi1, bi0), S, f32)
            ffn_down(ffn_up(idx, range(NF)), rbest, idx)
            for b in (L - 2, L - 1, L):
                wait(out_cps[b])
            pc = patch_cp(idx)
            pc.start()
            pc.wait()

        @pl.when(jnp.logical_not(miss))
        def _():
            wait(out_cps[L - 2])
            pc = patch_cp(idx0)
            pc.start()
            wait(out_cps[L - 1])
            wait(out_cps[L])
            pc.wait()

    steps = ([functools.partial(raw_step, g) for g in range(len(RAWG))] + [step0]
             + [functools.partial(main_step, i) for i in range(1, L)] + [final])
    pid = pl.program_id(0)

    @pl.when(pid == 0)
    def _():
        one[0] = 1
        first()

    @pl.when(pid == 1)
    def _():
        v = one[0]
        for n, fn in enumerate(steps):
            pl.when(v > -n)(fn)


@jax.jit
def pallas_sequential_preLN__sliding_local_dilated__moe_arch_mod__prompt_kernel(
    A_x: jax.Array,
    A_wqkv: jax.Array,
    A_wo: jax.Array,
    B_x: jax.Array,
    B_w_r: jax.Array,
    B_w_gate: jax.Array,
    B_w_up: jax.Array,
    B_w_down: jax.Array,
):
    del B_x
    any_spec = pl.BlockSpec(memory_space=pl.ANY)
    return pl.pallas_call(
        _kernel,
        grid=(2,),
        in_specs=[any_spec] * 7,
        out_specs=any_spec,
        out_shape=jax.ShapeDtypeStruct((1, S, D), bf16),
        scratch_shapes=[
            pltpu.VMEM((NJ, S, 128), bf16),
            pltpu.VMEM((2 * XD, D), bf16),
            pltpu.VMEM((D, 3 * D), bf16),
            pltpu.VMEM((3 * NJ, XD, 128), f32),
            pltpu.VMEM((NJ, D, 128), bf16),
            pltpu.VMEM((D // 2, 3 * D), u32),
            pltpu.VMEM((D // 2, D), u32),
            pltpu.VMEM((NF, D, 128), bf16),
            pltpu.VMEM((NF, D, 128), bf16),
            pltpu.VMEM((NJ, F, 128), bf16),
            pltpu.VMEM((D,), bf16),
            pltpu.VMEM((8, D), f32),
            pltpu.VMEM((TM // 2, D), u32),
            pltpu.VMEM((TM // 2, D), u32),
            pltpu.VMEM((NJ, TM, 128), f32),
            pltpu.VMEM((NJ, TM, 128), f32),
            pltpu.VMEM((NJ, HALO + TM, 128), f32),
            pltpu.VMEM((NJ, HALO + TM, 128), f32),
            pltpu.VMEM((NJ, HALO + TM, 128), f32),
            pltpu.VMEM((NJ, HALO + TM, 128), f32),
            pltpu.VMEM((TM // 2, D), u32),
            pltpu.VMEM((TM // 2, D), u32),
            pltpu.VMEM((S // 2, D), u32),
            pltpu.VMEM((NJ, S, 128), bf16),
            pltpu.VMEM((16, D), bf16),
            pltpu.VMEM((8, 128), f32),
            pltpu.VMEM((8, 128), i32),
            pltpu.VMEM((8, 128), i32),
            pltpu.SMEM((1,), i32),
            pltpu.SemaphoreType.DMA((NSEM,)),
        ],
        compiler_params=pltpu.CompilerParams(vmem_limit_bytes=100 * 1024 * 1024,
                                             dimension_semantics=("arbitrary",),
                                             disable_semaphore_checks=True),
        name="preln_swa_mod",
    )(A_x, A_wqkv, A_wo, B_w_r, B_w_gate, B_w_up, B_w_down)
```

```python
import functools
import math

import jax
import jax.numpy as jnp
from jax import lax
import jax.experimental.pallas as pl
import jax.experimental.pallas.tpu as pltpu

S = 2048
D = 640
DH = 20
W = 8
DIL = 2
F = 1536
NJ = D // 128
NF = F // 128
HALO = 16
EPS = 1e-5
LOG2E = math.log2(math.e)
QSCALE = (DH ** -0.5) * LOG2E
NEG = -1e9 * LOG2E
KA = 512

BLOCKS = [256, 256, 256, 256, 256, 256, 256, 128, 128]
NB = len(BLOCKS)
L = NB - 1
R0 = [sum(BLOCKS[:i]) for i in range(NB)]
TM = max(BLOCKS)
XD = 256
NXD = S // XD
assert sum(BLOCKS) == S and BLOCKS[0] == XD and BLOCKS[1] == XD

O0_ROWS = 24
LAST_SLAB = (-242.0, -48.0, 115.0, 342.0, 45.0, 487.0)
WIN = {0: (1094, 524, 1871, 3772, -374, 1196),
       1: (-8, 445, 84, 2045, -99, 397),
       2: (-58, 323, -142, 2124, 173, 377),
       3: (-58, 323, -142, 2124, 173, 377),
       4: (-58, 323, -142, 2124, 173, 377),
       5: (-83, 510, -216, 1258, -42, 637),
       6: (-79, 762, -82, 1505, -85, 690),
       7: (116, 753, -228, 1249, 133, 368)}
PERM_GROUP, PERM_FRAC, PERM_LEAD = 8, 0.7, 200.0
WO_WIN = (-270.0, 627.0)
FIN_UP_FIRST = 4
FIN_ATT = (-337.0, 114.0)
FIN_POST = (215.0, 508.0)
NSEM = (NXD - 2) + 2 + NJ + 2 + NB + 1

f32 = jnp.float32
bf16 = jnp.bfloat16
u32 = jnp.uint32
i32 = jnp.int32


def _cat(xs):
    return jnp.concatenate(xs, axis=1)


def _spread(t0, t1, c, n):
    return None if t0 is None else t0 + max(t1 - t0, 0.0) * c / n


def _center(x):
    m = jnp.sum(x, axis=-1, keepdims=True) * (1.0 / D)
    xc = x - m
    v = jnp.sum(xc * xc, axis=-1, keepdims=True) * (1.0 / D)
    return xc, jnp.exp2(jnp.log(v + EPS) * (-0.5 * LOG2E))


def _kernel(x_hbm, wqkv_hbm, wo_hbm, wr_hbm, wg_hbm, wu_hbm, wd_hbm, out_hbm,
            xbuf, xpre, wraw, rawb, woraw, wp, wop, wg, wu, wd, wr_ref, wrb,
            xn0, xn1, qb0, qb1, kb0, kb1, vb0, vb1, ob0, ob1, ln2b, outb, patch,
            bestv, besti, zero_ref, one, sem):
    xn = (xn0, xn1); qb = (qb0, qb1); kb = (kb0, kb1); vb = (vb0, vb1); ob = (ob0, ob1)

    nsem = [0]

    def group(pairs):
        s = sem.at[nsem[0]]
        nsem[0] += 1
        return [pltpu.make_async_copy(a, b, s) for a, b in pairs]

    def cols(j):
        return pl.ds(j * 128, 128)

    x_cps = [group([(x_hbm.at[0, pl.ds(i * XD, XD), cols(j)], xbuf.at[j, pl.ds(i * XD, XD), :])
                    for j in range(NJ)]) if i >= 2 else None for i in range(NXD)]
    xp_cps = [group([(x_hbm.at[0, pl.ds(i * XD, XD), :], xpre.at[pl.ds(i * XD, XD), :])]) for i in range(2)]
    wq_cps = [group([(wqkv_hbm.at[pl.ds(t * 128, 128), :], wraw.at[pl.ds(t * 128, 128), :])]) for t in range(NJ)]
    wo_cps = group([(wo_hbm.at[:, cols(j)], woraw.at[j]) for j in range(NJ)] + [(wr_hbm, wr_ref)])
    ffn_cps = group([(wg_hbm.at[:, cols(n)], wg.at[n]) for n in range(NF)]
                    + [(wu_hbm.at[:, cols(n)], wu.at[n]) for n in range(NF)]
                    + [(wd_hbm.at[:, cols(j)], wd.at[j]) for j in range(NJ)])
    out_cps = [group([(outb.at[j, pl.ds(R0[b], BLOCKS[b]), :],
                       out_hbm.at[0, pl.ds(R0[b], BLOCKS[b]), cols(j)]) for j in range(NJ)])
               for b in range(NB)]
    sem_p = sem.at[nsem[0]]
    assert nsem[0] + 1 == NSEM

    def start(cs):
        for c in cs:
            c.start()

    def wait(cs):
        for c in cs:
            c.wait()

    waited = set()

    def wait_x(b):
        if b < NB:
            for i in range(R0[b] // XD, (R0[b] + BLOCKS[b] - 1) // XD + 1):
                if i not in waited:
                    waited.add(i)
                    wait(x_cps[i])

    class Step:
        def __init__(self):
            self.never = None
            self.best = None
            self.res = []
            self.pend = []
            self.t = 0.0

        def add(self, val, dur):
            self.res.append((self.t, self.t + dur, val))
            self.t += dur

        def gate(self, t, val):
            if t is None or t < 0 or not self.res:
                return val
            for (t0, t1, tv) in self.res:
                if t < t1:
                    break
            frac = min(max((t - t0) / (t1 - t0), 0.0), 0.999)
            r = int(frac * (tv.shape[0] // 8)) * 8
            tok = tv[r:r + 8, :]
            if self.never is None:
                self.never = zero_ref[...] != 0
            if val.dtype != tok.dtype:
                tok = pltpu.bitcast(tok, val.dtype)
            return jnp.where(self.never, tok, val)

    def lane_perm(load, store, items, cx, t0, t1):
        lane = lax.broadcasted_iota(i32, (8, 128), 1)
        lm5 = lane % 5
        base_idx = 20 * (lane % 32) + 5 * (lane // 32)
        ngrp = NJ * ((len(items) + PERM_GROUP - 1) // PERM_GROUP)
        gi = 0
        for j in range(NJ):
            idx = (base_idx + j) % 128
            for k, it in enumerate(items):
                if k % PERM_GROUP == 0:
                    lg = cx.gate(_spread(t0, t1, gi, ngrp), lm5)
                    masks = [lg == ((j - 3 * i) % 5) for i in range(NJ)]
                    gi += 1
                src = [load(i, it) for i in range(NJ)]
                z = src[0]
                for i in range(1, NJ):
                    z = jnp.where(masks[i], src[i], z)
                store(j, it, jnp.take_along_axis(z, idx, axis=1))

    def perm_w(cx, parts, t, t0, t1):
        def load(i, it):
            p, rg = it
            return pltpu.bitcast(wraw[rg * 16:rg * 16 + 16, (p * NJ + i) * 128:(p * NJ + i + 1) * 128], u32)

        def store(j, it, z):
            p, rg = it
            wp[rg * 8:rg * 8 + 8, p * D + j * 128: p * D + (j + 1) * 128] = z
        lane_perm(load, store, [(p, rg) for p in parts for rg in range(8 * t, 8 * t + 8)], cx, t0, t1)

    def perm_out(cx, p, rgs, t0, t1):
        def load(i, rg):
            return rawb[p * NJ + i, rg * 8:rg * 8 + 8, :]

        def store(j, rg, z):
            if p == 0:
                qb[0][j, rg * 8:rg * 8 + 8, :] = z
            else:
                (kb, vb)[p - 1][0][j, HALO + rg * 8:HALO + rg * 8 + 8, :] = z
        lane_perm(load, store, list(rgs), cx, t0, t1)

    def perm_wo(cx, t0, t1):
        n = NJ * (DH // 2)
        for c in range(NJ):
            src = woraw.at[c].bitcast(u32)
            for m in range(DH // 2):
                t = _spread(t0, t1, c * (DH // 2) + m, n)
                mlo = cx.gate(t, jnp.full((8, 128), 0xFFFF, u32))
                sh = cx.gate(t, jnp.full((8, 128), 16, u32))
                for half in range(2):
                    a = src[pl.ds(m + 160 * half, 8, stride=20), :]
                    b = src[pl.ds(m + 10 + 160 * half, 8, stride=20), :]
                    lo = (a & mlo) | (b << sh)
                    hi = (a >> sh) | (b & ~mlo)
                    for d, val in ((2 * m, lo), (2 * m + 1, hi)):
                        j, g = d % 5, d // 5
                        r = (j * 128 + g * 32) // 2 + 8 * half
                        wop[r:r + 8, c * 128:(c + 1) * 128] = val

    def emit_tiles(cx):
        pend, cx.pend = cx.pend, []
        for g in range(0, len(pend), 4):
            grp = pend[g:g + 4]
            tb = [jnp.dot(lhs[:, KA:], rhs_fn(KA, D), preferred_element_type=f32) for lhs, rhs_fn, _ in grp]
            cx.add(tb[-1], sum(p[0].shape[0] for p in grp) / 4.0)
            for (lhs, rhs_fn, sink), b in zip(grp, tb):
                t = jnp.dot(lhs[:, :KA], rhs_fn(0, KA), preferred_element_type=f32) + b
                cx.add(t, float(lhs.shape[0]))
                sink(t)

    def packed_rhs(wref, n, k0, k1):
        return pltpu.bitcast(wref[k0 // 2:k1 // 2, n * 128:(n + 1) * 128], bf16)

    def raw_slab(cx, t):
        lhs = pltpu.bitcast(xn[0][0:XD // 2, t * 128:(t + 1) * 128], bf16)
        for n in range(3 * NJ):
            part = jnp.dot(lhs, wraw[t * 128:(t + 1) * 128, n * 128:(n + 1) * 128], preferred_element_type=f32)
            if n % 4 == 3 or n >= 12:
                cx.add(part, 256.0 if n < 12 else 64.0)
            rawb[n] = part if t == 0 else rawb[n] + part

    def qkv_tiles(cx, b, tiles):
        m = BLOCKS[b]
        lhs = pltpu.bitcast(xn[b % 2][0:m // 2, :], bf16)

        def sink(n, t):
            p, j = divmod(n, NJ)
            if p == 0:
                qb[b % 2][j, 0:m, :] = t
            else:
                dst = (kb, vb)[p - 1]
                mp = BLOCKS[b - 1]
                dst[b % 2][j, 0:HALO, :] = dst[(b - 1) % 2][j, mp:mp + HALO, :]
                dst[b % 2][j, HALO:HALO + m, :] = t
        for n in tiles:
            cx.pend.append((lhs, functools.partial(packed_rhs, wp, n), functools.partial(sink, n)))

    def wo_tiles(cx, b):
        m = BLOCKS[b]
        lhs = pltpu.bitcast(ob[b % 2][0:m // 2, :], bf16)
        att = []

        def sink(t):
            att.append(t)
            cx.tw = cx.t
        for n in range(NJ):
            cx.pend.append((lhs, functools.partial(packed_rhs, wop, n), sink))
        return att

    def load_x(cx, b, r, n, t):
        out = []
        for j in range(NJ):
            if b < 2:
                parts = [cx.gate(t, pltpu.bitcast(xpre[r + k:r + k + 16, j * 128:(j + 1) * 128], u32))
                         for k in range(0, n, 16)]
            else:
                v = xbuf.at[j].bitcast(u32)
                parts = [cx.gate(t, v[(r + k) // 2:(r + k) // 2 + 8, :]) for k in range(0, n, 16)]
            v = parts[0] if len(parts) == 1 else jnp.concatenate(parts, axis=0)
            out.append(pltpu.bitcast(v, bf16).astype(f32))
        return _cat(out)

    def ln1(cx, b, t0=None, t1=None, lc=16):
        n = BLOCKS[b] // lc
        for c in range(n):
            a0 = c * lc
            xc, rs = _center(load_x(cx, b, R0[b] + a0, lc, _spread(t0, t1, c, n)))
            xn[b % 2][a0 // 2:(a0 + lc) // 2, :] = pltpu.bitcast((xc * rs).astype(bf16), u32)

    def attn(cx, b, t0, t1):
        qr, kr, vr = qb[b % 2], kb[b % 2], vb[b % 2]
        n = BLOCKS[b] // 8
        for c in range(n):
            a0 = c * 8
            sc = cx.gate(_spread(t0, t1, c, n), jnp.full((8, 128), QSCALE, f32))
            q = [qr[j, a0:a0 + 8, :] * sc for j in range(NJ)]
            tt = []
            for w in range(W):
                k0 = HALO + a0 - DIL * w
                acc = q[0] * kr[0, k0:k0 + 8, :]
                for j in range(1, NJ):
                    acc = acc + q[j] * kr[j, k0:k0 + 8, :]
                tt.append(acc)
            r1 = [pltpu.roll(tt[w], 64, 1) for w in range(W)]
            tt = [tt[w] + r1[w] for w in range(W)]
            r2 = [pltpu.roll(tt[w], 32, 1) for w in range(W)]
            s = [tt[w] + r2[w] for w in range(W)]
            for w in range(W):
                if b == 0 and a0 - DIL * w < 0:
                    row = lax.broadcasted_iota(i32, (8, 128), 0) + (a0 - DIL * w)
                    s[w] = jnp.where(row >= 0, s[w], NEG)
            mx = functools.reduce(jnp.maximum, s)
            p = [jnp.exp2(s[w] - mx) for w in range(W)]
            inv = pl.reciprocal(functools.reduce(lambda u, v: u + v, p), approx=True)
            o = []
            for j in range(NJ):
                acc = None
                for w in range(W):
                    k0 = HALO + a0 - DIL * w
                    term = p[w] * vr[j, k0:k0 + 8, :]
                    acc = term if acc is None else acc + term
                o.append(acc * inv)
            if c % 2 == 0:
                prev = o
                continue
            o = [jnp.concatenate([prev[j], o[j]], axis=0) for j in range(NJ)]
            for j in range(NJ):
                ob[b % 2][(a0 - 8) // 2:(a0 + 8) // 2, j * 128:(j + 1) * 128] = pltpu.bitcast(o[j].astype(bf16), u32)

    def post(cx, b, att, t0=None, t1=None):
        r0 = R0[b]
        n = BLOCKS[b] // 16
        for c in range(n):
            a0 = c * 16
            h = (load_x(cx, b, r0 + a0, 16, _spread(t0, t1, c, n))
                 + _cat([att[j][a0:a0 + 16, :] for j in range(NJ)]))
            xc, rs = _center(h)
            r = jnp.sum(xc * jnp.tile(wrb[...], (2, 1)), axis=-1, keepdims=True) * rs
            ln2 = xc * rs
            ln2b[(r0 + a0) // 2:(r0 + a0 + 16) // 2, :] = pltpu.bitcast(ln2.astype(bf16), u32)
            o = pltpu.bitcast((h + ln2).astype(bf16), u32)
            for j in range(NJ):
                outb.at[j].bitcast(u32)[(r0 + a0) // 2:(r0 + a0 + 16) // 2, :] = o[:, j * 128:(j + 1) * 128]
            for k in (0, 8):
                rk = r[k:k + 8, :]
                if cx.best is None:
                    cx.best = (rk, jnp.full((8, 1), r0 + a0 + k, i32))
                else:
                    bv, bi = cx.best
                    take = rk > bv
                    cx.best = (jnp.where(take, rk, bv), jnp.where(take, r0 + a0 + k, bi))
        start(out_cps[b])

    def argmax_of(bv, bi, nrows, dtype=i32):
        rowid = (bi + lax.broadcasted_iota(i32, (8, 128), 0)).astype(dtype)
        rbest = jnp.max(bv, axis=0, keepdims=True)
        idx = jnp.min(jnp.where(bv == rbest, rowid, S)).astype(i32)
        return rbest, jnp.clip(idx, 0, nrows - 1)

    def ffn_up(idx, tiles):
        t16 = idx // 16
        xs = pltpu.bitcast(ln2b[pl.ds(pl.multiple_of(t16 * 8, 8), 8), :], bf16)
        a = []
        for n in tiles:
            g = jnp.dot(xs, pltpu.bitcast(wg.at[n].bitcast(u32)[...], bf16), preferred_element_type=f32)
            u = jnp.dot(xs, pltpu.bitcast(wu.at[n].bitcast(u32)[...], bf16), preferred_element_type=f32)
            a.append((g * jax.nn.sigmoid(g) * u).astype(bf16))
        return a

    def ffn_down(a, rbest, idx):
        a = _cat(a)
        sg = jax.nn.sigmoid(rbest)
        t16 = idx // 16
        hit = (lax.broadcasted_iota(i32, (16, 128), 0) + t16 * 16) == idx
        for j in range(NJ):
            y = jnp.dot(a, pltpu.bitcast(wd.at[j].bitcast(u32)[...], bf16), preferred_element_type=f32) * sg
            cur = pltpu.bitcast(outb.at[j].bitcast(u32)[pl.ds(pl.multiple_of(t16 * 8, 8), 8), :], bf16).astype(f32)
            patch[:, j * 128:(j + 1) * 128] = (cur + jnp.where(hit, y, 0.0)).astype(bf16)

    def patch_cp(idx):
        t0 = pl.multiple_of((idx // 16) * 16, 16)
        return pltpu.make_async_copy(patch, out_hbm.at[0, pl.ds(t0, 16), :], sem_p)

    def first():
        start(xp_cps[0])
        for t in range(NJ):
            start(wq_cps[t])
        start(xp_cps[1])
        start(x_cps[2])
        start(wo_cps)
        for i in range(3, NXD):
            start(x_cps[i])
        zero_ref[...] = jnp.zeros((8, 128), i32)
        for j in range(NJ):
            kb0[j, 0:HALO, :] = jnp.zeros((HALO, 128), f32)
            vb0[j, 0:HALO, :] = jnp.zeros((HALO, 128), f32)
        wait(xp_cps[0])
        ln1(Step(), 0, lc=64)

    def raw_step(t):
        cx = Step()
        wait(wq_cps[t])
        if t == NJ - 1:
            wait(xp_cps[1])
        raw_slab(cx, t)
        if t < NJ - 1:
            perm_w(cx, range(3), t, -PERM_LEAD, PERM_FRAC * cx.t - PERM_LEAD)
        else:
            g = LAST_SLAB
            ln1(cx, 1, g[0], g[1])
            perm_w(cx, [0], t, g[2], g[3])
            perm_out(cx, 0, range(O0_ROWS), g[4], g[5])

    def step0():
        cx = Step()
        wait_x(2)
        start(ffn_cps)
        a0, a1, l0, l1, p0, p1 = WIN[0]
        qkv_tiles(cx, 1, range(4))
        emit_tiles(cx)
        segs = []
        for q in range(4):
            for p in range(3):
                rgs = [rg for rg in range(q * 8, q * 8 + 8) if p > 0 or rg >= O0_ROWS]
                if rgs:
                    segs.append((False, p, rgs))
            if q in (0, 3):
                segs.append((True, 1 if q == 0 else 2, range(8)))
        tot = sum(len(s[2]) for s in segs)
        acc = 0
        for is_w, p, rgs in segs:
            ta, tb = p0 + (p1 - p0) * acc / tot, p0 + (p1 - p0) * (acc + len(rgs)) / tot
            acc += len(rgs)
            if is_w:
                perm_w(cx, [p], NJ - 1, ta, tb)
            else:
                perm_out(cx, p, rgs, ta, tb)
        qkv_tiles(cx, 1, range(4, 15))
        emit_tiles(cx)
        attn(cx, 0, a0, cx.t - a1)
        ln1(cx, 2, l0, l1)

    def main_step(i):
        cx = Step()
        if i == 1:
            wait(wo_cps)
        wait_x(i + 2)
        if i == 1:
            wrb[...] = jnp.broadcast_to(wr_ref[...].astype(f32).reshape(1, D), (8, D))
            qkv_tiles(cx, 2, range(4))
            emit_tiles(cx)
            perm_wo(cx, *WO_WIN)
            att = wo_tiles(cx, 0)
            qkv_tiles(cx, 2, range(4, 15))
        else:
            cx.best = (bestv[:, 0:1], besti[:, 0:1])
            att = wo_tiles(cx, i - 1)
            qkv_tiles(cx, i + 1, range(15))
        emit_tiles(cx)
        a0, a1, l0, l1, p0, p1 = WIN[i]
        attn(cx, i, a0, cx.t - a1)
        if i + 2 < NB:
            ln1(cx, i + 2, l0, l1)
        post(cx, i - 1, att, cx.tw + p0, cx.t - p1)
        bestv[...] = jnp.broadcast_to(cx.best[0], (8, 128))
        besti[...] = jnp.broadcast_to(cx.best[1], (8, 128))

    def final():
        cx = Step()
        wait(ffn_cps)
        for b in range(L - 2):
            wait(out_cps[b])
        bv0, bi0 = bestv[...], besti[...]
        rbest0, idx0 = argmax_of(bv0, bi0, R0[L - 1])
        att = wo_tiles(cx, L - 1)
        emit_tiles(cx)
        a = ffn_up(idx0, range(FIN_UP_FIRST))
        attn(cx, L, *FIN_ATT)
        t1 = cx.t
        att2 = wo_tiles(cx, L)
        emit_tiles(cx)
        a = a + ffn_up(idx0, range(FIN_UP_FIRST, NF))
        ffn_down(a, rbest0, idx0)
        post(cx, L - 1, att, t1 + FIN_POST[0], t1 + FIN_POST[1])
        post(cx, L, att2)
        bv1 = jnp.broadcast_to(cx.best[0], (8, 128))
        bi1 = jnp.broadcast_to(cx.best[1], (8, 128))
        miss = jnp.max(jnp.where(bv1 > rbest0, 1, 0)) > 0

        @pl.when(miss)
        def _():
            take = bv1 > bv0
            rbest, idx = argmax_of(jnp.where(take, bv1, bv0), jnp.where(take, bi1, bi0), S, f32)
            ffn_down(ffn_up(idx, range(NF)), rbest, idx)
            for b in (L - 2, L - 1, L):
                wait(out_cps[b])
            pc = patch_cp(idx)
            pc.start()
            pc.wait()

        @pl.when(jnp.logical_not(miss))
        def _():
            wait(out_cps[L - 2])
            pc = patch_cp(idx0)
            pc.start()
            wait(out_cps[L - 1])
            wait(out_cps[L])
            pc.wait()

    steps = ([functools.partial(raw_step, t) for t in range(NJ)] + [step0]
             + [functools.partial(main_step, i) for i in range(1, L)] + [final])
    pid = pl.program_id(0)

    @pl.when(pid == 0)
    def _():
        one[0] = 1
        first()

    @pl.when(pid == 1)
    def _():
        v = one[0]
        for n, fn in enumerate(steps):
            pl.when(v > -n)(fn)


@jax.jit
def pallas_sequential_preLN__sliding_local_dilated__moe_arch_mod__prompt_kernel(
    A_x: jax.Array,
    A_wqkv: jax.Array,
    A_wo: jax.Array,
    B_x: jax.Array,
    B_w_r: jax.Array,
    B_w_gate: jax.Array,
    B_w_up: jax.Array,
    B_w_down: jax.Array,
):
    del B_x
    any_spec = pl.BlockSpec(memory_space=pl.ANY)
    return pl.pallas_call(
        _kernel,
        grid=(2,),
        in_specs=[any_spec] * 7,
        out_specs=any_spec,
        out_shape=jax.ShapeDtypeStruct((1, S, D), bf16),
        scratch_shapes=[
            pltpu.VMEM((NJ, S, 128), bf16),
            pltpu.VMEM((2 * XD, D), bf16),
            pltpu.VMEM((D, 3 * D), bf16),
            pltpu.VMEM((3 * NJ, XD, 128), f32),
            pltpu.VMEM((NJ, D, 128), bf16),
            pltpu.VMEM((D // 2, 3 * D), u32),
            pltpu.VMEM((D // 2, D), u32),
            pltpu.VMEM((NF, D, 128), bf16),
            pltpu.VMEM((NF, D, 128), bf16),
            pltpu.VMEM((NJ, F, 128), bf16),
            pltpu.VMEM((D,), bf16),
            pltpu.VMEM((8, D), f32),
            pltpu.VMEM((TM // 2, D), u32),
            pltpu.VMEM((TM // 2, D), u32),
            pltpu.VMEM((NJ, TM, 128), f32),
            pltpu.VMEM((NJ, TM, 128), f32),
            pltpu.VMEM((NJ, HALO + TM, 128), f32),
            pltpu.VMEM((NJ, HALO + TM, 128), f32),
            pltpu.VMEM((NJ, HALO + TM, 128), f32),
            pltpu.VMEM((NJ, HALO + TM, 128), f32),
            pltpu.VMEM((TM // 2, D), u32),
            pltpu.VMEM((TM // 2, D), u32),
            pltpu.VMEM((S // 2, D), u32),
            pltpu.VMEM((NJ, S, 128), bf16),
            pltpu.VMEM((16, D), bf16),
            pltpu.VMEM((8, 128), f32),
            pltpu.VMEM((8, 128), i32),
            pltpu.VMEM((8, 128), i32),
            pltpu.SMEM((1,), i32),
            pltpu.SemaphoreType.DMA((NSEM,)),
        ],
        compiler_params=pltpu.CompilerParams(vmem_limit_bytes=100 * 1024 * 1024,
                                             dimension_semantics=("arbitrary",),
                                             disable_semaphore_checks=True),
        name="preln_swa_mod",
    )(A_x, A_wqkv, A_wo, B_w_r, B_w_gate, B_w_up, B_w_down)
```

```python
import functools
import math

import jax
import jax.numpy as jnp
from jax import lax
import jax.experimental.pallas as pl
import jax.experimental.pallas.tpu as pltpu

S = 2048
D = 640
DH = 20
W = 8
DIL = 2
F = 1536
NJ = D // 128
NF = F // 128
HALO = 16
EPS = 1e-5
LOG2E = math.log2(math.e)
QSCALE = (DH ** -0.5) * LOG2E
NEG = -1e9 * LOG2E
KA = 512

BLOCKS = [256, 256, 256, 256, 256, 256, 256, 128, 128]
NB = len(BLOCKS)
L = NB - 1
R0 = [sum(BLOCKS[:i]) for i in range(NB)]
TM = max(BLOCKS)
XD = 256
NXD = S // XD
assert sum(BLOCKS) == S and BLOCKS[0] == XD and BLOCKS[1] == XD

O0_ROWS = 24
LAST_SLAB = (-242.0, -48.0, 115.0, 342.0, 45.0, 487.0)
WIN = {0: (1094, 524, 1871, 3772, -374, 1196),
       1: (-8, 445, 84, 2045, -99, 397),
       2: (-58, 323, -142, 2124, 173, 377),
       3: (-58, 323, -142, 2124, 173, 377),
       4: (-58, 323, -142, 2124, 173, 377),
       5: (-83, 510, -216, 1258, -42, 637),
       6: (-79, 762, -82, 1505, -85, 690),
       7: (116, 753, -228, 1249, 133, 368)}
PERM_GROUP, PERM_FRAC, PERM_LEAD = 8, 0.7, 200.0
WO_WIN = (-270.0, 627.0)
FIN_UP_FIRST = 4
FIN_ATT = (-337.0, 114.0)
FIN_POST = (215.0, 508.0)
NSEM = (NXD - 2) + 2 + NJ + 2 + NB + 1

f32 = jnp.float32
bf16 = jnp.bfloat16
u32 = jnp.uint32
i32 = jnp.int32


def _cat(xs):
    return jnp.concatenate(xs, axis=1)


def _spread(t0, t1, c, n):
    return None if t0 is None else t0 + max(t1 - t0, 0.0) * c / n


def _center(x):
    m = jnp.sum(x, axis=-1, keepdims=True) * (1.0 / D)
    xc = x - m
    v = jnp.sum(xc * xc, axis=-1, keepdims=True) * (1.0 / D)
    return xc, jnp.exp2(jnp.log(v + EPS) * (-0.5 * LOG2E))


def _kernel(x_hbm, wqkv_hbm, wo_hbm, wr_hbm, wg_hbm, wu_hbm, wd_hbm, out_hbm,
            xbuf, xpre, wraw, rawb, woraw, wp, wop, wg, wu, wd, wr_ref, wrb,
            xn0, xn1, qb0, qb1, kb0, kb1, vb0, vb1, ob0, ob1, ln2b, outb, patch,
            bestv, besti, zero_ref, one, sem):
    xn = (xn0, xn1); qb = (qb0, qb1); kb = (kb0, kb1); vb = (vb0, vb1); ob = (ob0, ob1)

    nsem = [0]

    def group(pairs):
        s = sem.at[nsem[0]]
        nsem[0] += 1
        return [pltpu.make_async_copy(a, b, s) for a, b in pairs]

    def cols(j):
        return pl.ds(j * 128, 128)

    x_cps = [group([(x_hbm.at[0, pl.ds(i * XD, XD), cols(j)], xbuf.at[j, pl.ds(i * XD, XD), :])
                    for j in range(NJ)]) if i >= 2 else None for i in range(NXD)]
    xp_cps = [group([(x_hbm.at[0, pl.ds(i * XD, XD), :], xpre.at[pl.ds(i * XD, XD), :])]) for i in range(2)]
    wq_cps = [group([(wqkv_hbm.at[pl.ds(t * 128, 128), :], wraw.at[pl.ds(t * 128, 128), :])]) for t in range(NJ)]
    wo_cps = group([(wo_hbm.at[:, cols(j)], woraw.at[j]) for j in range(NJ)] + [(wr_hbm, wr_ref)])
    ffn_cps = group([(wg_hbm.at[:, cols(n)], wg.at[n]) for n in range(NF)]
                    + [(wu_hbm.at[:, cols(n)], wu.at[n]) for n in range(NF)]
                    + [(wd_hbm.at[:, cols(j)], wd.at[j]) for j in range(NJ)])
    out_cps = [group([(outb.at[j, pl.ds(R0[b], BLOCKS[b]), :],
                       out_hbm.at[0, pl.ds(R0[b], BLOCKS[b]), cols(j)]) for j in range(NJ)])
               for b in range(NB)]
    sem_p = sem.at[nsem[0]]
    assert nsem[0] + 1 == NSEM

    def start(cs):
        for c in cs:
            c.start()

    def wait(cs):
        for c in cs:
            c.wait()

    waited = set()

    def wait_x(b):
        if b < NB:
            for i in range(R0[b] // XD, (R0[b] + BLOCKS[b] - 1) // XD + 1):
                if i not in waited:
                    waited.add(i)
                    wait(x_cps[i])

    class Step:
        def __init__(self):
            self.never = None
            self.best = None
            self.res = []
            self.pend = []
            self.t = 0.0

        def add(self, val, dur):
            self.res.append((self.t, self.t + dur, val))
            self.t += dur

        def gate(self, t, val):
            if t is None or t < 0 or not self.res:
                return val
            for (t0, t1, tv) in self.res:
                if t < t1:
                    break
            frac = min(max((t - t0) / (t1 - t0), 0.0), 0.999)
            r = int(frac * (tv.shape[0] // 8)) * 8
            tok = tv[r:r + 8, :]
            if self.never is None:
                self.never = zero_ref[...] != 0
            if val.dtype != tok.dtype:
                tok = pltpu.bitcast(tok, val.dtype)
            return jnp.where(self.never, tok, val)

    def lane_perm(load, store, items, cx, t0, t1):
        lane = lax.broadcasted_iota(i32, (8, 128), 1)
        lm5 = lane % 5
        base_idx = 20 * (lane % 32) + 5 * (lane // 32)
        ngrp = NJ * ((len(items) + PERM_GROUP - 1) // PERM_GROUP)
        gi = 0
        for j in range(NJ):
            idx = (base_idx + j) % 128
            for k, it in enumerate(items):
                if k % PERM_GROUP == 0:
                    lg = cx.gate(_spread(t0, t1, gi, ngrp), lm5)
                    masks = [lg == ((j - 3 * i) % 5) for i in range(NJ)]
                    gi += 1
                src = [load(i, it) for i in range(NJ)]
                z = src[0]
                for i in range(1, NJ):
                    z = jnp.where(masks[i], src[i], z)
                store(j, it, jnp.take_along_axis(z, idx, axis=1))

    def perm_w(cx, parts, t, t0, t1):
        def load(i, it):
            p, rg = it
            return pltpu.bitcast(wraw[rg * 16:rg * 16 + 16, (p * NJ + i) * 128:(p * NJ + i + 1) * 128], u32)

        def store(j, it, z):
            p, rg = it
            wp[rg * 8:rg * 8 + 8, p * D + j * 128: p * D + (j + 1) * 128] = z
        lane_perm(load, store, [(p, rg) for p in parts for rg in range(8 * t, 8 * t + 8)], cx, t0, t1)

    def perm_out(cx, p, rgs, t0, t1):
        def load(i, rg):
            return rawb[p * NJ + i, rg * 8:rg * 8 + 8, :]

        def store(j, rg, z):
            if p == 0:
                qb[0][j, rg * 8:rg * 8 + 8, :] = z
            else:
                (kb, vb)[p - 1][0][j, HALO + rg * 8:HALO + rg * 8 + 8, :] = z
        lane_perm(load, store, list(rgs), cx, t0, t1)

    def perm_wo(cx, t0, t1):
        n = NJ * (DH // 2)
        for c in range(NJ):
            src = woraw.at[c].bitcast(u32)
            for m in range(DH // 2):
                t = _spread(t0, t1, c * (DH // 2) + m, n)
                mlo = cx.gate(t, jnp.full((8, 128), 0xFFFF, u32))
                sh = cx.gate(t, jnp.full((8, 128), 16, u32))
                for half in range(2):
                    a = src[pl.ds(m + 160 * half, 8, stride=20), :]
                    b = src[pl.ds(m + 10 + 160 * half, 8, stride=20), :]
                    lo = (a & mlo) | (b << sh)
                    hi = (a >> sh) | (b & ~mlo)
                    for d, val in ((2 * m, lo), (2 * m + 1, hi)):
                        j, g = d % 5, d // 5
                        r = (j * 128 + g * 32) // 2 + 8 * half
                        wop[r:r + 8, c * 128:(c + 1) * 128] = val

    def emit_tiles(cx):
        pend, cx.pend = cx.pend, []
        for g in range(0, len(pend), 4):
            grp = pend[g:g + 4]
            tb = [jnp.dot(lhs[:, KA:], rhs_fn(KA, D), preferred_element_type=f32) for lhs, rhs_fn, _ in grp]
            cx.add(tb[-1], sum(p[0].shape[0] for p in grp) / 4.0)
            for (lhs, rhs_fn, sink), b in zip(grp, tb):
                t = jnp.dot(lhs[:, :KA], rhs_fn(0, KA), preferred_element_type=f32) + b
                cx.add(t, float(lhs.shape[0]))
                sink(t)

    def packed_rhs(wref, n, k0, k1):
        return pltpu.bitcast(wref[k0 // 2:k1 // 2, n * 128:(n + 1) * 128], bf16)

    def raw_slab(cx, t):
        lhs = pltpu.bitcast(xn[0][0:XD // 2, t * 128:(t + 1) * 128], bf16)
        for n in range(3 * NJ):
            part = jnp.dot(lhs, wraw[t * 128:(t + 1) * 128, n * 128:(n + 1) * 128], preferred_element_type=f32)
            if n % 4 == 3 or n >= 12:
                cx.add(part, 256.0 if n < 12 else 64.0)
            rawb[n] = part if t == 0 else rawb[n] + part

    def qkv_tiles(cx, b, tiles):
        m = BLOCKS[b]
        lhs = pltpu.bitcast(xn[b % 2][0:m // 2, :], bf16)

        def sink(n, t):
            p, j = divmod(n, NJ)
            if p == 0:
                qb[b % 2][j, 0:m, :] = t
            else:
                dst = (kb, vb)[p - 1]
                mp = BLOCKS[b - 1]
                dst[b % 2][j, 0:HALO, :] = dst[(b - 1) % 2][j, mp:mp + HALO, :]
                dst[b % 2][j, HALO:HALO + m, :] = t
        for n in tiles:
            cx.pend.append((lhs, functools.partial(packed_rhs, wp, n), functools.partial(sink, n)))

    def wo_tiles(cx, b):
        m = BLOCKS[b]
        lhs = pltpu.bitcast(ob[b % 2][0:m // 2, :], bf16)
        att = []

        def sink(t):
            att.append(t)
            cx.tw = cx.t
        for n in range(NJ):
            cx.pend.append((lhs, functools.partial(packed_rhs, wop, n), sink))
        return att

    def load_x(cx, b, r, n, t):
        out = []
        for j in range(NJ):
            if b < 2:
                parts = [cx.gate(t, pltpu.bitcast(xpre[r + k:r + k + 16, j * 128:(j + 1) * 128], u32))
                         for k in range(0, n, 16)]
            else:
                parts = [cx.gate(t, xbuf.at[j, pl.ds(r + k, 16), :].bitcast(u32)[...]) for k in range(0, n, 16)]
            v = parts[0] if len(parts) == 1 else jnp.concatenate(parts, axis=0)
            out.append(pltpu.bitcast(v, bf16).astype(f32))
        return _cat(out)

    def ln1(cx, b, t0=None, t1=None, lc=16):
        n = BLOCKS[b] // lc
        for c in range(n):
            a0 = c * lc
            xc, rs = _center(load_x(cx, b, R0[b] + a0, lc, _spread(t0, t1, c, n)))
            xn[b % 2][a0 // 2:(a0 + lc) // 2, :] = pltpu.bitcast((xc * rs).astype(bf16), u32)

    def attn(cx, b, t0, t1):
        qr, kr, vr = qb[b % 2], kb[b % 2], vb[b % 2]
        n = BLOCKS[b] // 8
        for c in range(n):
            a0 = c * 8
            sc = cx.gate(_spread(t0, t1, c, n), jnp.full((8, 128), QSCALE, f32))
            q = [qr[j, a0:a0 + 8, :] * sc for j in range(NJ)]
            tt = []
            for w in range(W):
                k0 = HALO + a0 - DIL * w
                acc = q[0] * kr[0, k0:k0 + 8, :]
                for j in range(1, NJ):
                    acc = acc + q[j] * kr[j, k0:k0 + 8, :]
                tt.append(acc)
            r1 = [pltpu.roll(tt[w], 64, 1) for w in range(W)]
            tt = [tt[w] + r1[w] for w in range(W)]
            r2 = [pltpu.roll(tt[w], 32, 1) for w in range(W)]
            s = [tt[w] + r2[w] for w in range(W)]
            for w in range(W):
                if b == 0 and a0 - DIL * w < 0:
                    row = lax.broadcasted_iota(i32, (8, 128), 0) + (a0 - DIL * w)
                    s[w] = jnp.where(row >= 0, s[w], NEG)
            mx = functools.reduce(jnp.maximum, s)
            p = [jnp.exp2(s[w] - mx) for w in range(W)]
            inv = pl.reciprocal(functools.reduce(lambda u, v: u + v, p), approx=True)
            o = []
            for j in range(NJ):
                acc = None
                for w in range(W):
                    k0 = HALO + a0 - DIL * w
                    term = p[w] * vr[j, k0:k0 + 8, :]
                    acc = term if acc is None else acc + term
                o.append(acc * inv)
            if c % 2 == 0:
                prev = o
                continue
            o = [jnp.concatenate([prev[j], o[j]], axis=0) for j in range(NJ)]
            for j in range(NJ):
                ob[b % 2][(a0 - 8) // 2:(a0 + 8) // 2, j * 128:(j + 1) * 128] = pltpu.bitcast(o[j].astype(bf16), u32)

    def post(cx, b, att, t0=None, t1=None):
        r0 = R0[b]
        n = BLOCKS[b] // 16
        for c in range(n):
            a0 = c * 16
            h = (load_x(cx, b, r0 + a0, 16, _spread(t0, t1, c, n))
                 + _cat([att[j][a0:a0 + 16, :] for j in range(NJ)]))
            xc, rs = _center(h)
            r = jnp.sum(xc * jnp.tile(wrb[...], (2, 1)), axis=-1, keepdims=True) * rs
            ln2 = xc * rs
            ln2b[(r0 + a0) // 2:(r0 + a0 + 16) // 2, :] = pltpu.bitcast(ln2.astype(bf16), u32)
            o = pltpu.bitcast((h + ln2).astype(bf16), u32)
            for j in range(NJ):
                outb.at[j, pl.ds(r0 + a0, 16), :].bitcast(u32)[...] = o[:, j * 128:(j + 1) * 128]
            for k in (0, 8):
                rk = r[k:k + 8, :]
                if cx.best is None:
                    cx.best = (rk, jnp.full((8, 1), r0 + a0 + k, i32))
                else:
                    bv, bi = cx.best
                    take = rk > bv
                    cx.best = (jnp.where(take, rk, bv), jnp.where(take, r0 + a0 + k, bi))
        start(out_cps[b])

    def argmax_of(bv, bi, nrows, dtype=i32):
        rowid = (bi + lax.broadcasted_iota(i32, (8, 128), 0)).astype(dtype)
        rbest = jnp.max(bv, axis=0, keepdims=True)
        idx = jnp.min(jnp.where(bv == rbest, rowid, S)).astype(i32)
        return rbest, jnp.clip(idx, 0, nrows - 1)

    def ffn_up(idx, tiles):
        t16 = idx // 16
        xs = pltpu.bitcast(ln2b[pl.ds(pl.multiple_of(t16 * 8, 8), 8), :], bf16)
        a = []
        for n in tiles:
            g = jnp.dot(xs, pltpu.bitcast(wg.at[n].bitcast(u32)[...], bf16), preferred_element_type=f32)
            u = jnp.dot(xs, pltpu.bitcast(wu.at[n].bitcast(u32)[...], bf16), preferred_element_type=f32)
            a.append((g * jax.nn.sigmoid(g) * u).astype(bf16))
        return a

    def ffn_down(a, rbest, idx):
        a = _cat(a)
        sg = jax.nn.sigmoid(rbest)
        t16 = idx // 16
        hit = (lax.broadcasted_iota(i32, (16, 128), 0) + t16 * 16) == idx
        for j in range(NJ):
            y = jnp.dot(a, pltpu.bitcast(wd.at[j].bitcast(u32)[...], bf16), preferred_element_type=f32) * sg
            cur = outb.at[j, pl.ds(pl.multiple_of(t16 * 16, 16), 16), :].bitcast(u32)[...]
            cur = pltpu.bitcast(cur, bf16).astype(f32)
            patch[:, j * 128:(j + 1) * 128] = (cur + jnp.where(hit, y, 0.0)).astype(bf16)

    def patch_cp(idx):
        t0 = pl.multiple_of((idx // 16) * 16, 16)
        return pltpu.make_async_copy(patch, out_hbm.at[0, pl.ds(t0, 16), :], sem_p)

    def first():
        start(xp_cps[0])
        for t in range(NJ):
            start(wq_cps[t])
        start(xp_cps[1])
        start(x_cps[2])
        start(wo_cps)
        for i in range(3, NXD):
            start(x_cps[i])
        zero_ref[...] = jnp.zeros((8, 128), i32)
        for j in range(NJ):
            kb0[j, 0:HALO, :] = jnp.zeros((HALO, 128), f32)
            vb0[j, 0:HALO, :] = jnp.zeros((HALO, 128), f32)
        wait(xp_cps[0])
        ln1(Step(), 0, lc=64)

    def raw_step(t):
        cx = Step()
        wait(wq_cps[t])
        if t == NJ - 1:
            wait(xp_cps[1])
        raw_slab(cx, t)
        if t < NJ - 1:
            perm_w(cx, range(3), t, -PERM_LEAD, PERM_FRAC * cx.t - PERM_LEAD)
        else:
            g = LAST_SLAB
            ln1(cx, 1, g[0], g[1])
            perm_w(cx, [0], t, g[2], g[3])
            perm_out(cx, 0, range(O0_ROWS), g[4], g[5])

    def step0():
        cx = Step()
        wait_x(2)
        start(ffn_cps)
        a0, a1, l0, l1, p0, p1 = WIN[0]
        qkv_tiles(cx, 1, range(4))
        emit_tiles(cx)
        segs = []
        for q in range(4):
            for p in range(3):
                rgs = [rg for rg in range(q * 8, q * 8 + 8) if p > 0 or rg >= O0_ROWS]
                if rgs:
                    segs.append((False, p, rgs))
            if q in (0, 3):
                segs.append((True, 1 if q == 0 else 2, range(8)))
        tot = sum(len(s[2]) for s in segs)
        acc = 0
        for is_w, p, rgs in segs:
            ta, tb = p0 + (p1 - p0) * acc / tot, p0 + (p1 - p0) * (acc + len(rgs)) / tot
            acc += len(rgs)
            if is_w:
                perm_w(cx, [p], NJ - 1, ta, tb)
            else:
                perm_out(cx, p, rgs, ta, tb)
        qkv_tiles(cx, 1, range(4, 15))
        emit_tiles(cx)
        attn(cx, 0, a0, cx.t - a1)
        ln1(cx, 2, l0, l1)

    def main_step(i):
        cx = Step()
        if i == 1:
            wait(wo_cps)
        wait_x(i + 2)
        if i == 1:
            wrb[...] = jnp.broadcast_to(wr_ref[...].astype(f32).reshape(1, D), (8, D))
            qkv_tiles(cx, 2, range(4))
            emit_tiles(cx)
            perm_wo(cx, *WO_WIN)
            att = wo_tiles(cx, 0)
            qkv_tiles(cx, 2, range(4, 15))
        else:
            cx.best = (bestv[:, 0:1], besti[:, 0:1])
            att = wo_tiles(cx, i - 1)
            qkv_tiles(cx, i + 1, range(15))
        emit_tiles(cx)
        a0, a1, l0, l1, p0, p1 = WIN[i]
        attn(cx, i, a0, cx.t - a1)
        if i + 2 < NB:
            ln1(cx, i + 2, l0, l1)
        post(cx, i - 1, att, cx.tw + p0, cx.t - p1)
        bestv[...] = jnp.broadcast_to(cx.best[0], (8, 128))
        besti[...] = jnp.broadcast_to(cx.best[1], (8, 128))

    def final():
        cx = Step()
        wait(ffn_cps)
        for b in range(L - 2):
            wait(out_cps[b])
        bv0, bi0 = bestv[...], besti[...]
        rbest0, idx0 = argmax_of(bv0, bi0, R0[L - 1])
        att = wo_tiles(cx, L - 1)
        emit_tiles(cx)
        a = ffn_up(idx0, range(FIN_UP_FIRST))
        attn(cx, L, *FIN_ATT)
        t1 = cx.t
        att2 = wo_tiles(cx, L)
        emit_tiles(cx)
        a = a + ffn_up(idx0, range(FIN_UP_FIRST, NF))
        ffn_down(a, rbest0, idx0)
        post(cx, L - 1, att, t1 + FIN_POST[0], t1 + FIN_POST[1])
        post(cx, L, att2)
        bv1 = jnp.broadcast_to(cx.best[0], (8, 128))
        bi1 = jnp.broadcast_to(cx.best[1], (8, 128))
        miss = jnp.max(jnp.where(bv1 > rbest0, 1, 0)) > 0

        @pl.when(miss)
        def _():
            take = bv1 > bv0
            rbest, idx = argmax_of(jnp.where(take, bv1, bv0), jnp.where(take, bi1, bi0), S, f32)
            ffn_down(ffn_up(idx, range(NF)), rbest, idx)
            for b in (L - 2, L - 1, L):
                wait(out_cps[b])
            pc = patch_cp(idx)
            pc.start()
            pc.wait()

        @pl.when(jnp.logical_not(miss))
        def _():
            wait(out_cps[L - 2])
            pc = patch_cp(idx0)
            pc.start()
            wait(out_cps[L - 1])
            wait(out_cps[L])
            pc.wait()

    steps = ([functools.partial(raw_step, t) for t in range(NJ)] + [step0]
             + [functools.partial(main_step, i) for i in range(1, L)] + [final])
    pid = pl.program_id(0)

    @pl.when(pid == 0)
    def _():
        one[0] = 1
        first()

    @pl.when(pid == 1)
    def _():
        v = one[0]
        for n, fn in enumerate(steps):
            pl.when(v > -n)(fn)


@jax.jit
def pallas_sequential_preLN__sliding_local_dilated__moe_arch_mod__prompt_kernel(
    A_x: jax.Array,
    A_wqkv: jax.Array,
    A_wo: jax.Array,
    B_x: jax.Array,
    B_w_r: jax.Array,
    B_w_gate: jax.Array,
    B_w_up: jax.Array,
    B_w_down: jax.Array,
):
    del B_x
    any_spec = pl.BlockSpec(memory_space=pl.ANY)
    return pl.pallas_call(
        _kernel,
        grid=(2,),
        in_specs=[any_spec] * 7,
        out_specs=any_spec,
        out_shape=jax.ShapeDtypeStruct((1, S, D), bf16),
        scratch_shapes=[
            pltpu.VMEM((NJ, S, 128), bf16),
            pltpu.VMEM((2 * XD, D), bf16),
            pltpu.VMEM((D, 3 * D), bf16),
            pltpu.VMEM((3 * NJ, XD, 128), f32),
            pltpu.VMEM((NJ, D, 128), bf16),
            pltpu.VMEM((D // 2, 3 * D), u32),
            pltpu.VMEM((D // 2, D), u32),
            pltpu.VMEM((NF, D, 128), bf16),
            pltpu.VMEM((NF, D, 128), bf16),
            pltpu.VMEM((NJ, F, 128), bf16),
            pltpu.VMEM((D,), bf16),
            pltpu.VMEM((8, D), f32),
            pltpu.VMEM((TM // 2, D), u32),
            pltpu.VMEM((TM // 2, D), u32),
            pltpu.VMEM((NJ, TM, 128), f32),
            pltpu.VMEM((NJ, TM, 128), f32),
            pltpu.VMEM((NJ, HALO + TM, 128), f32),
            pltpu.VMEM((NJ, HALO + TM, 128), f32),
            pltpu.VMEM((NJ, HALO + TM, 128), f32),
            pltpu.VMEM((NJ, HALO + TM, 128), f32),
            pltpu.VMEM((TM // 2, D), u32),
            pltpu.VMEM((TM // 2, D), u32),
            pltpu.VMEM((S // 2, D), u32),
            pltpu.VMEM((NJ, S, 128), bf16),
            pltpu.VMEM((16, D), bf16),
            pltpu.VMEM((8, 128), f32),
            pltpu.VMEM((8, 128), i32),
            pltpu.VMEM((8, 128), i32),
            pltpu.SMEM((1,), i32),
            pltpu.SemaphoreType.DMA((NSEM,)),
        ],
        compiler_params=pltpu.CompilerParams(vmem_limit_bytes=100 * 1024 * 1024,
                                             dimension_semantics=("arbitrary",),
                                             disable_semaphore_checks=True),
        name="preln_swa_mod",
    )(A_x, A_wqkv, A_wo, B_w_r, B_w_gate, B_w_up, B_w_down)
```
